```python
import jax
import jax.numpy as jnp

def _softmax(x, axis=-1):
    return jax.nn.softmax(x, axis=axis)

def _gelu(x):
    return jax.nn.gelu(x, approximate=True)

def _silu(x):
    return jax.nn.silu(x)

def _sigmoid(x):
    return jax.nn.sigmoid(x)

def _layernorm(x, axis=-1, eps=1e-05):
    m = jnp.mean(x, axis=axis, keepdims=True)
    v = jnp.var(x, axis=axis, keepdims=True)
    return (x - m) / jnp.sqrt(v + eps)

def _scatter_add(tgt, idx, src, axis=0):
    return tgt.at[idx].add(src)

def _segment_sum(src, seg, n):
    return jax.ops.segment_sum(src, seg, n)

class _Rng:

    def __init__(self, key):
        self._k = key

    def _next(self):
        self._k, sub = jax.random.split(self._k)
        return sub

    def normal(self, shape):
        return jax.random.normal(self._next(), shape, dtype=jnp.bfloat16)

    def randint(self, lo, hi, shape):
        return jax.random.randint(self._next(), shape, lo, hi, dtype=jnp.int32)

    def uniform(self, shape, lo=0.0, hi=1.0):
        return jax.random.uniform(self._next(), shape, jnp.bfloat16, lo, hi)

    def permutation(self, n):
        return jax.random.permutation(self._next(), n)
kernel_name = 'recurrent_scan__memory_aug_recurrent_mem_tr__moe_arch_mod__prompt'

def setup_inputs():
    _rng = _Rng(jax.random.key(int.from_bytes(__import__("os").urandom(4), "little")))
    _w = lambda a: (lambda t: t.astype(jnp.bfloat16) if jnp.issubdtype(t.dtype, jnp.floating) else t)(jnp.asarray(a))

    def _A_setup():
        B, S, Dm = (1, 2048, 640)
        H, Dh = (32, 128)
        M, seg = (8, 32)
        seg = min(seg, S)
        S = S // seg * seg
        return {'x': _w((lambda *s: _rng.normal(s) * 0.05)(B, S, Dm)), 'mem0': _w((lambda *s: _rng.normal(s) * 0.05)(B, M, Dm)), 'Wq': _w((lambda *s: _rng.normal(s) * 0.05)(Dm, H, Dh) * Dm ** (-0.5)), 'Wk': _w((lambda *s: _rng.normal(s) * 0.05)(Dm, H, Dh) * Dm ** (-0.5)), 'Wv': _w((lambda *s: _rng.normal(s) * 0.05)(Dm, H, Dh) * Dm ** (-0.5)), 'Wo': _w((lambda *s: _rng.normal(s) * 0.05)(H, Dh, Dm) * (H * Dh) ** (-0.5)), 'seg_len': seg}
    _A_in = _A_setup()

    def _B_setup():
        B, S, D, F, C = (1, 2048, 640, 1728, 8)
        return {'x': _w((lambda *s: _rng.normal(s) * 0.05)(B, S, D)), 'w_r': _w((lambda *s: _rng.normal(s) * 0.05)(D)), 'w_gate': _w((lambda *s: _rng.normal(s) * 0.05)(D, F)), 'w_up': _w((lambda *s: _rng.normal(s) * 0.05)(D, F)), 'w_down': _w((lambda *s: _rng.normal(s) * 0.05)(F, D))}
    _B_in = _B_setup()
    return {'A_x': _A_in['x'], 'A_mem0': _A_in['mem0'], 'A_Wq': _A_in['Wq'], 'A_Wk': _A_in['Wk'], 'A_Wv': _A_in['Wv'], 'A_Wo': _A_in['Wo'], 'A_seg_len': _A_in['seg_len'], 'B_x': _B_in['x'], 'B_w_r': _B_in['w_r'], 'B_w_gate': _B_in['w_gate'], 'B_w_up': _B_in['w_up'], 'B_w_down': _B_in['w_down']}

def reference(A_x, A_mem0, A_Wq, A_Wk, A_Wv, A_Wo, A_seg_len, B_x, B_w_r, B_w_gate, B_w_up, B_w_down):

    def _A_ref(x, mem0, Wq, Wk, Wv, Wo, seg_len):
        B, S, Dm = x.shape
        H, Dh = (Wq.shape[1], Wq.shape[2])
        M = mem0.shape[1]
        scale = Dh ** (-0.5)
        n_seg = S // seg_len
        L = M + seg_len
        idx = jnp.arange(L)
        mask = (idx[:, None] < M) | (idx[:, None] >= idx[None, :])
        mem = mem0
        outs = []
        for s in range(n_seg):
            xs = x[:, s * seg_len:(s + 1) * seg_len, :].copy()
            h = jnp.concatenate([mem, xs], axis=1)
            q = jnp.einsum('btd,dhe->bhte', h, Wq)
            k = jnp.einsum('btd,dhe->bhte', h, Wk)
            v = jnp.einsum('btd,dhe->bhte', h, Wv)
            scores = jnp.einsum('bhqe,bhke->bhqk', q, k) * scale
            scores = jnp.where(mask[None, None], scores, -1000000000.0)
            p = _softmax(scores, axis=-1)
            o = jnp.einsum('bhqk,bhke->bhqe', p, v)
            o = jnp.einsum('bhte,hed->btd', o, Wo)
            mem = o[:, :M, :].copy()
            outs.append(o[:, M:, :])
        return jnp.concatenate(outs, axis=1)

    def _B_ref(x, w_r, w_gate, w_up, w_down):
        B, S, D = x.shape
        C = 8
        r = x @ w_r
        idx = jnp.argsort(-r, axis=-1)[:, :C]
        idx_e = jnp.repeat(idx.reshape(B, C, 1), D, axis=2)
        x_sel = jnp.take_along_axis(x, idx_e, axis=1)
        g = _silu(x_sel @ w_gate)
        u = x_sel @ w_up
        y = g * u @ w_down
        r_sel = _sigmoid(jnp.take_along_axis(r, idx, axis=1))
        y = y * r_sel.reshape(B, C, 1)
        b_off = (jnp.arange(B) * S).reshape(B, 1)
        flat_idx = (idx + b_off).reshape(B * C)
        zero = (x * 0.0).reshape(B * S, D)
        upd = _scatter_add(zero, flat_idx, y.reshape(B * C, D), axis=0)
        return x + upd.reshape(B, S, D)
    x = A_x
    xn = _layernorm(x, axis=-1)
    s = _A_ref(xn, A_mem0, A_Wq, A_Wk, A_Wv, A_Wo, A_seg_len)
    g = _silu(_B_ref(xn, B_w_r, B_w_gate, B_w_up, B_w_down))
    return x + s * g
```

```python
import math

import jax
import jax.numpy as jnp
from jax import lax
import jax.experimental.pallas as pl
import jax.experimental.pallas.tpu as pltpu

bf16 = jnp.bfloat16
f32 = jnp.float32
u32 = jnp.uint32
i32 = jnp.int32

S = 2048
D = 640
H = 32
DH = 128
NP = H // 2
M = 8
SEG = 32
NSEG = S // SEG
F = 1728
C = 8
CH = 8
NCH = NSEG // CH
NJ = D // 128
EPS = 1e-5
NEG = -1e30
CEXP = (DH ** -0.5) * math.log2(math.e)

LAG_B = 1
LAG_D = 3
E_BOUNDS = (0, 3, 7, 11, 14, 16)


def _tob(x):
    return pltpu.bitcast(x, bf16)


def _tou(x):
    return pltpu.bitcast(x, u32)


def _rb(x):
    return x.astype(bf16).astype(f32)


def _layernorm(xb):
    x = xb.astype(f32)
    mu = jnp.sum(x, axis=-1, keepdims=True) * (1.0 / D)
    xc = x - mu
    var = jnp.sum(xc * xc, axis=-1, keepdims=True) * (1.0 / D)
    den = _rb(jnp.sqrt(_rb(_rb(var) + EPS)))
    return (_rb(x - _rb(mu)) / den).astype(bf16)


def _silu(z):
    return z * (0.5 + 0.5 * jnp.tanh(0.5 * z))


def _kernel(x_hbm, mem0_ref, wq_hbm, wk_hbm, wv_hbm, wo_hbm, wr_ref, wg_hbm, wu_hbm, wd_hbm,
            out_hbm,
            xv, lhs, xpre, zbuf, raw, wqkv, wo, pre, wg, wu, wd, opost, sres, outv, mask_ref,
            sem_x, sem_w, sem_o, sem_f, sem_out):
    x_cp = pltpu.make_async_copy(x_hbm, xv, sem_x.at[0])
    x_cp.start()
    w32 = [w.bitcast(u32) for w in (wq_hbm, wk_hbm, wv_hbm)]

    def w_cp(p, m):
        return pltpu.make_async_copy(w32[m].at[:, p, :], raw.at[p * 3 + m], sem_w.at[p * 3 + m])

    for p in range(NP):
        for m in range(3):
            w_cp(p, m).start()
    wo32 = wo_hbm.bitcast(u32)
    wo_cps = [pltpu.make_async_copy(wo32.at[:, pl.ds(j * 128, 128)], wo.at[j], sem_o.at[j])
              for j in range(NJ)]
    for c in wo_cps:
        c.start()
    f_cps = [pltpu.make_async_copy(a, b, sem_f.at[i])
             for i, (a, b) in enumerate(((wg_hbm, wg), (wu_hbm, wu), (wd_hbm, wd)))]
    for c in f_cps:
        c.start()

    r = lax.broadcasted_iota(i32, (80, 80), 0)
    c = lax.broadcasted_iota(i32, (80, 80), 1)

    def head_pos(i):
        head = jnp.where(i < 32, 0, jnp.where(i < 64, 1, jnp.where(i < 72, 0, 1)))
        j = i & 31
        pos = jnp.where(i < 64, jnp.where(j < 8, j, j + 8), 8 + (i & 7))
        return head, pos

    hr, pr = head_pos(r)
    hc, pc = head_pos(c)
    ok = (hr == hc) & ((pr < M) | (pr >= pc))
    mask_ref[...] = jnp.where(ok, 1.0, 0.0).astype(f32)

    x_cp.wait()
    wr = jnp.broadcast_to(wr_ref[...].astype(f32).reshape(1, D), (16, D)).astype(bf16)
    row16 = lax.broadcasted_iota(i32, (16, 128), 0)

    def ln_body(i, rd):
        r0 = pl.multiple_of(i * 128, 128)
        xn = _layernorm(xv[pl.ds(r0, 128), :])
        xn32 = xn.astype(f32)
        zbuf[pl.ds(r0, 128), :] = xn32
        lhs[pl.ds(pl.multiple_of(i * 64, 64), 64), :] = _tou(xn)
        xp = jnp.concatenate([xn32[k * SEG:k * SEG + 8] for k in range(4)], axis=0).astype(bf16)
        xpre[pl.ds(pl.multiple_of(i * 16, 16), 16), :] = _tou(xp)
        rr = lax.dot_general(wr, xn, (((1,), (1,)), ((), ())), preferred_element_type=f32)
        return jnp.where(row16 == i, rr, rd)

    rd = lax.fori_loop(0, S // 128, ln_body, jnp.zeros((16, 128), f32))

    m0 = jnp.concatenate([mem0_ref[...].astype(f32), jnp.zeros((8, D), f32)], axis=0)
    lhs[pl.ds(0, 4), :] = _tou(m0.astype(bf16))[0:4]

    def pre_body(p, carry):
        for m in range(3):
            w_cp(p, m).wait()
            w = raw[p * 3 + m]
            lo = pltpu.bitcast(w << 16, f32).astype(bf16)
            hi = pltpu.bitcast(w & jnp.uint32(0xFFFF0000), f32).astype(bf16)
            wqkv[p * 6 + 2 * m] = _tou(lo)
            wqkv[p * 6 + 2 * m + 1] = _tou(hi)
        for m in range(3):
            for b in range(4):
                xb = _tob(xpre[pl.ds(b * 64, 64), :])
                a0 = jnp.dot(xb, _tob(wqkv[p * 6 + 2 * m]), preferred_element_type=f32)
                a1 = jnp.dot(xb, _tob(wqkv[p * 6 + 2 * m + 1]), preferred_element_type=f32)
                parts = []
                for k in range(16):
                    parts += [a0[k * 8:(k + 1) * 8], a1[k * 8:(k + 1) * 8]]
                pk = _tou(jnp.concatenate(parts, axis=0).astype(bf16))
                pre[p * 3 + m, pl.ds(b * 128, 128), :] = pk
        return carry

    lax.fori_loop(0, NP, pre_body, 0)

    rd = _rb(rd)
    rd = jnp.where(rd == 0.0, 0.0, rd)
    bits = pltpu.bitcast(rd, i32)
    mono = jnp.where(bits < 0, bits ^ jnp.int32(0x7FFFFFFF), bits)
    lane16 = lax.broadcasted_iota(i32, (16, 128), 1)
    key = (mono & jnp.int32(-65536)) | (65535 - (row16 * 128 + lane16))
    row8 = lax.broadcasted_iota(i32, (8, 1), 0)
    ksel = jnp.zeros((8, 1), i32)
    idxs = []
    rows = []
    for t in range(C):
        km = jnp.max(jnp.max(key, axis=0, keepdims=True), axis=1, keepdims=True)
        key = jnp.where(key == km, jnp.int32(-2147483648), key)
        ksel = jnp.where(row8 == t, km, ksel)
        idx = 65535 - (km[0, 0] & 65535)
        idx = jnp.clip(idx, 0, S - 1)
        idxs.append(idx)
        rows.append(zbuf[pl.ds(idx, 1), :])
    xs = jnp.concatenate(rows, axis=0)
    hi16 = ksel & jnp.int32(-65536)
    rbits = jnp.where(ksel < 0, hi16 ^ jnp.int32(0x7FFF0000), hi16)
    rsel = pltpu.bitcast(rbits, f32)
    rsel = _rb(0.5 + 0.5 * jnp.tanh(0.5 * rsel))
    for cp in f_cps:
        cp.wait()
    xsb = xs.astype(bf16)
    gate = _rb(lax.dot_general(xsb, wg[...], (((1,), (1,)), ((), ())), preferred_element_type=f32))
    up = _rb(lax.dot_general(xsb, wu[...], (((1,), (1,)), ((), ())), preferred_element_type=f32))
    hid = (_rb(_silu(gate)) * up).astype(bf16)
    y = _rb(jnp.dot(hid, wd[...], preferred_element_type=f32))
    zs = _rb(xs + _rb(y * rsel))
    for t in range(C):
        zbuf[pl.ds(idxs[t], 1), :] = zs[t:t + 1]

    for cp in wo_cps:
        cp.wait()

    def step(sg, sl):
        x = _tob(lhs[pl.ds(pl.multiple_of(sg * 16, 16), 16), :])
        prow = pl.multiple_of(sg * 8, 8)
        orow = pl.multiple_of(sl * 8, 8)
        st = {}
        oc = {}

        def stage_a(p):
            outs = []
            for m in range(3):
                a = jnp.dot(x, _tob(wqkv[p * 6 + 2 * m]), preferred_element_type=f32)
                b = jnp.dot(x, _tob(wqkv[p * 6 + 2 * m + 1]), preferred_element_type=f32)
                ab = jnp.concatenate([a, b], axis=0).astype(bf16)
                outs.append(jnp.concatenate([ab, _tob(pre[p * 3 + m, pl.ds(prow, 8), :])], axis=0))
            st[p] = outs

        def stage_b(p):
            q, k, v = st[p]
            sc = lax.dot_general(q, k, (((1,), (1,)), ((), ())), preferred_element_type=f32)
            sc = jnp.where(mask_ref[...] > 0.5, sc, NEG)
            mx = jnp.max(sc, axis=-1, keepdims=True)
            e = jnp.exp2((sc - mx) * CEXP)
            l = jnp.sum(e, axis=-1, keepdims=True)
            st[p] = ((e * pl.reciprocal(l, approx=True)).astype(bf16), v)

        def stage_d(p):
            e, v = st[p]
            o = jnp.dot(e, v, preferred_element_type=f32)
            opost[pl.ds(orow, 8), (2 * p) * 128:(2 * p + 1) * 128] = o[64:72]
            opost[pl.ds(orow, 8), (2 * p + 1) * 128:(2 * p + 2) * 128] = o[72:80]
            ob = o[0:64].astype(bf16)
            oc[2 * p] = ob[0:32]
            oc[2 * p + 1] = ob[32:64]

        def stage_e(h0, h1):
            o2 = jnp.concatenate([oc[h] for h in range(h0, h1)], axis=1)
            return [jnp.dot(o2, _tob(wo[j, h0 * 64:h1 * 64, :]), preferred_element_type=f32)
                    for j in range(NJ)]

        acc = None
        for slot in range(NP + len(E_BOUNDS) - 1):
            if slot < NP:
                stage_a(slot)
            else:
                i = slot - NP
                t = stage_e(2 * E_BOUNDS[i], 2 * E_BOUNDS[i + 1])
                acc = t if acc is None else [b + a for a, b in zip(acc, t)]
            if 0 <= slot - LAG_B < NP:
                stage_b(slot - LAG_B)
            if 0 <= slot - LAG_D < NP:
                stage_d(slot - LAG_D)
        acc = jnp.concatenate(acc, axis=1)
        lhs[pl.ds(pl.multiple_of((sg + 1) * 16, 16), 4), :] = _tou(acc[0:16].astype(bf16))[0:4]
        sres[pl.ds(pl.multiple_of(sl * SEG + 8, 8), 24), :] = acc[8:32]

    def out_cp(ci):
        r0 = pl.multiple_of(ci * (CH * SEG), CH * SEG)
        return pltpu.make_async_copy(outv.at[pl.ds(r0, CH * SEG), :],
                                     out_hbm.at[pl.ds(r0, CH * SEG), :], sem_out.at[ci])

    def chunk(ci, carry):
        def inner(sl, c2):
            step(ci * CH + sl, sl)
            return c2

        lax.fori_loop(0, CH, inner, 0)
        ob = opost[...].astype(bf16)
        for j in range(NJ):
            t = jnp.dot(ob, _tob(wo[j]), preferred_element_type=f32)
            for k in range(CH):
                sres[k * SEG:k * SEG + 8, j * 128:(j + 1) * 128] = t[k * 8:(k + 1) * 8]
        r0 = pl.multiple_of(ci * (CH * SEG), CH * SEG)
        rows = pl.ds(r0, CH * SEG)
        outv[rows, :] = (xv[rows, :].astype(f32) + sres[...] * _silu(zbuf[rows, :])).astype(bf16)
        out_cp(ci).start()
        return carry

    lax.fori_loop(0, NCH, chunk, 0)
    for ci in range(NCH):
        out_cp(ci).wait()


@jax.jit
def pallas_recurrent_scan__memory_aug_recurrent_mem_tr__moe_arch_mod__prompt_kernel(
    A_x, A_mem0, A_Wq, A_Wk, A_Wv, A_Wo, A_seg_len, B_x, B_w_r, B_w_gate, B_w_up, B_w_down,
):
    any_spec = pl.BlockSpec(memory_space=pltpu.MemorySpace.HBM)
    vmem_spec = pl.BlockSpec(memory_space=pltpu.VMEM)
    out = pl.pallas_call(
        _kernel,
        out_shape=jax.ShapeDtypeStruct((S, D), bf16),
        in_specs=[any_spec, vmem_spec, any_spec, any_spec, any_spec, any_spec, vmem_spec,
                  any_spec, any_spec, any_spec],
        out_specs=any_spec,
        scratch_shapes=[
            pltpu.VMEM((S, D), bf16),
            pltpu.VMEM(((NSEG + 1) * 16, D), u32),
            pltpu.VMEM((NSEG * 4, D), u32),
            pltpu.VMEM((S, D), f32),
            pltpu.VMEM((NP * 3, D, 128), u32),
            pltpu.VMEM((NP * 6, D // 2, 128), u32),
            pltpu.VMEM((NJ, H * DH // 2, 128), u32),
            pltpu.VMEM((NP * 3, NSEG * 8, 128), u32),
            pltpu.VMEM((F, D), bf16),
            pltpu.VMEM((F, D), bf16),
            pltpu.VMEM((F, D), bf16),
            pltpu.VMEM((CH * 8, H * DH), f32),
            pltpu.VMEM((CH * SEG, D), f32),
            pltpu.VMEM((S, D), bf16),
            pltpu.VMEM((80, 80), f32),
            pltpu.SemaphoreType.DMA((1,)),
            pltpu.SemaphoreType.DMA((NP * 3,)),
            pltpu.SemaphoreType.DMA((NJ,)),
            pltpu.SemaphoreType.DMA((3,)),
            pltpu.SemaphoreType.DMA((NCH,)),
        ],
        compiler_params=pltpu.CompilerParams(vmem_limit_bytes=100 * 1024 * 1024),
        name="rmt_mod",
    )(A_x.reshape(S, D), A_mem0.reshape(M, D), A_Wq, A_Wk, A_Wv, A_Wo.reshape(H * DH, D),
      B_w_r, B_w_gate.T, B_w_up.T, B_w_down)
    return out.reshape(1, S, D)
```

```python
import math
import os
import contextlib

import jax
import jax.numpy as jnp
from jax import lax
import jax.experimental.pallas as pl
import jax.experimental.pallas.tpu as pltpu

bf16 = jnp.bfloat16
f32 = jnp.float32
u32 = jnp.uint32
i32 = jnp.int32

S = 2048
D = 640
H = 32
DH = 128
NP = H // 2
NU = NP * 3
M = 8
SEG = 32
NSEG = S // SEG
F = 1728
C = 8
CH = 4
NCH = NSEG // CH
NJ = D // 128
EPS = 1e-5
NEG = -1e30
LOG2E = math.log2(math.e)
CEXP = (DH ** -0.5) * LOG2E

LAG_B = 1
LAG_D = 3
E_BOUNDS = (0, 3, 7, 11, 14, 16)
FILL_BOUNDS = (0, 11, 22, 32)

GROUPS = (
    ("p0",), ("w0", "p1"), ("w1", "p2", "p3"), ("w2", "w3"),
    tuple("w%d" % u for u in range(4, 8)),
    tuple("w%d" % u for u in range(8, 16)),
    ("mem0", "wr", "x") + tuple("w%d" % u for u in range(16, 25)),
    tuple("w%d" % u for u in range(25, 42)),
    tuple("w%d" % u for u in range(42, 48)) + ("f0", "f1", "f2"),
    tuple("o%d" % j for j in range(NJ)),
)
TIE_LAG = int(os.environ.get("TIE_LAG", 6))
LN_NUM, LN_DEN = [int(v) for v in os.environ.get("LNR", "8,7").split(',')]
NT = (((1,), (1,)), ((), ()))
SCOPES = bool(os.environ.get("SCOPES"))


def _tob(x):
    return pltpu.bitcast(x, bf16)


def _tou(x):
    return pltpu.bitcast(x, u32)


def _zero_of(x):
    return (pltpu.bitcast(x, u32) >> 16) >> 16


def _rb(x):
    return x.astype(bf16).astype(f32)


def _layernorm(x, tie=None):
    ps = x[:, 0:128]
    if tie is not None:
        ps = ps + jnp.concatenate([tie] * (x.shape[0] // 8), axis=0)
    for j in range(1, NJ):
        ps = ps + x[:, j * 128:(j + 1) * 128]
    mu = jnp.sum(ps, axis=-1, keepdims=True) * (1.0 / D)
    xc = x - mu
    var = jnp.sum(xc * xc, axis=-1, keepdims=True) * (1.0 / D)
    den = _rb(jnp.sqrt(_rb(_rb(var) + EPS)))
    return (_rb(x - _rb(mu)) * pl.reciprocal(den, approx=False, full_range=False)).astype(bf16)


def _sigmoid(z):
    return pl.reciprocal(1.0 + jnp.exp2(z * (-LOG2E)), approx=True)


def _silu(z):
    return z * _sigmoid(z)


def _kernel(x_hbm, mem0_hbm, wq_hbm, wk_hbm, wv_hbm, wo_hbm, wr_hbm, wg_hbm, wu_hbm, wd_hbm,
            out_hbm,
            xv, lhs, xpre, zbuf, raw, wqkv, wo, pre, wg, wu, wd, opost, obf, pacc, outv, mask_ref,
            xst, memv, mem0_v, wr_v, sem, sem_out):
    es = contextlib.ExitStack()

    def scope(name):
        es.close()
        if SCOPES and name:
            es.enter_context(jax.named_scope(name))

    w32 = [w.bitcast(u32) for w in (wq_hbm, wk_hbm, wv_hbm)]
    wo32 = wo_hbm.bitcast(u32)

    def src_dst(name):
        if name == "mem0":
            return mem0_hbm, mem0_v
        if name == "wr":
            return wr_hbm, wr_v
        if name == "x":
            return x_hbm.at[:, pl.ds(8, 24), :], xv.at[:, pl.ds(8, 24), :]
        k, n = name[0], int(name[1:])
        if k == "p":
            return x_hbm.at[pl.ds(n * 16, 16), pl.ds(0, 8), :], xv.at[pl.ds(n * 16, 16), pl.ds(0, 8), :]
        if k == "w":
            return w32[n % 3].at[:, n // 3, :], raw.at[n]
        if k == "f":
            return ((wg_hbm, wg), (wu_hbm, wu), (wd_hbm, wd))[n]
        return wo32.at[:, pl.ds(n * 128, 128)], wo.at[n]

    cps = [[pltpu.make_async_copy(*src_dst(nm), sem.at[gi]) for nm in grp] for gi, grp in enumerate(GROUPS)]
    for grp in cps:
        for cp in grp:
            cp.start()

    r = lax.broadcasted_iota(i32, (80, 80), 0)
    c = lax.broadcasted_iota(i32, (80, 80), 1)

    def head_pos(i):
        head = jnp.where(i < 32, 0, jnp.where(i < 64, 1, jnp.where(i < 72, 0, 1)))
        j = i & 31
        pos = jnp.where(i < 64, jnp.where(j < 8, j, j + 8), 8 + (i & 7))
        return head, pos

    hr, pr = head_pos(r)
    hc, pc = head_pos(c)
    ok = (hr == hc) & ((pr < M) | (pr >= pc))
    mask_ref[...] = jnp.where(ok, 1.0, 0.0).astype(f32)
    opost[...] = jnp.zeros(opost.shape, f32)

    def ln_pre(b):
        xb = xv[pl.ds(b * 16, 16), pl.ds(0, 8), :].astype(f32).reshape(128, D)
        xpre[pl.ds(b * 64, 64), :] = _tou(_layernorm(xb))

    def repack(u):
        for k in range(NJ):
            ev = raw[u, pl.ds(k * 128, 64, stride=2), :]
            od = raw[u, pl.ds(k * 128 + 1, 64, stride=2), :]
            wqkv[2 * u, k * 64:(k + 1) * 64, :] = (ev & jnp.uint32(0xFFFF)) | (od << 16)
            wqkv[2 * u + 1, k * 64:(k + 1) * 64, :] = (ev >> 16) | (od & jnp.uint32(0xFFFF0000))

    def pre_dots(u, b, hook):
        xu = xpre[pl.ds(b * 64, 64), :]
        res = []
        for hh in range(2):
            tie = hook()
            xt = xu
            if tie is not None:
                top = jnp.concatenate([xu[0:8, 0:128] ^ tie, xu[0:8, 128:]], axis=1)
                xt = jnp.concatenate([top, xu[8:]], axis=0)
            res.append(jnp.dot(_tob(xt), _tob(wqkv[2 * u + hh]), preferred_element_type=f32))
            st["after"] = res[-1][0:8]
        parts = []
        for k in range(16):
            parts += [res[0][k * 8:(k + 1) * 8], res[1][k * 8:(k + 1) * 8]]
        pre[u, pl.ds(b * 128, 128), :] = _tou(jnp.concatenate(parts, axis=0).astype(bf16))

    lane8 = lax.broadcasted_iota(i32, (8, 128), 1)
    sub8 = lax.broadcasted_iota(i32, (8, 128), 0)
    st = {"rd": [jnp.zeros((8, 128), f32), jnp.zeros((8, 128), f32)]}

    def score(g, xn32):
        zbuf[pl.ds(g * 8, 8), :] = xn32
        rc = jnp.sum(xn32 * st["wr"], axis=-1, keepdims=True)
        st["rd"][g // 128] = jnp.where(lane8 == g % 128, rc, st["rd"][g // 128])

    def ln_group(s, k):
        tie = None
        if st["after"] is not None:
            tie = pltpu.bitcast(_zero_of(st["after"]), f32)
        xn = _layernorm(xv[s, k * 8:(k + 1) * 8, :].astype(f32), tie)
        score(s * 4 + k, xn.astype(f32))
        if k == 1 and s % 2 == 0:
            xp = _tob(xpre[pl.ds(s * 4, 8), :]).astype(f32)
            score(s * 4, xp[0:8])
            score(s * 4 + 4, xp[8:16])
        if k == 2:
            st["xn2"] = xn
        else:
            xu = _tou(jnp.concatenate([xn if k == 1 else st["xn2"], xn], axis=0))
            lhs[pl.ds(s * 16 + (k // 2) * 8, 8), :] = xu
            if s < CH:
                xst[s, (k // 2) * 8:(k // 2) * 8 + 8, :] = xu
        return _zero_of(st["rd"][(s * 4) // 128])

    def topk():
        rd = _rb(jnp.concatenate(st["rd"], axis=0))
        rd = jnp.where(rd == 0.0, 0.0, rd)
        bits = pltpu.bitcast(rd, i32)
        mono = jnp.where(bits < 0, bits ^ jnp.int32(0x7FFFFFFF), bits)
        rowid = jnp.concatenate([lane8 * 8 + sub8, lane8 * 8 + sub8 + 1024], axis=0)
        key = (mono & jnp.int32(-65536)) | (65535 - rowid)
        row8 = lax.broadcasted_iota(i32, (8, 1), 0)
        ksel = jnp.zeros((8, 1), i32)
        idxs = []
        rows = []
        for t in range(C):
            km = jnp.max(jnp.max(key, axis=0, keepdims=True), axis=1, keepdims=True)
            key = jnp.where(key == km, jnp.int32(-2147483648), key)
            ksel = jnp.where(row8 == t, km, ksel)
            idx = jnp.clip(65535 - (km[0, 0] & 65535), 0, S - 1)
            idxs.append(idx)
            rows.append(zbuf[pl.ds(idx, 1), :])
        xs = jnp.concatenate(rows, axis=0)
        hi16 = ksel & jnp.int32(-65536)
        rbits = jnp.where(ksel < 0, hi16 ^ jnp.int32(0x7FFF0000), hi16)
        st["rsel"] = _rb(_sigmoid(pltpu.bitcast(rbits, f32)))
        st["idxs"] = idxs
        st["xs"] = xs
        st["xsb"] = xs.astype(bf16)

    fcols = [(k * 128, min(F, (k + 1) * 128)) for k in range((F + 127) // 128)]

    def ffn_tasks():
        hid = []
        tmp = {}

        def gate(k):
            a, b = fcols[k]
            tmp["g"] = _rb(lax.dot_general(st["xsb"], wg[a:b, :], NT, preferred_element_type=f32))

        def up(k):
            a, b = fcols[k]
            u_ = _rb(lax.dot_general(st["xsb"], wu[a:b, :], NT, preferred_element_type=f32))
            hid.append((_rb(_silu(tmp["g"])) * u_).astype(bf16))

        def down(k):
            a, b = fcols[k]
            t = jnp.dot(hid[k], wd[a:b, :], preferred_element_type=f32)
            tmp["y"] = t if k == 0 else t + tmp["y"]

        def fin():
            zs = _rb(st["xs"] + _rb(_rb(tmp["y"]) * st["rsel"]))
            for t in range(C):
                zbuf[pl.ds(st["idxs"][t], 1), :] = zs[t:t + 1]

        n = len(fcols)
        tasks = []
        for k in range(n):
            tasks += [lambda k=k: gate(k), lambda k=k: up(k)]
        tasks += [lambda k=k: down(k) for k in range(n)]
        tasks.append(fin)
        return tasks

    pending = []
    units, blocks = [], []
    side = []
    st["credit"] = 0
    tasks = None
    for gi, grp in enumerate(GROUPS):
        scope("wait%d" % gi)
        for cp in cps[gi]:
            cp.wait()
        scope("region%d" % gi)
        if grp[0] == "o0":
            break
        final = "f0" in grp
        new_u = [int(nm[1:]) for nm in grp if nm[0] == "w" and nm != "wr"]
        new_b = [int(nm[1:]) for nm in grp if nm[0] == "p"]
        for u in new_u:
            repack(u)
            pending += [(u, b) for b in blocks]
            units.append(u)
        for b in new_b:
            ln_pre(b)
            pending += [(u, b) for u in units]
            blocks.append(b)
        if "x" in grp:
            side = [(s_, k) for s_ in range(NSEG) for k in (1, 2, 3)]
            st["wr"] = jnp.broadcast_to(wr_v[...].astype(f32).reshape(1, D), (8, D))
            m0 = jnp.concatenate([mem0_v[...].astype(f32), jnp.zeros((8, D), f32)], axis=0)
            memv[...] = _tou(m0.astype(bf16))
        hold = 0 if (final or gi < 2) else (1 if gi == 2 else 2)
        work, pending = pending[:len(pending) - hold], pending[len(pending) - hold:]
        ties = []
        if final:
            tasks = ffn_tasks()
        st["after"] = None
        cnt = [0]

        def hook():
            di = cnt[0]
            cnt[0] += 1
            if tasks:
                tasks.pop(0)()
            tie = None
            if ties and ties[0][0] <= di:
                tie = ties.pop(0)[1]
            if side and di + TIE_LAG < 2 * len(work):
                st["credit"] += LN_NUM
                last = None
                while side and st["credit"] >= LN_DEN:
                    st["credit"] -= LN_DEN
                    last = ln_group(*side.pop(0))
                    if not side:
                        topk()
                if last is not None:
                    ties.append((di + TIE_LAG, last))
            return tie

        for u, b in work:
            pre_dots(u, b, hook)
        assert not ties
    assert not side and not tasks and not pending
    scope(None)

    sub4 = lax.broadcasted_iota(i32, (8, D), 0) < 4

    def finalize(sg, r0, r1, sv):
        rows = pl.ds(pl.multiple_of(sg * SEG + r0, 8), r1 - r0)
        xr = xv[sg, r0:r1, :].astype(f32)
        outv[rows, :] = (xr + sv * _silu(zbuf[rows, :])).astype(bf16)

    def step(sg, sl, mem):
        xu = xst[sl]
        x = _tob(jnp.concatenate([jnp.where(sub4, mem, xu[0:8]), xu[8:16]], axis=0))
        prow = pl.multiple_of(sg * 8, 8)
        sd = {}
        oc = {}

        def stage_a(p):
            outs = []
            for m in range(3):
                u = p * 3 + m
                a = jnp.dot(x, _tob(wqkv[2 * u]), preferred_element_type=f32)
                b = jnp.dot(x, _tob(wqkv[2 * u + 1]), preferred_element_type=f32)
                ab = jnp.concatenate([a, b], axis=0).astype(bf16)
                outs.append(jnp.concatenate([ab, _tob(pre[u, pl.ds(prow, 8), :])], axis=0))
            sd[p] = outs

        def stage_b(p):
            q, k, v = sd[p]
            sc = lax.dot_general(q, k, NT, preferred_element_type=f32)
            sc = jnp.where(mask_ref[...] > 0.5, sc, NEG)
            mx = jnp.max(sc, axis=-1, keepdims=True)
            e = jnp.exp2((sc - mx) * CEXP)
            l = jnp.sum(e, axis=-1, keepdims=True)
            sd[p] = ((e * pl.reciprocal(l, approx=True)).astype(bf16), v)

        def stage_d(p):
            e, v = sd[p]
            o = jnp.dot(e, v, preferred_element_type=f32)
            opost[sl * 8:sl * 8 + 8, (2 * p) * 128:(2 * p + 1) * 128] = o[64:72]
            opost[sl * 8:sl * 8 + 8, (2 * p + 1) * 128:(2 * p + 2) * 128] = o[72:80]
            ob = o[0:64].astype(bf16)
            oc[2 * p] = ob[0:32]
            oc[2 * p + 1] = ob[32:64]

        def stage_e(h0, h1):
            o2 = jnp.concatenate([oc[h] for h in range(h0, h1)], axis=1)
            return [jnp.dot(o2, _tob(wo[j, h0 * 64:h1 * 64, :]), preferred_element_type=f32)
                    for j in range(NJ)]

        acc = None
        for slot in range(NP + len(E_BOUNDS) - 1):
            if slot < NP:
                stage_a(slot)
            else:
                i = slot - NP
                t = stage_e(2 * E_BOUNDS[i], 2 * E_BOUNDS[i + 1])
                acc = t if acc is None else [b + a for a, b in zip(acc, t)]
            if slot == NP:
                nx = jnp.minimum(sg + CH, NSEG - 1)
                xst[sl] = lhs[pl.ds(pl.multiple_of(nx * 16, 16), 16), :]
            if 0 <= slot - LAG_B < NP:
                stage_b(slot - LAG_B)
            if 0 <= slot - LAG_D < NP:
                stage_d(slot - LAG_D)
        acc = jnp.concatenate(acc, axis=1)
        finalize(sg, 8, SEG, acc[8:32])
        return _tou(acc[0:16].astype(bf16))

    def pack_post():
        obf[...] = _tou(opost[...].astype(bf16))

    def post_proj(ci, h0, h1):
        ob = _tob(obf[:, h0 * 128:h1 * 128])
        ts = []
        for j in range(NJ):
            t = jnp.dot(ob, _tob(wo[j, h0 * 64:h1 * 64, :]), preferred_element_type=f32)
            if h0 > 0:
                t = t + pacc[:, j * 128:(j + 1) * 128]
            ts.append(t)
        t = jnp.concatenate(ts, axis=1)
        if h1 < H:
            pacc[...] = t
        else:
            for k in range(CH):
                finalize(ci * CH + k, 0, 8, t[k * 8:(k + 1) * 8])

    def out_cp(ci):
        r0 = pl.multiple_of(ci * (CH * SEG), CH * SEG)
        return pltpu.make_async_copy(outv.at[pl.ds(r0, CH * SEG), :],
                                     out_hbm.at[pl.ds(r0, CH * SEG), :], sem_out.at[0])

    def chunk(ci, carry):
        prev = jnp.maximum(ci - 1, 0)
        pack_post()
        mem = memv[...]
        for sl in range(CH):
            if sl > 0:
                post_proj(prev, FILL_BOUNDS[sl - 1], FILL_BOUNDS[sl])
            mem = step(ci * CH + sl, sl, mem)
        memv[...] = mem

        @pl.when(ci > 0)
        def _():
            out_cp(prev).start()

        return carry

    scope("mainloop")
    if not os.environ.get('NOMAIN'):
        lax.fori_loop(0, NCH, chunk, 0)
    else:
        def dummy(i, c):
            opost[...] = opost[...] + pltpu.bitcast(pre[i, 0:32, :], f32)[:, 0:1] + pltpu.bitcast(lhs[pl.ds(pl.multiple_of(i*16, 16), 32), :], f32)[:, 0:1] + pltpu.bitcast(wqkv[i, 0:32, :], f32)[:, 0:1] + pltpu.bitcast(xst[i % 4, 0:8, :], f32)[0:1, 0:1] + pltpu.bitcast(memv[...], f32)[0:1, 0:1] + mask_ref[0:1, 0:1]
            finalize(i, 0, 32, opost[:, 0:640])
            return c
        lax.fori_loop(0, 48, dummy, 0)
    scope("epi")
    pack_post()
    post_proj(NCH - 1, 0, H)
    out_cp(NCH - 1).start()
    scope("waitout")
    for ci in range(NCH):
        out_cp(ci).wait()
    scope(None)


@jax.jit
def pallas_recurrent_scan__memory_aug_recurrent_mem_tr__moe_arch_mod__prompt_kernel(
    A_x, A_mem0, A_Wq, A_Wk, A_Wv, A_Wo, A_seg_len, B_x, B_w_r, B_w_gate, B_w_up, B_w_down,
):
    hbm = pl.BlockSpec(memory_space=pltpu.MemorySpace.HBM)
    out = pl.pallas_call(
        _kernel,
        out_shape=jax.ShapeDtypeStruct((S, D), bf16),
        in_specs=[hbm] * 10,
        out_specs=hbm,
        scratch_shapes=[
            pltpu.VMEM((NSEG, SEG, D), bf16),
            pltpu.VMEM((NSEG * 16, D), u32),
            pltpu.VMEM((NSEG * 4, D), u32),
            pltpu.VMEM((S, D), f32),
            pltpu.VMEM((NU, D, 128), u32),
            pltpu.VMEM((NU * 2, D // 2, 128), u32),
            pltpu.VMEM((NJ, H * DH // 2, 128), u32),
            pltpu.VMEM((NU, NSEG * 8, 128), u32),
            pltpu.VMEM((F, D), bf16),
            pltpu.VMEM((F, D), bf16),
            pltpu.VMEM((F, D), bf16),
            pltpu.VMEM((CH * 8, H * DH), f32),
            pltpu.VMEM((CH * 4, H * DH), u32),
            pltpu.VMEM((CH * 8, D), f32),
            pltpu.VMEM((S, D), bf16),
            pltpu.VMEM((80, 80), f32),
            pltpu.VMEM((CH, 16, D), u32),
            pltpu.VMEM((8, D), u32),
            pltpu.VMEM((M, D), bf16),
            pltpu.VMEM((D,), bf16),
            pltpu.SemaphoreType.DMA((len(GROUPS),)),
            pltpu.SemaphoreType.DMA((1,)),
        ],
        compiler_params=pltpu.CompilerParams(vmem_limit_bytes=100 * 1024 * 1024),
        name="rmt_mod",
    )(A_x.reshape(NSEG, SEG, D), A_mem0.reshape(M, D), A_Wq, A_Wk, A_Wv, A_Wo.reshape(H * DH, D),
      B_w_r, B_w_gate.T, B_w_up.T, B_w_down)
    return out.reshape(1, S, D)
```

```python
import math
import os
import contextlib

import jax
import jax.numpy as jnp
from jax import lax
import jax.experimental.pallas as pl
import jax.experimental.pallas.tpu as pltpu

bf16 = jnp.bfloat16
f32 = jnp.float32
u32 = jnp.uint32
i32 = jnp.int32

S = 2048
D = 640
H = 32
DH = 128
NP = H // 2
NU = NP * 3
M = 8
SEG = 32
NSEG = S // SEG
F = 1728
C = 8
CH = int(os.environ.get('CH', 4))
NCH = NSEG // CH
NJ = D // 128
EPS = 1e-5
NEG = -1e30
LOG2E = math.log2(math.e)
CEXP = (DH ** -0.5) * LOG2E

LAG_B = int(os.environ.get('LAG_B', 1))
LAG_D = int(os.environ.get('LAG_D', 3))
E_BOUNDS = tuple(int(v) for v in os.environ.get('EB', '0,3,7,10,13,16').split(','))
VAR = os.environ.get('VAR', 'f32cat,of32')
DELAY = int(os.environ.get('DELAY', 0))
POS_B = int(os.environ.get('POS_B', 3))
POS_D = int(os.environ.get('POS_D', 6))
MORDS = [[int(c) for c in os.environ.get('M%d' % i, '012')] for i in range(4)]
STAG = os.environ.get('STAG', '00000')
P_BOUNDS = tuple(int(v) for v in os.environ.get('PB', '0,8,16,24,32').split(','))
KMAJ = [int(c) for c in os.environ.get('KMAJ', '0545')]
EBS = [tuple(int(v) for v in e.split(',')) for e in os.environ.get('EBS', '0,3,6,9,12,16;0,3,6,9,13,16;0,3,6,9,12,16;0,3,7,10,13,16').split(';')]

NPL = 4
UPL = 8
U0 = 9
CPL = NCH // NPL
SPL = NSEG // NPL
HEAD_GROUPS = tuple(tuple(g.split(",")) for g in os.environ.get(
    "HG", "p0;w0,p1;w1,p2,p3;w2,w3;mem0,wr,w4,w5,w6,w7,w8").split(";"))
HOLD = [int(c) for c in os.environ.get("HOLD", "00112")]
LOOP_GROUPS = tuple(
    tuple("w%d" % u for u in range(U0 + i * UPL, U0 + (i + 1) * UPL)) + ("x%d" % i,) for i in range(NPL))
TAIL_GROUPS = (
    tuple("w%d" % u for u in range(U0 + NPL * UPL, NU)) + ("f0", "f1", "f2"),
    tuple("o%d" % j for j in range(NJ)),
)
GROUPS = HEAD_GROUPS + LOOP_GROUPS + TAIL_GROUPS
FFN_SKIP = int(os.environ.get("FFN_SKIP", 16))
TIE_LAG = int(os.environ.get("TIE_LAG", 6))
LN_NUM, LN_DEN = [int(v) for v in os.environ.get("LNR", "6,7").split(',')]
NT = (((1,), (1,)), ((), ()))
SCOPES = bool(os.environ.get("SCOPES"))


def _tob(x):
    return pltpu.bitcast(x, bf16)


def _tou(x):
    return pltpu.bitcast(x, u32)


def _zero_of(x):
    return (pltpu.bitcast(x, u32) >> 16) >> 16


def _rb(x):
    return x.astype(bf16).astype(f32)


def _layernorm(x, tie=None):
    ps = x[:, 0:128]
    if tie is not None:
        ps = ps + jnp.concatenate([tie] * (x.shape[0] // 8), axis=0)
    for j in range(1, NJ):
        ps = ps + x[:, j * 128:(j + 1) * 128]
    mu = jnp.sum(ps, axis=-1, keepdims=True) * (1.0 / D)
    xc = x - mu
    var = jnp.sum(xc * xc, axis=-1, keepdims=True) * (1.0 / D)
    den = _rb(jnp.sqrt(_rb(_rb(var) + EPS)))
    return (_rb(x - _rb(mu)) * pl.reciprocal(den, approx=False, full_range=False)).astype(bf16)


def _sigmoid(z):
    return pl.reciprocal(1.0 + jnp.exp2(z * (-LOG2E)), approx=True)


def _silu(z):
    return z * _sigmoid(z)


def _kernel(x_hbm, mem0_hbm, wq_hbm, wk_hbm, wv_hbm, wo_hbm, wr_hbm, wg_hbm, wu_hbm, wd_hbm,
            out_hbm,
            xv, lhs, xpre, zbuf, raw, wqkv, wo, pre, wg, wu, wd, outv, mask_ref,
            memv, rds, wr8, mem0_v, wr_v, sem, sem_out):
    es = contextlib.ExitStack()

    def scope(name):
        es.close()
        if SCOPES and name:
            es.enter_context(jax.named_scope(name))

    w32 = [w.bitcast(u32) for w in (wq_hbm, wk_hbm, wv_hbm)]
    wo32 = wo_hbm.bitcast(u32)

    def src_dst(name):
        if name == "mem0":
            return mem0_hbm, mem0_v
        if name == "wr":
            return wr_hbm, wr_v
        k, n = name[0], int(name[1:])
        if k == "x":
            return (x_hbm.at[pl.ds(n * CPL, CPL), :, pl.ds(8, 24), :], xv.at[pl.ds(n * CPL, CPL), :, pl.ds(8, 24), :])
        if k == "p":
            return x_hbm.at[pl.ds(n * 4, 4), :, pl.ds(0, 8), :], xv.at[pl.ds(n * 4, 4), :, pl.ds(0, 8), :]
        if k == "w":
            return w32[n % 3].at[:, n // 3, :], raw.at[n]
        if k == "f":
            return ((wg_hbm, wg), (wu_hbm, wu), (wd_hbm, wd))[n]
        return wo32.at[:, pl.ds(n * 128, 128)], wo.at[n]

    cps = [[pltpu.make_async_copy(*src_dst(nm), sem.at[gi]) for nm in grp] for gi, grp in enumerate(GROUPS)]
    for grp in cps:
        for cp in grp:
            cp.start()

    r = lax.broadcasted_iota(i32, (80, 80), 0)
    c = lax.broadcasted_iota(i32, (80, 80), 1)

    def head_pos(i):
        head = jnp.where(i < 32, 0, jnp.where(i < 64, 1, jnp.where(i < 72, 0, 1)))
        j = i & 31
        pos = jnp.where(i < 64, jnp.where(j < 8, j, j + 8), 8 + (i & 7))
        return head, pos

    hr, pr = head_pos(r)
    hc, pc = head_pos(c)
    ok = (hr == hc) & ((pr < M) | (pr >= pc))
    mask_ref[...] = (jnp.where(ok, 0.0, NEG) if 'bias' in VAR else jnp.where(ok, 1.0, 0.0)).astype(f32)

    def ln_pre(b):
        xb = xv[b * 4:(b + 1) * 4, :, 0:8, :].astype(f32).reshape(128, D)
        xpre[b] = _tou(_layernorm(xb))

    def repack(u):
        ev = raw[u, pl.ds(0, D // 2, stride=2), :]
        od = raw[u, pl.ds(1, D // 2, stride=2), :]
        ws = ((ev & jnp.uint32(0xFFFF)) | (od << 16), (ev >> 16) | (od & jnp.uint32(0xFFFF0000)))
        if 'fpack' in VAR:
            w = raw[u]
            ws = (_tou(pltpu.bitcast(w << 16, f32).astype(bf16)),
                  _tou(pltpu.bitcast(w & jnp.uint32(0xFFFF0000), f32).astype(bf16)))
        wqkv[2 * u] = ws[0]
        wqkv[2 * u + 1] = ws[1]
        return ws

    def pre_dots(u, b, hook, ws=None):
        xu = xpre[b]
        res = []
        for hh in range(2):
            tie = hook()
            xt = xu
            if tie is not None:
                top = jnp.concatenate([xu[0:8, 0:128] ^ tie, xu[0:8, 128:]], axis=1)
                xt = jnp.concatenate([top, xu[8:]], axis=0)
            w = wqkv[2 * u + hh] if ws is None else ws[hh]
            res.append(jnp.dot(_tob(xt), _tob(w), preferred_element_type=f32))
            st["after"] = res[-1][0:8]
        parts = []
        for k in range(16):
            parts += [res[0][k * 8:(k + 1) * 8], res[1][k * 8:(k + 1) * 8]]
        pre[u, b * 4:(b + 1) * 4] = _tou(jnp.concatenate(parts, axis=0).astype(bf16)).reshape(4, CH * 8, 128)

    lane8 = lax.broadcasted_iota(i32, (8, 128), 1)
    sub8 = lax.broadcasted_iota(i32, (8, 128), 0)
    st = {}

    def al(x, m):
        return x if isinstance(x, int) else pl.multiple_of(x, m)

    def score(i, gl, xn32):
        zbuf[i * CPL + gl // 16, (gl % 16) * 8:(gl % 16) * 8 + 8, :] = xn32
        rc = jnp.sum(xn32 * st["wr"], axis=-1, keepdims=True)
        st["rd"] = jnp.where(lane8 == gl, rc, st["rd"])

    def ln_group(i, s, k):
        tie = None
        if st["after"] is not None:
            tie = pltpu.bitcast(_zero_of(st["after"]), f32)
        xn = _layernorm(xv[i * CPL + s // CH, s % CH, k * 8:(k + 1) * 8, :].astype(f32), tie)
        score(i, s * 4 + k, xn.astype(f32))
        if k == 1 and s % 2 == 0:
            xp = _tob(xpre[i, s * 4:s * 4 + 8, :]).astype(f32)
            score(i, s * 4, xp[0:8])
            score(i, s * 4 + 4, xp[8:16])
        if k == 2:
            st["xn2"] = xn
        else:
            xu = _tou(jnp.concatenate([xn if k == 1 else st["xn2"], xn], axis=0))
            r0 = (s % CH) * 16 + (k // 2) * 8
            lhs[i * CPL + s // CH, r0:r0 + 8, :] = xu
        return _zero_of(st["rd"])

    def topk():
        rd = _rb(rds[0:NPL].reshape(NPL * 8, 128))
        rd = jnp.where(rd == 0.0, 0.0, rd)
        bits = pltpu.bitcast(rd, i32)
        mono = jnp.where(bits < 0, bits ^ jnp.int32(0x7FFFFFFF), bits)
        rowid = jnp.concatenate([lane8 * 8 + sub8 + i * SPL * SEG for i in range(NPL)], axis=0)
        key = (mono & jnp.int32(-65536)) | (65535 - rowid)
        key = jnp.where(jnp.concatenate([lane8] * NPL, axis=0) < SPL * 4, key, jnp.int32(-2147483648))
        row8 = lax.broadcasted_iota(i32, (8, 1), 0)
        ksel = jnp.zeros((8, 1), i32)
        idxs = []
        rows = []
        for t in range(C):
            km = jnp.max(jnp.max(key, axis=0, keepdims=True), axis=1, keepdims=True)
            key = jnp.where(key == km, jnp.int32(-2147483648), key)
            ksel = jnp.where(row8 == t, km, ksel)
            idx = jnp.clip(65535 - (km[0, 0] & 65535), 0, S - 1)
            idxs.append(idx)
            rows.append(zbuf[idx >> 7, pl.ds(idx & 127, 1), :])
        xs = jnp.concatenate(rows, axis=0)
        hi16 = ksel & jnp.int32(-65536)
        rbits = jnp.where(ksel < 0, hi16 ^ jnp.int32(0x7FFF0000), hi16)
        st["rsel"] = _rb(_sigmoid(pltpu.bitcast(rbits, f32)))
        st["idxs"] = idxs
        st["xs"] = xs
        st["xsb"] = xs.astype(bf16)

    fcols = [(k * 128, min(F, (k + 1) * 128)) for k in range((F + 127) // 128)]

    def ffn_tasks():
        hid = []
        tmp = {}

        def gate(k):
            a, b = fcols[k]
            tmp["g"] = _rb(lax.dot_general(st["xsb"], wg[a:b, :], NT, preferred_element_type=f32))

        def up(k):
            a, b = fcols[k]
            u_ = _rb(lax.dot_general(st["xsb"], wu[a:b, :], NT, preferred_element_type=f32))
            hid.append((_rb(_silu(tmp["g"])) * u_).astype(bf16))

        def down(k):
            a, b = fcols[k]
            t = jnp.dot(hid[k], wd[a:b, :], preferred_element_type=f32)
            tmp["y"] = t if k == 0 else t + tmp["y"]

        def fin():
            zs = _rb(st["xs"] + _rb(_rb(tmp["y"]) * st["rsel"]))
            for t in range(C):
                zbuf[st["idxs"][t] >> 7, pl.ds(st["idxs"][t] & 127, 1), :] = zs[t:t + 1]

        n = len(fcols)
        tasks = []
        for k in range(n):
            tasks += [lambda k=k: gate(k), lambda k=k: up(k)]
        tasks += [lambda k=k: down(k) for k in range(n)]
        tasks.append(fin)
        return tasks

    def run_region(work, side=(), tasks=(), skip=0):
        side, tasks = list(side), list(tasks)
        ties = []
        st["after"] = None
        st["credit"] = 0
        cnt = [0]

        def hook():
            di = cnt[0]
            cnt[0] += 1
            if tasks and di >= skip:
                tasks.pop(0)()
            tie = None
            if ties and ties[0][0] <= di:
                tie = ties.pop(0)[1]
            if side and di + TIE_LAG < 2 * len(work):
                st["credit"] += LN_NUM
                if st["credit"] >= LN_DEN:
                    st["credit"] -= LN_DEN
                    ties.append((di + TIE_LAG, ln_group(*side.pop(0))))
            return tie

        for u, b, *ws in work:
            pre_dots(u, b, hook, *ws)
        assert not ties and not side and not tasks

    NOPRO = bool(os.environ.get('NOPRO'))
    if NOPRO:
        pre_dots = lambda *a: None
        repack = lambda *a: None
        ln_pre = lambda *a: None
        run_region = lambda *a, **k: None
        topk = lambda: None
    pending = []
    units, blocks = [], []
    for gi, grp in enumerate(HEAD_GROUPS):
        scope("wait%d" % gi)
        for cp in cps[gi]:
            cp.wait()
        scope("region%d" % gi)
        for u in [int(nm[1:]) for nm in grp if nm[0] == "w" and nm != "wr"]:
            repack(u)
            pending += [(u, b) for b in blocks]
            units.append(u)
        for b in [int(nm[1:]) for nm in grp if nm[0] == "p"]:
            ln_pre(b)
            pending += [(u, b) for u in units]
            blocks.append(b)
        if "mem0" in grp:
            m0 = jnp.concatenate([mem0_v[...].astype(f32), jnp.zeros((8, D), f32)], axis=0)
            memv[...] = _tou(m0.astype(bf16))
            wr8[...] = jnp.broadcast_to(wr_v[...].astype(f32).reshape(1, D), (8, D))
        hold = HOLD[gi]
        work, pending = pending[:len(pending) - hold], pending[len(pending) - hold:]
        run_region(work)
    assert pending == [(U0 - 1, 2), (U0 - 1, 3)]

    def pro_body(i, carry):
        g0 = len(HEAD_GROUPS)
        e2 = contextlib.ExitStack()
        if SCOPES: e2.enter_context(jax.named_scope('pw'))
        for nm in LOOP_GROUPS[0]:
            src, dst = src_dst(nm)
            if nm[0] == "w":
                dst = raw.at[int(nm[1:]) + i * UPL]
            else:
                dst = xv.at[pl.ds(i * CPL, CPL), :, pl.ds(8, 24), :]
            pltpu.make_async_copy(src, dst, sem.at[g0 + i]).wait()
        e2.close()
        if SCOPES: e2.enter_context(jax.named_scope('pb'))
        ub = U0 + i * UPL
        wv_ = [None] + [repack(ub + k) for k in range(UPL)]
        if 'dynw' in VAR:
            wv_ = [None] * (UPL + 1)
        work = [(ub - 1 + k // 4, k % 4, wv_[k // 4]) for k in range(2, 2 + 4 * UPL)]
        st["wr"] = wr8[...]
        st["rd"] = jnp.zeros((8, 128), f32)
        run_region(work, side=[(i, s_, k) for s_ in range(SPL) for k in (1, 2, 3)])
        rds[i] = st["rd"]
        e2.close()
        return carry

    scope("proloop")
    lax.fori_loop(0, NPL, pro_body, 0)

    gi = len(HEAD_GROUPS) + NPL
    scope("waitf")
    for cp in cps[gi]:
        cp.wait()
    scope("regionf")
    ub = U0 + NPL * UPL
    for u in range(ub, NU):
        repack(u)
    topk()
    run_region([(ub - 1 + k // 4, k % 4) for k in range(2, 4 + 4 * (NU - ub))], tasks=ffn_tasks(), skip=FFN_SKIP)
    scope("waito")
    for cp in cps[gi + 1]:
        cp.wait()
    scope(None)

    sub4 = lax.broadcasted_iota(i32, (8, D), 0) < 4

    def finalize(ci, sl, r0, r1, sv):
        a, b = sl * SEG + r0, sl * SEG + r1
        xr = xv[ci, sl, r0:r1, :].astype(f32)
        outv[ci, sl, r0:r1, :] = (xr + sv * _silu(zbuf[ci, a:b, :])).astype(bf16)

    ost = {}

    def step(ci, sl, mem):
        MORD = MORDS[sl]
        xu = lhs[ci, sl * 16:(sl + 1) * 16, :]
        x = _tob(jnp.concatenate([jnp.where(sub4, mem, xu[0:8]), xu[8:16]], axis=0))
        sd = {}
        oc = {}

        early = {}
        first = [(d // 6, MORD[(d % 6) // 2], d % 2) for d in range(KMAJ[sl])]
        for k in range(NJ):
            for key in first:
                w = _tob(wqkv[2 * (key[0] * 3 + key[1]) + key[2], k * 64:(k + 1) * 64, :])
                t = jnp.dot(x[:, k * 128:(k + 1) * 128], w, preferred_element_type=f32)
                early[key] = t if k == 0 else t + early[key]

        def a_dot(p, m, hh):
            u = p * 3 + m
            outs = sd.setdefault(p, [None, None, None])
            if (p, m, hh) in early:
                r_ = early[p, m, hh]
            else:
                r_ = jnp.dot(x, _tob(wqkv[2 * u + hh]), preferred_element_type=f32)
            if hh == 0:
                outs[m] = r_
            else:
                pb = _tob(pre[u, ci, sl * 8:(sl + 1) * 8, :])
                if "f32cat" in VAR:
                    outs[m] = jnp.concatenate([outs[m], r_, pb.astype(f32)], axis=0).astype(bf16)
                else:
                    ab = jnp.concatenate([outs[m], r_], axis=0).astype(bf16)
                    outs[m] = jnp.concatenate([ab, pb], axis=0)

        def stage_b(p):
            q, k, v = sd[p]
            sc = lax.dot_general(q, k, NT, preferred_element_type=f32)
            if "bias" in VAR:
                sc = sc + mask_ref[...]
            else:
                sc = jnp.where(mask_ref[...] > 0.5, sc, NEG)
            mx = jnp.max(sc, axis=-1, keepdims=True)
            e = jnp.exp2((sc - mx) * CEXP)
            l = jnp.sum(e, axis=-1, keepdims=True)
            sd[p][0] = (e * pl.reciprocal(l, approx=True)).astype(bf16)

        def stage_d(p):
            e, _, v = sd[p]
            o = jnp.dot(e, v, preferred_element_type=f32)
            for hh in range(2):
                rows = [o[hh * 32:(hh + 1) * 32]]
                post = o[64 + hh * 8:72 + hh * 8]
                if sl % 2 == 0:
                    ost[2 * p + hh] = post
                else:
                    rows += [post, ost[2 * p + hh]]
                oh = jnp.concatenate(rows, axis=0)
                oc[2 * p + hh] = oh if "of32" in VAR else oh.astype(bf16)

        def stage_e(h0, h1):
            o2 = jnp.concatenate([oc[h] for h in range(h0, h1)], axis=1).astype(bf16)
            return [jnp.dot(o2, _tob(wo[j, h0 * 64:h1 * 64, :]), preferred_element_type=f32)
                    for j in range(NJ)]

        acc = None
        eb = EBS[sl]
        for slot in range(NP + len(eb) - 1):
            def do_b():
                if 0 <= slot - LAG_B < NP:
                    stage_b(slot - LAG_B)

            def do_d():
                if 0 <= slot - LAG_D < NP:
                    stage_d(slot - LAG_D)

            if slot < NP:
                for di in range(7):
                    if di == POS_B and di == POS_D and "dfirst" in VAR:
                        do_d()
                        do_b()
                    else:
                        if di == POS_B:
                            do_b()
                        if di == POS_D:
                            do_d()
                    if di < 6:
                        a_dot(slot, MORD[di // 2], di % 2)
                continue
            else:
                i = slot - NP
                t = stage_e(2 * eb[i], 2 * eb[i + 1])
                acc = t if acc is None else [b + a for a, b in zip(acc, t)]
            if "dfirst" in VAR:
                do_d()
                do_b()
            else:
                do_b()
                do_d()
        acc = jnp.concatenate(acc, axis=1)
        finalize(ci, sl, 8, SEG, acc[8:32])
        if sl % 2 == 1:
            finalize(ci, sl, 0, 8, acc[32:40])
            finalize(ci, sl - 1, 0, 8, acc[40:48])
        return _tou(acc[0:16].astype(bf16))

    def out_cp(*idx):
        return pltpu.make_async_copy(outv.at[idx], out_hbm.at[idx], sem_out.at[0])

    def chunk(ci, carry):
        e2 = contextlib.ExitStack()
        if SCOPES: e2.enter_context(jax.named_scope('chunk'))
        def sc(n):
            if 'fine' in VAR or (':' + n) in VAR:
                e2.close()
                e2.enter_context(jax.named_scope(n))
        mem = memv[...]
        if DELAY:
            z = mem[:, 0:128]
            for _ in range(DELAY):
                z = (z >> 1) + 1
            zs = []
            for c_ in STAG:
                for _ in range(int(c_)):
                    z = (z >> 1) + 1
                zs.append((z >> 16) >> 16)
            mem = mem ^ jnp.concatenate(zs, axis=1)
        for sl in range(CH):
            mem = step(ci, sl, mem)
            if sl % 2 == 1:
                out_cp(ci, pl.ds(sl - 1, 2)).start()
        memv[...] = mem


        e2.close()
        return carry

    scope("mainloop")
    lax.fori_loop(0, NCH, chunk, 0)
    scope("epi")
    scope("waitout")
    for ci in range(NCH):
        out_cp(ci).wait()
    scope(None)


@jax.jit
def pallas_recurrent_scan__memory_aug_recurrent_mem_tr__moe_arch_mod__prompt_kernel(
    A_x, A_mem0, A_Wq, A_Wk, A_Wv, A_Wo, A_seg_len, B_x, B_w_r, B_w_gate, B_w_up, B_w_down,
):
    hbm = pl.BlockSpec(memory_space=pltpu.MemorySpace.HBM)
    out = pl.pallas_call(
        _kernel,
        out_shape=jax.ShapeDtypeStruct((NCH, CH, SEG, D), bf16),
        in_specs=[hbm] * 10,
        out_specs=hbm,
        scratch_shapes=[
            pltpu.VMEM((NCH, CH, SEG, D), bf16),
            pltpu.VMEM((NCH, CH * 16, D), u32),
            pltpu.VMEM((4, 64, D), u32),
            pltpu.VMEM((NCH, CH * SEG, D), f32),
            pltpu.VMEM((NU, D, 128), u32),
            pltpu.VMEM((NU * 2, D // 2, 128), u32),
            pltpu.VMEM((NJ, H * DH // 2, 128), u32),
            pltpu.VMEM((NU, NCH, CH * 8, 128), u32),
            pltpu.VMEM((F, D), bf16),
            pltpu.VMEM((F, D), bf16),
            pltpu.VMEM((F, D), bf16),
            pltpu.VMEM((NCH, CH, SEG, D), bf16),
            pltpu.VMEM((80, 80), f32),
            pltpu.VMEM((8, D), u32),
            pltpu.VMEM((NPL + int(os.environ.get("RPAD", 3)), 8, 128), f32),
            pltpu.VMEM((8, D), f32),
            pltpu.VMEM((M, D), bf16),
            pltpu.VMEM((D,), bf16),
            pltpu.SemaphoreType.DMA((len(GROUPS),)),
            pltpu.SemaphoreType.DMA((1,)),
        ],
        compiler_params=pltpu.CompilerParams(vmem_limit_bytes=100 * 1024 * 1024, disable_bounds_checks=True, disable_semaphore_checks=True, internal_scratch_in_bytes=int(os.environ.get("ISC", 49152))),
        name="rmt_mod",
    )(A_x.reshape(NCH, CH, SEG, D), A_mem0.reshape(M, D), A_Wq, A_Wk, A_Wv, A_Wo.reshape(H * DH, D),
      B_w_r, B_w_gate.T, B_w_up.T, B_w_down)
    return out.reshape(1, S, D)
```

```python
import math

import jax
import jax.numpy as jnp
from jax import lax
import jax.experimental.pallas as pl
import jax.experimental.pallas.tpu as pltpu

bf16 = jnp.bfloat16
f32 = jnp.float32
u32 = jnp.uint32
i32 = jnp.int32

S = 2048
D = 640
H = 32
DH = 128
NP = H // 2
NU = NP * 3
M = 8
SEG = 32
NSEG = S // SEG
F = 1728
C = 8
CH = 4
NCH = NSEG // CH
NJ = D // 128
EPS = 1e-5
NEG = -1e30
LOG2E = math.log2(math.e)
CEXP = (DH ** -0.5) * LOG2E
NT = (((1,), (1,)), ((), ()))

LAG_B, POS_B = 1, 3
LAG_D, POS_D = 3, 6
KMAJ = (5, 5, 4, 5)
MORDS = ((0, 1, 2), (0, 1, 2), (0, 1, 2), (1, 0, 2))
EBS = ((0, 3, 6, 9, 12, 16), (0, 4, 8, 11, 13, 16), (0, 3, 6, 9, 12, 16), (0, 3, 6, 10, 14))
HL = 2 * EBS[CH - 1][-1]

NPL = 4
UPL = 8
U0 = 9
CPL = NCH // NPL
SPL = NSEG // NPL
HEAD_GROUPS = (("p0",), ("w0", "p1"), ("w1", "p2", "p3"), ("w2", "w3", "w4"),
               ("mem0", "wr", "w5", "w6", "w7", "w8"))
HOLD = (0, 0, 0, 2, 2)
LOOP_GROUPS = tuple(
    tuple("w%d" % u for u in range(U0 + i * UPL, U0 + (i + 1) * UPL)) + ("x%d" % i,) for i in range(NPL))
TAIL_GROUPS = (tuple("w%d" % u for u in range(U0 + NPL * UPL, NU)) + ("f0", "f1", "f2"),
               tuple("o%d" % j for j in range(NJ)))
GROUPS = HEAD_GROUPS + LOOP_GROUPS + TAIL_GROUPS
TIE_LAG = 6
LN_NUM, LN_DEN = 6, 7
FFN_SKIP = 14


def _tob(x):
    return pltpu.bitcast(x, bf16)


def _tou(x):
    return pltpu.bitcast(x, u32)


def _zero_of(x):
    return (pltpu.bitcast(x, u32) >> 16) >> 16


def _rb(x):
    return x.astype(bf16).astype(f32)


def _layernorm(x, tie=None):
    ps = x[:, 0:128]
    if tie is not None:
        ps = ps + tie
    for j in range(1, NJ):
        ps = ps + x[:, j * 128:(j + 1) * 128]
    mu = jnp.sum(ps, axis=-1, keepdims=True) * (1.0 / D)
    xc = x - mu
    var = jnp.sum(xc * xc, axis=-1, keepdims=True) * (1.0 / D)
    den = _rb(jnp.sqrt(_rb(_rb(var) + EPS)))
    return (_rb(x - _rb(mu)) * pl.reciprocal(den, approx=False, full_range=False)).astype(bf16)


def _sigmoid(z):
    return pl.reciprocal(1.0 + jnp.exp2(z * (-LOG2E)), approx=True)


def _silu(z):
    return z * _sigmoid(z)


def _dot(a, b):
    return jnp.dot(a, b, preferred_element_type=f32)


def _dot_t(a, b):
    return lax.dot_general(a, b, NT, preferred_element_type=f32)


def _kernel(x_hbm, mem0_hbm, wq_hbm, wk_hbm, wv_hbm, wo_hbm, wr_hbm, wg_hbm, wu_hbm, wd_hbm,
            out_hbm,
            xv, lhs, xpre, zbuf, raw, wqkv, wo, pre, wg, wu, wd, outv, mask_ref,
            accv, ocv, rds, wr8, mem0_v, wr_v, sem, sem_out):
    w32 = [w.bitcast(u32) for w in (wq_hbm, wk_hbm, wv_hbm)]
    wo32 = wo_hbm.bitcast(u32)

    def src_dst(name):
        if name == "mem0":
            return mem0_hbm, mem0_v
        if name == "wr":
            return wr_hbm, wr_v
        k, n = name[0], int(name[1:])
        if k == "x":
            idx = (pl.ds(n * CPL, CPL), slice(None), pl.ds(8, SEG - 8), slice(None))
            return x_hbm.at[idx], xv.at[idx]
        if k == "p":
            idx = (pl.ds(n * 4, 4), slice(None), pl.ds(0, 8), slice(None))
            return x_hbm.at[idx], xv.at[idx]
        if k == "w":
            return w32[n % 3].at[:, n // 3, :], raw.at[n]
        if k == "f":
            return ((wg_hbm, wg), (wu_hbm, wu), (wd_hbm, wd))[n]
        return wo32.at[:, pl.ds(n * 128, 128)], wo.at[n]

    cps = [[pltpu.make_async_copy(*src_dst(nm), sem.at[gi]) for nm in grp]
           for gi, grp in enumerate(GROUPS)]
    for grp in cps:
        for cp in grp:
            cp.start()

    def head_pos(i):
        head = jnp.where(i < 32, 0, jnp.where(i < 64, 1, jnp.where(i < 72, 0, 1)))
        j = i & 31
        pos = jnp.where(i < 64, jnp.where(j < 8, j, j + 8), 8 + (i & 7))
        return head, pos

    hr, pr = head_pos(lax.broadcasted_iota(i32, (80, 80), 0))
    hc, pc = head_pos(lax.broadcasted_iota(i32, (80, 80), 1))
    mask_ref[...] = jnp.where((hr == hc) & ((pr < M) | (pr >= pc)), 1.0, 0.0).astype(f32)

    st = {}
    lane8 = lax.broadcasted_iota(i32, (8, 128), 1)
    sub8 = lax.broadcasted_iota(i32, (8, 128), 0)

    def ln_pre(b):
        xb = xv[b * 4:(b + 1) * 4, :, 0:8, :].astype(f32).reshape(128, D)
        xpre[b] = _tou(_layernorm(xb))

    def repack(u):
        ev = raw[u, pl.ds(0, D // 2, stride=2), :]
        od = raw[u, pl.ds(1, D // 2, stride=2), :]
        ws = ((ev & jnp.uint32(0xFFFF)) | (od << 16), (ev >> 16) | (od & jnp.uint32(0xFFFF0000)))
        wqkv[2 * u] = ws[0]
        wqkv[2 * u + 1] = ws[1]
        return ws

    def pre_dots(u, b, hook, ws=None):
        xu = xpre[b]
        res = []
        for hh in range(2):
            tie = hook()
            xt = xu
            if tie is not None:
                top = jnp.concatenate([xu[0:8, 0:128] ^ tie, xu[0:8, 128:]], axis=1)
                xt = jnp.concatenate([top, xu[8:]], axis=0)
            w = wqkv[2 * u + hh] if ws is None else ws[hh]
            res.append(_dot(_tob(xt), _tob(w)))
            st["after"] = res[-1][0:8]
        parts = []
        for k in range(16):
            parts += [res[0][k * 8:(k + 1) * 8], res[1][k * 8:(k + 1) * 8]]
        pre[u, b * 4:(b + 1) * 4] = _tou(jnp.concatenate(parts, axis=0).astype(bf16)).reshape(4, CH * 8, 128)

    def score(i, gl, xn32):
        zbuf[i * CPL + gl // 16, (gl % 16) * 8:(gl % 16) * 8 + 8, :] = xn32
        rc = jnp.sum(xn32 * st["wr"], axis=-1, keepdims=True)
        st["rd"] = jnp.where(lane8 == gl, rc, st["rd"])

    def ln_group(i, s, k):
        tie = None
        if st["after"] is not None:
            tie = pltpu.bitcast(_zero_of(st["after"]), f32)
        xn = _layernorm(xv[i * CPL + s // CH, s % CH, k * 8:(k + 1) * 8, :].astype(f32), tie)
        score(i, s * 4 + k, xn.astype(f32))
        if k == 1 and s % 2 == 0:
            xp = _tob(xpre[i, s * 4:s * 4 + 8, :]).astype(f32)
            score(i, s * 4, xp[0:8])
            score(i, s * 4 + 4, xp[8:16])
        if k == 2:
            st["xn2"] = xn
        else:
            r0 = (s % CH) * 16 + (k // 2) * 8
            pair = jnp.concatenate([xn if k == 1 else st["xn2"], xn], axis=0)
            lhs[i * CPL + s // CH, r0:r0 + 8, :] = _tou(pair)
        return _zero_of(st["rd"])

    def topk():
        rd = _rb(rds[...].reshape(NPL * 8, 128))
        rd = jnp.where(rd == 0.0, 0.0, rd)
        bits = pltpu.bitcast(rd, i32)
        mono = jnp.where(bits < 0, bits ^ jnp.int32(0x7FFFFFFF), bits)
        rowid = jnp.concatenate([lane8 * 8 + sub8 + i * SPL * SEG for i in range(NPL)], axis=0)
        key = ((((mono >> 16) + 32768) << 11) | (S - 1 - rowid)) | jnp.int32(0x20000000)
        key = jnp.where(jnp.concatenate([lane8] * NPL, axis=0) < SPL * 4, pltpu.bitcast(key, f32), 0.0)
        row8 = lax.broadcasted_iota(i32, (8, 1), 0)
        ksel = jnp.zeros((8, 1), f32)
        for t in range(C):
            km = jnp.max(jnp.max(key, axis=0, keepdims=True), axis=1, keepdims=True)
            key = jnp.where(key == km, 0.0, key)
            ksel = jnp.where(row8 == t, km, ksel)
        ksel = pltpu.bitcast(ksel, i32)
        iv = S - 1 - (ksel & (S - 1))
        idxs = [iv[t, 0] for t in range(C)]
        xs = jnp.concatenate([zbuf[i_ >> 7, pl.ds(i_ & 127, 1), :] for i_ in idxs], axis=0)
        hi16 = (((ksel >> 11) & 65535) - 32768) << 16
        rbits = jnp.where(hi16 < 0, hi16 ^ jnp.int32(0x7FFF0000), hi16)
        return idxs, xs, _rb(_sigmoid(pltpu.bitcast(rbits, f32)))

    def ffn_tasks(idxs, xs, rsel):
        cols = [(k * 128, min(F, (k + 1) * 128)) for k in range(pl.cdiv(F, 128))]
        xsb = xs.astype(bf16)
        hid = []
        tmp = {}

        def gate(a, b):
            tmp["g"] = _rb(_dot_t(xsb, wg[a:b, :]))

        def up(a, b):
            hid.append((_rb(_silu(tmp["g"])) * _rb(_dot_t(xsb, wu[a:b, :]))).astype(bf16))

        def down(k):
            t = _dot(hid[k], wd[cols[k][0]:cols[k][1], :])
            tmp["y"] = t if k == 0 else t + tmp["y"]

        def fin():
            zs = _rb(xs + _rb(_rb(tmp["y"]) * rsel))
            for t in range(C):
                zbuf[idxs[t] >> 7, pl.ds(idxs[t] & 127, 1), :] = zs[t:t + 1]

        tasks = []
        for a, b in cols:
            tasks += [lambda a=a, b=b: gate(a, b), lambda a=a, b=b: up(a, b)]
        tasks += [lambda k=k: down(k) for k in range(len(cols))]
        return tasks + [fin]

    def run_region(work, side=(), tasks=(), skip=0):
        side, tasks = list(side), list(tasks)
        ties = []
        st["after"] = None
        cnt = {"dot": 0, "credit": 0}

        def hook():
            di = cnt["dot"]
            cnt["dot"] += 1
            if tasks and di >= skip:
                tasks.pop(0)()
            tie = None
            if ties and ties[0][0] <= di:
                tie = ties.pop(0)[1]
            if side and di + TIE_LAG < 2 * len(work):
                cnt["credit"] += LN_NUM
                if cnt["credit"] >= LN_DEN:
                    cnt["credit"] -= LN_DEN
                    ties.append((di + TIE_LAG, ln_group(*side.pop(0))))
            return tie

        for u, b, *ws in work:
            pre_dots(u, b, hook, *ws)
        assert not ties and not side and not tasks

    pending = []
    units, blocks = [], []
    for gi, grp in enumerate(HEAD_GROUPS):
        for cp in cps[gi]:
            cp.wait()
        for u in [int(nm[1:]) for nm in grp if nm[0] == "w" and nm != "wr"]:
            repack(u)
            pending += [(u, b) for b in blocks]
            units.append(u)
        for b in [int(nm[1:]) for nm in grp if nm[0] == "p"]:
            ln_pre(b)
            pending += [(u, b) for u in units]
            blocks.append(b)
        if "mem0" in grp:
            accv[...] = jnp.concatenate([mem0_v[...].astype(f32), jnp.zeros((40, D), f32)], axis=0)
            ocv[...] = jnp.zeros(ocv.shape, f32)
            wr8[...] = jnp.broadcast_to(wr_v[...].astype(f32).reshape(1, D), (8, D))
        n = len(pending) - HOLD[gi]
        work, pending = pending[:n], pending[n:]
        run_region(work)
    assert pending == [(U0 - 1, 2), (U0 - 1, 3)]

    def pro_body(i, carry):
        ub = U0 + i * UPL
        for k in range(UPL):
            pltpu.make_async_copy(w32[0].at[:, 0, :], raw.at[ub + k], sem.at[len(HEAD_GROUPS) + i]).wait()
        idx = (pl.ds(i * CPL, CPL), slice(None), pl.ds(8, SEG - 8), slice(None))
        pltpu.make_async_copy(x_hbm.at[idx], xv.at[idx], sem.at[len(HEAD_GROUPS) + i]).wait()
        ws = [None] + [repack(ub + k) for k in range(UPL)]
        work = [(ub - 1 + k // 4, k % 4, ws[k // 4]) for k in range(2, 2 + 4 * UPL)]
        st["wr"] = wr8[...]
        st["rd"] = jnp.zeros((8, 128), f32)
        run_region(work, side=[(i, s, k) for s in range(SPL) for k in (1, 2, 3)])
        rds[i] = st["rd"]
        return carry

    lax.fori_loop(0, NPL, pro_body, 0)

    for cp in cps[-2]:
        cp.wait()
    ub = U0 + NPL * UPL
    for u in range(ub, NU):
        repack(u)
    run_region([(ub - 1 + k // 4, k % 4) for k in range(2, 4 + 4 * (NU - ub))],
               tasks=ffn_tasks(*topk()), skip=FFN_SKIP)
    for cp in cps[-1]:
        cp.wait()

    sub4 = lax.broadcasted_iota(i32, (8, D), 0) < 4
    ost = {}

    def finalize(ci, sl, r0, r1, sv):
        xr = xv[ci, sl, r0:r1, :].astype(f32)
        g = _silu(zbuf[ci, sl * SEG + r0:sl * SEG + r1, :])
        outv[ci, sl, r0:r1, :] = (xr + sv * g).astype(bf16)

    def finish(ci, sl, acc):
        acc = jnp.concatenate(acc, axis=1)
        finalize(ci, sl, 8, SEG, acc[8:32])
        if sl % 2 == 1:
            finalize(ci, sl, 0, 8, acc[32:40])
            finalize(ci, sl - 1, 0, 8, acc[40:48])
        return _tou(acc[0:16].astype(bf16))

    def finish_last(ci):
        o2 = ocv[...].astype(bf16)
        acc = [_dot(o2, _tob(wo[j, HL * 64:, :])) + accv[:, j * 128:(j + 1) * 128] for j in range(NJ)]
        return finish(ci, CH - 1, acc)

    def step(ci, sl, mem):
        xu = lhs[ci, sl * 16:(sl + 1) * 16, :]
        x = _tob(jnp.concatenate([jnp.where(sub4, mem, xu[0:8]), xu[8:16]], axis=0))
        mord, eb = MORDS[sl], EBS[sl]
        sd = {}
        oc = {}

        early = {}
        for k in range(NJ):
            for d in range(KMAJ[sl]):
                key = (d // 6, mord[(d % 6) // 2], d % 2)
                w = _tob(wqkv[2 * (key[0] * 3 + key[1]) + key[2], k * 64:(k + 1) * 64, :])
                t = _dot(x[:, k * 128:(k + 1) * 128], w)
                early[key] = t if k == 0 else t + early[key]

        def project(p, m, hh):
            u = p * 3 + m
            outs = sd.setdefault(p, [None, None, None])
            r = early[p, m, hh] if (p, m, hh) in early else _dot(x, _tob(wqkv[2 * u + hh]))
            if hh == 0:
                outs[m] = r
            else:
                pb = _tob(pre[u, ci, sl * 8:(sl + 1) * 8, :]).astype(f32)
                outs[m] = jnp.concatenate([outs[m], r, pb], axis=0).astype(bf16)

        def scores(p):
            if not 0 <= p < NP:
                return
            sc = jnp.where(mask_ref[...] > 0.5, _dot_t(sd[p][0], sd[p][1]), NEG)
            e = jnp.exp2((sc - jnp.max(sc, axis=-1, keepdims=True)) * CEXP)
            l = jnp.sum(e, axis=-1, keepdims=True)
            sd[p][0] = (e * pl.reciprocal(l, approx=True)).astype(bf16)

        def attend(p):
            if not 0 <= p < NP:
                return
            o = _dot(sd[p][0], sd[p][2])
            for hh in range(2):
                rows = [o[hh * 32:(hh + 1) * 32]]
                first = o[64 + hh * 8:72 + hh * 8]
                if sl % 2 == 0:
                    ost[2 * p + hh] = first
                else:
                    rows += [first, ost[2 * p + hh]]
                oc[2 * p + hh] = jnp.concatenate(rows, axis=0)

        for slot in range(NP):
            for di in range(7):
                if di == POS_B:
                    scores(slot - LAG_B)
                if di == POS_D:
                    attend(slot - LAG_D)
                if di < 6:
                    project(slot, mord[di // 2], di % 2)
        acc = None
        for i in range(len(eb) - 1):
            h0, h1 = 2 * eb[i], 2 * eb[i + 1]
            o2 = jnp.concatenate([oc[h] for h in range(h0, h1)], axis=1).astype(bf16)
            t = [_dot(o2, _tob(wo[j, h0 * 64:h1 * 64, :])) for j in range(NJ)]
            acc = t if acc is None else [b + a for a, b in zip(acc, t)]
            scores(NP + i - LAG_B)
            attend(NP + i - LAG_D)
        if sl == CH - 1:
            accv[...] = jnp.concatenate(acc, axis=1)
            ocv[...] = jnp.concatenate([oc[h] for h in range(HL, H)], axis=1)
            return None
        return finish(ci, sl, acc)

    def out_cp(*idx):
        return pltpu.make_async_copy(outv.at[idx], out_hbm.at[idx], sem_out.at[0])

    def chunk(ci, carry):
        prev = jnp.maximum(ci - 1, 0)
        mem = finish_last(prev)

        @pl.when(ci >= 1)
        def _():
            out_cp(prev, pl.ds(2, 2)).start()

        for sl in range(CH):
            mem = step(ci, sl, mem)
            if sl == 1:
                out_cp(ci, pl.ds(0, 2)).start()
        return carry

    lax.fori_loop(0, NCH, chunk, 0)
    finish_last(NCH - 1)
    out_cp(NCH - 1, pl.ds(2, 2)).start()
    pltpu.make_async_copy(outv, out_hbm, sem_out.at[0]).wait()


@jax.jit
def pallas_recurrent_scan__memory_aug_recurrent_mem_tr__moe_arch_mod__prompt_kernel(
    A_x, A_mem0, A_Wq, A_Wk, A_Wv, A_Wo, A_seg_len, B_x, B_w_r, B_w_gate, B_w_up, B_w_down,
):
    hbm = pl.BlockSpec(memory_space=pltpu.MemorySpace.HBM)
    out = pl.pallas_call(
        _kernel,
        out_shape=jax.ShapeDtypeStruct((NCH, CH, SEG, D), bf16),
        in_specs=[hbm] * 10,
        out_specs=hbm,
        scratch_shapes=[
            pltpu.VMEM((NCH, CH, SEG, D), bf16),
            pltpu.VMEM((NCH, CH * 16, D), u32),
            pltpu.VMEM((4, 64, D), u32),
            pltpu.VMEM((NCH, CH * SEG, D), f32),
            pltpu.VMEM((NU, D, 128), u32),
            pltpu.VMEM((NU * 2, D // 2, 128), u32),
            pltpu.VMEM((NJ, H * DH // 2, 128), u32),
            pltpu.VMEM((NU, NCH, CH * 8, 128), u32),
            pltpu.VMEM((F, D), bf16),
            pltpu.VMEM((F, D), bf16),
            pltpu.VMEM((F, D), bf16),
            pltpu.VMEM((NCH, CH, SEG, D), bf16),
            pltpu.VMEM((80, 80), f32),
            pltpu.VMEM((48, D), f32),
            pltpu.VMEM((48, (H - HL) * DH), f32),
            pltpu.VMEM((NPL, 8, 128), f32),
            pltpu.VMEM((8, D), f32),
            pltpu.VMEM((M, D), bf16),
            pltpu.VMEM((D,), bf16),
            pltpu.SemaphoreType.DMA((len(GROUPS),)),
            pltpu.SemaphoreType.DMA((1,)),
        ],
        compiler_params=pltpu.CompilerParams(
            vmem_limit_bytes=100 * 1024 * 1024,
            disable_bounds_checks=True,
            disable_semaphore_checks=True,
            internal_scratch_in_bytes=48 * 1024,
        ),
        name="rmt_mod",
    )(A_x.reshape(NCH, CH, SEG, D), A_mem0.reshape(M, D), A_Wq, A_Wk, A_Wv, A_Wo.reshape(H * DH, D),
      B_w_r, B_w_gate.T, B_w_up.T, B_w_down)
    return out.reshape(1, S, D)
```

```python
import math

import jax
import jax.numpy as jnp
from jax import lax
import jax.experimental.pallas as pl
import jax.experimental.pallas.tpu as pltpu

bf16 = jnp.bfloat16
f32 = jnp.float32
u32 = jnp.uint32
i32 = jnp.int32

S = 2048
D = 640
H = 32
DH = 128
NP = H // 2
NU = NP * 3
M = 8
SEG = 32
NSEG = S // SEG
F = 1728
C = 8
CH = 4
NCH = NSEG // CH
NJ = D // 128
EPS = 1e-5
NEG = -1e30
LOG2E = math.log2(math.e)
CEXP = (DH ** -0.5) * LOG2E
NT = (((1,), (1,)), ((), ()))

LAG_B, POS_B = 1, 3
LAG_D, POS_D = 3, 6
KMAJ = (5, 5, 4, 5)
MORDS = ((0, 1, 2), (1, 0, 2), (1, 0, 2), (1, 0, 2))
EBS = ((0, 6, 12, 20, 22, 32), (0, 8, 16, 21, 23, 32), (0, 8, 12, 17, 23, 32), (0, 6, 12, 20, 28))
EPOS = ((2, 4), (4, 4), (1, 3), (4, 4))
HL = EBS[CH - 1][-1]

NPL = 4
UPL = 8
U0 = 9
CPL = NCH // NPL
SPL = NSEG // NPL
HEAD_GROUPS = (("p0",), ("w0", "p1"), ("w1", "p2", "p3"), ("w2", "w3", "w4"),
               ("mem0", "wr", "w5", "w6", "w7", "w8"))
HOLD = (0, 0, 0, 2, 2)
LOOP_GROUPS = tuple(
    tuple("w%d" % u for u in range(U0 + i * UPL, U0 + (i + 1) * UPL)) + ("x%d" % i,) for i in range(NPL))
TAIL_GROUPS = (tuple("w%d" % u for u in range(U0 + NPL * UPL, NU)) + ("f0", "f1", "f2"),
               tuple("o%d" % j for j in range(NJ)))
GROUPS = HEAD_GROUPS + LOOP_GROUPS + TAIL_GROUPS
TIE_LAG = 6
LN_NUM, LN_DEN = 6, 7
FFN_SKIP = 14


def _tob(x):
    return pltpu.bitcast(x, bf16)


def _tou(x):
    return pltpu.bitcast(x, u32)


def _zero_of(x):
    return (pltpu.bitcast(x, u32) >> 16) >> 16


def _rb(x):
    return x.astype(bf16).astype(f32)


def _layernorm(x, tie=None):
    ps = x[:, 0:128]
    if tie is not None:
        ps = ps + tie
    for j in range(1, NJ):
        ps = ps + x[:, j * 128:(j + 1) * 128]
    mu = jnp.sum(ps, axis=-1, keepdims=True) * (1.0 / D)
    xc = x - mu
    var = jnp.sum(xc * xc, axis=-1, keepdims=True) * (1.0 / D)
    den = _rb(jnp.sqrt(_rb(_rb(var) + EPS)))
    return (_rb(x - _rb(mu)) * pl.reciprocal(den, approx=False, full_range=False)).astype(bf16)


def _sigmoid(z):
    return pl.reciprocal(1.0 + jnp.exp2(z * (-LOG2E)), approx=True)


def _silu(z):
    return z * _sigmoid(z)


def _dot(a, b):
    return jnp.dot(a, b, preferred_element_type=f32)


def _dot_t(a, b):
    return lax.dot_general(a, b, NT, preferred_element_type=f32)


def _kernel(x_hbm, mem0_hbm, wq_hbm, wk_hbm, wv_hbm, wo_hbm, wr_hbm, wg_hbm, wu_hbm, wd_hbm,
            out_hbm,
            xv, lhs, xpre, zbuf, raw, wqkv, wo, pre, wg, wu, wd, outv, mask_ref,
            accv, ocv, rds, wr8, mem0_v, wr_v, sem, sem_out):
    w32 = [w.bitcast(u32) for w in (wq_hbm, wk_hbm, wv_hbm)]
    wo32 = wo_hbm.bitcast(u32)

    def src_dst(name):
        if name == "mem0":
            return mem0_hbm, mem0_v
        if name == "wr":
            return wr_hbm, wr_v
        k, n = name[0], int(name[1:])
        if k == "x":
            idx = (pl.ds(n * CPL, CPL), slice(None), pl.ds(8, SEG - 8), slice(None))
            return x_hbm.at[idx], xv.at[idx]
        if k == "p":
            idx = (pl.ds(n * 4, 4), slice(None), pl.ds(0, 8), slice(None))
            return x_hbm.at[idx], xv.at[idx]
        if k == "w":
            return w32[n % 3].at[:, n // 3, :], raw.at[n]
        if k == "f":
            return ((wg_hbm, wg), (wu_hbm, wu), (wd_hbm, wd))[n]
        return wo32.at[:, pl.ds(n * 128, 128)], wo.at[n]

    cps = [[pltpu.make_async_copy(*src_dst(nm), sem.at[gi]) for nm in grp]
           for gi, grp in enumerate(GROUPS)]
    for grp in cps:
        for cp in grp:
            cp.start()

    def head_pos(i):
        head = jnp.where(i < 32, 0, jnp.where(i < 64, 1, jnp.where(i < 72, 0, 1)))
        j = i & 31
        pos = jnp.where(i < 64, jnp.where(j < 8, j, j + 8), 8 + (i & 7))
        return head, pos

    hr, pr = head_pos(lax.broadcasted_iota(i32, (80, 80), 0))
    hc, pc = head_pos(lax.broadcasted_iota(i32, (80, 80), 1))
    mask_ref[...] = jnp.where((hr == hc) & ((pr < M) | (pr >= pc)), 1.0, 0.0).astype(f32)

    st = {}
    lane8 = lax.broadcasted_iota(i32, (8, 128), 1)
    sub8 = lax.broadcasted_iota(i32, (8, 128), 0)

    def ln_pre(b):
        xb = xv[b * 4:(b + 1) * 4, :, 0:8, :].astype(f32).reshape(128, D)
        xpre[b] = _tou(_layernorm(xb))

    def repack(u):
        ev = raw[u, pl.ds(0, D // 2, stride=2), :]
        od = raw[u, pl.ds(1, D // 2, stride=2), :]
        ws = ((ev & jnp.uint32(0xFFFF)) | (od << 16), (ev >> 16) | (od & jnp.uint32(0xFFFF0000)))
        wqkv[2 * u] = ws[0]
        wqkv[2 * u + 1] = ws[1]
        return ws

    def pre_dots(u, b, hook, ws=None):
        xu = xpre[b]
        res = []
        for hh in range(2):
            tie = hook()
            xt = xu
            if tie is not None:
                top = jnp.concatenate([xu[0:8, 0:128] ^ tie, xu[0:8, 128:]], axis=1)
                xt = jnp.concatenate([top, xu[8:]], axis=0)
            w = wqkv[2 * u + hh] if ws is None else ws[hh]
            res.append(_dot(_tob(xt), _tob(w)))
            st["after"] = res[-1][0:8]
        parts = []
        for k in range(16):
            parts += [res[0][k * 8:(k + 1) * 8], res[1][k * 8:(k + 1) * 8]]
        pre[u, b * 4:(b + 1) * 4] = _tou(jnp.concatenate(parts, axis=0).astype(bf16)).reshape(4, CH * 8, 128)

    def score(i, gl, xn32):
        zbuf[i * CPL + gl // 16, (gl % 16) * 8:(gl % 16) * 8 + 8, :] = xn32
        rc = jnp.sum(xn32 * st["wr"], axis=-1, keepdims=True)
        st["rd"] = jnp.where(lane8 == gl, rc, st["rd"])

    def ln_group(i, s, k):
        tie = None
        if st["after"] is not None:
            tie = pltpu.bitcast(_zero_of(st["after"]), f32)
        xn = _layernorm(xv[i * CPL + s // CH, s % CH, k * 8:(k + 1) * 8, :].astype(f32), tie)
        score(i, s * 4 + k, xn.astype(f32))
        if k == 1 and s % 2 == 0:
            xp = _tob(xpre[i, s * 4:s * 4 + 8, :]).astype(f32)
            score(i, s * 4, xp[0:8])
            score(i, s * 4 + 4, xp[8:16])
        if k == 2:
            st["xn2"] = xn
        else:
            r0 = (s % CH) * 16 + (k // 2) * 8
            pair = jnp.concatenate([xn if k == 1 else st["xn2"], xn], axis=0)
            lhs[i * CPL + s // CH, r0:r0 + 8, :] = _tou(pair)
        return _zero_of(st["rd"])

    def topk():
        rd = _rb(rds[...].reshape(NPL * 8, 128))
        rd = jnp.where(rd == 0.0, 0.0, rd)
        bits = pltpu.bitcast(rd, i32)
        mono = jnp.where(bits < 0, bits ^ jnp.int32(0x7FFFFFFF), bits)
        rowid = jnp.concatenate([lane8 * 8 + sub8 + i * SPL * SEG for i in range(NPL)], axis=0)
        key = ((((mono >> 16) + 32768) << 11) | (S - 1 - rowid)) | jnp.int32(0x20000000)
        key = jnp.where(jnp.concatenate([lane8] * NPL, axis=0) < SPL * 4, pltpu.bitcast(key, f32), 0.0)
        row8 = lax.broadcasted_iota(i32, (8, 1), 0)
        ksel = jnp.zeros((8, 1), f32)
        for t in range(C):
            km = jnp.max(jnp.max(key, axis=0, keepdims=True), axis=1, keepdims=True)
            key = jnp.where(key == km, 0.0, key)
            ksel = jnp.where(row8 == t, km, ksel)
        ksel = pltpu.bitcast(ksel, i32)
        iv = S - 1 - (ksel & (S - 1))
        idxs = [iv[t, 0] for t in range(C)]
        xs = jnp.concatenate([zbuf[i_ >> 7, pl.ds(i_ & 127, 1), :] for i_ in idxs], axis=0)
        hi16 = (((ksel >> 11) & 65535) - 32768) << 16
        rbits = jnp.where(hi16 < 0, hi16 ^ jnp.int32(0x7FFF0000), hi16)
        return idxs, xs, _rb(_sigmoid(pltpu.bitcast(rbits, f32)))

    def ffn_tasks(idxs, xs, rsel):
        cols = [(k * 128, min(F, (k + 1) * 128)) for k in range(pl.cdiv(F, 128))]
        xsb = xs.astype(bf16)
        hid = []
        tmp = {}

        def gate(a, b):
            tmp["g"] = _rb(_dot_t(xsb, wg[a:b, :]))

        def up(a, b):
            hid.append((_rb(_silu(tmp["g"])) * _rb(_dot_t(xsb, wu[a:b, :]))).astype(bf16))

        def down(k):
            t = _dot(hid[k], wd[cols[k][0]:cols[k][1], :])
            tmp["y"] = t if k == 0 else t + tmp["y"]

        def fin():
            zs = _rb(xs + _rb(_rb(tmp["y"]) * rsel))
            for t in range(C):
                zbuf[idxs[t] >> 7, pl.ds(idxs[t] & 127, 1), :] = zs[t:t + 1]

        tasks = []
        for a, b in cols:
            tasks += [lambda a=a, b=b: gate(a, b), lambda a=a, b=b: up(a, b)]
        tasks += [lambda k=k: down(k) for k in range(len(cols))]
        return tasks + [fin]

    def run_region(work, side=(), tasks=(), skip=0):
        side, tasks = list(side), list(tasks)
        ties = []
        st["after"] = None
        cnt = {"dot": 0, "credit": 0}

        def hook():
            di = cnt["dot"]
            cnt["dot"] += 1
            if tasks and di >= skip:
                tasks.pop(0)()
            tie = None
            if ties and ties[0][0] <= di:
                tie = ties.pop(0)[1]
            if side and di + TIE_LAG < 2 * len(work):
                cnt["credit"] += LN_NUM
                if cnt["credit"] >= LN_DEN:
                    cnt["credit"] -= LN_DEN
                    ties.append((di + TIE_LAG, ln_group(*side.pop(0))))
            return tie

        for u, b, *ws in work:
            pre_dots(u, b, hook, *ws)
        assert not ties and not side and not tasks

    pending = []
    units, blocks = [], []
    for gi, grp in enumerate(HEAD_GROUPS):
        for cp in cps[gi]:
            cp.wait()
        for u in [int(nm[1:]) for nm in grp if nm[0] == "w" and nm != "wr"]:
            repack(u)
            pending += [(u, b) for b in blocks]
            units.append(u)
        for b in [int(nm[1:]) for nm in grp if nm[0] == "p"]:
            ln_pre(b)
            pending += [(u, b) for u in units]
            blocks.append(b)
        if "mem0" in grp:
            accv[...] = jnp.concatenate([mem0_v[...].astype(f32), jnp.zeros((40, D), f32)], axis=0)
            ocv[...] = jnp.zeros(ocv.shape, f32)
            wr8[...] = jnp.broadcast_to(wr_v[...].astype(f32).reshape(1, D), (8, D))
        n = len(pending) - HOLD[gi]
        work, pending = pending[:n], pending[n:]
        run_region(work)
    assert pending == [(U0 - 1, 2), (U0 - 1, 3)]

    def pro_body(i, carry):
        ub = U0 + i * UPL
        for k in range(UPL):
            pltpu.make_async_copy(w32[0].at[:, 0, :], raw.at[ub + k], sem.at[len(HEAD_GROUPS) + i]).wait()
        idx = (pl.ds(i * CPL, CPL), slice(None), pl.ds(8, SEG - 8), slice(None))
        pltpu.make_async_copy(x_hbm.at[idx], xv.at[idx], sem.at[len(HEAD_GROUPS) + i]).wait()
        ws = [None] + [repack(ub + k) for k in range(UPL)]
        work = [(ub - 1 + k // 4, k % 4, ws[k // 4]) for k in range(2, 2 + 4 * UPL)]
        st["wr"] = wr8[...]
        st["rd"] = jnp.zeros((8, 128), f32)
        run_region(work, side=[(i, s, k) for s in range(SPL) for k in (1, 2, 3)])
        rds[i] = st["rd"]
        return carry

    lax.fori_loop(0, NPL, pro_body, 0)

    for cp in cps[-2]:
        cp.wait()
    ub = U0 + NPL * UPL
    for u in range(ub, NU):
        repack(u)
    run_region([(ub - 1 + k // 4, k % 4) for k in range(2, 4 + 4 * (NU - ub))],
               tasks=ffn_tasks(*topk()), skip=FFN_SKIP)
    for cp in cps[-1]:
        cp.wait()

    sub4 = lax.broadcasted_iota(i32, (8, D), 0) < 4
    ost = {}

    def finalize(ci, sl, r0, r1, sv):
        xr = xv[ci, sl, r0:r1, :].astype(f32)
        g = _silu(zbuf[ci, sl * SEG + r0:sl * SEG + r1, :])
        outv[ci, sl, r0:r1, :] = (xr + sv * g).astype(bf16)

    def finish(ci, sl, acc):
        acc = jnp.concatenate(acc, axis=1)
        finalize(ci, sl, 8, SEG, acc[8:32])
        if sl % 2 == 1:
            finalize(ci, sl, 0, 8, acc[32:40])
            finalize(ci, sl - 1, 0, 8, acc[40:48])
        return _tou(acc[0:16].astype(bf16))

    def finish_last(ci):
        o2 = ocv[...].astype(bf16)
        acc = [_dot(o2, _tob(wo[j, HL * 64:, :])) + accv[:, j * 128:(j + 1) * 128] for j in range(NJ)]
        return finish(ci, CH - 1, acc)

    def step(ci, sl, mem):
        xu = lhs[ci, sl * 16:(sl + 1) * 16, :]
        x = _tob(jnp.concatenate([jnp.where(sub4, mem, xu[0:8]), xu[8:16]], axis=0))
        mord, eb = MORDS[sl], EBS[sl]
        sd = {}
        oc = {}

        early = {}
        for k in range(NJ):
            for d in range(KMAJ[sl]):
                key = (d // 6, mord[(d % 6) // 2], d % 2)
                w = _tob(wqkv[2 * (key[0] * 3 + key[1]) + key[2], k * 64:(k + 1) * 64, :])
                t = _dot(x[:, k * 128:(k + 1) * 128], w)
                early[key] = t if k == 0 else t + early[key]

        def project(p, m, hh):
            u = p * 3 + m
            outs = sd.setdefault(p, [None, None, None])
            r = early[p, m, hh] if (p, m, hh) in early else _dot(x, _tob(wqkv[2 * u + hh]))
            if hh == 0:
                outs[m] = r
            else:
                pb = _tob(pre[u, ci, sl * 8:(sl + 1) * 8, :]).astype(f32)
                outs[m] = jnp.concatenate([outs[m], r, pb], axis=0).astype(bf16)

        def scores(p):
            if not 0 <= p < NP:
                return
            sc = jnp.where(mask_ref[...] > 0.5, _dot_t(sd[p][0], sd[p][1]), NEG)
            e = jnp.exp2((sc - jnp.max(sc, axis=-1, keepdims=True)) * CEXP)
            l = jnp.sum(e, axis=-1, keepdims=True)
            sd[p][0] = (e * pl.reciprocal(l, approx=True)).astype(bf16)

        def attend(p):
            if not 0 <= p < NP:
                return
            o = _dot(sd[p][0], sd[p][2])
            for hh in range(2):
                rows = [o[hh * 32:(hh + 1) * 32]]
                first = o[64 + hh * 8:72 + hh * 8]
                if sl % 2 == 0:
                    ost[2 * p + hh] = first
                else:
                    rows += [first, ost[2 * p + hh]]
                oc[2 * p + hh] = jnp.concatenate(rows, axis=0)

        for slot in range(NP):
            for di in range(7):
                if di == POS_B:
                    scores(slot - LAG_B)
                if di == POS_D:
                    attend(slot - LAG_D)
                if di < 6:
                    project(slot, mord[di // 2], di % 2)
        acc = [None] * NJ
        for i in range(len(eb) - 1):
            h0, h1 = eb[i], eb[i + 1]
            o2 = jnp.concatenate([oc[h] for h in range(h0, h1)], axis=1).astype(bf16)
            for j in range(NJ):
                t = _dot(o2, _tob(wo[j, h0 * 64:h1 * 64, :]))
                acc[j] = t if acc[j] is None else t + acc[j]
                if j == EPOS[sl][0]:
                    scores(NP + i - LAG_B)
                if j == EPOS[sl][1]:
                    attend(NP + i - LAG_D)
        if sl == CH - 1:
            accv[...] = jnp.concatenate(acc, axis=1)
            ocv[...] = jnp.concatenate([oc[h] for h in range(HL, H)], axis=1)
            return None
        return finish(ci, sl, acc)

    def out_cp(*idx):
        return pltpu.make_async_copy(outv.at[idx], out_hbm.at[idx], sem_out.at[0])

    def chunk(ci, carry):
        prev = jnp.maximum(ci - 1, 0)
        mem = finish_last(prev)

        @pl.when(ci >= 1)
        def _():
            out_cp(prev, pl.ds(2, 2)).start()

        for sl in range(CH):
            mem = step(ci, sl, mem)
            if sl == 1:
                out_cp(ci, pl.ds(0, 2)).start()
        return carry

    lax.fori_loop(0, NCH, chunk, 0)
    finish_last(NCH - 1)
    out_cp(NCH - 1, pl.ds(2, 2)).start()
    pltpu.make_async_copy(outv, out_hbm, sem_out.at[0]).wait()


@jax.jit
def pallas_recurrent_scan__memory_aug_recurrent_mem_tr__moe_arch_mod__prompt_kernel(
    A_x, A_mem0, A_Wq, A_Wk, A_Wv, A_Wo, A_seg_len, B_x, B_w_r, B_w_gate, B_w_up, B_w_down,
):
    hbm = pl.BlockSpec(memory_space=pltpu.MemorySpace.HBM)
    out = pl.pallas_call(
        _kernel,
        out_shape=jax.ShapeDtypeStruct((NCH, CH, SEG, D), bf16),
        in_specs=[hbm] * 10,
        out_specs=hbm,
        scratch_shapes=[
            pltpu.VMEM((NCH, CH, SEG, D), bf16),
            pltpu.VMEM((NCH, CH * 16, D), u32),
            pltpu.VMEM((4, 64, D), u32),
            pltpu.VMEM((NCH, CH * SEG, D), f32),
            pltpu.VMEM((NU, D, 128), u32),
            pltpu.VMEM((NU * 2, D // 2, 128), u32),
            pltpu.VMEM((NJ, H * DH // 2, 128), u32),
            pltpu.VMEM((NU, NCH, CH * 8, 128), u32),
            pltpu.VMEM((F, D), bf16),
            pltpu.VMEM((F, D), bf16),
            pltpu.VMEM((F, D), bf16),
            pltpu.VMEM((NCH, CH, SEG, D), bf16),
            pltpu.VMEM((80, 80), f32),
            pltpu.VMEM((48, D), f32),
            pltpu.VMEM((48, (H - HL) * DH), f32),
            pltpu.VMEM((NPL, 8, 128), f32),
            pltpu.VMEM((8, D), f32),
            pltpu.VMEM((M, D), bf16),
            pltpu.VMEM((D,), bf16),
            pltpu.SemaphoreType.DMA((len(GROUPS),)),
            pltpu.SemaphoreType.DMA((1,)),
        ],
        compiler_params=pltpu.CompilerParams(
            vmem_limit_bytes=100 * 1024 * 1024,
            disable_bounds_checks=True,
            disable_semaphore_checks=True,
            internal_scratch_in_bytes=48 * 1024,
        ),
        name="rmt_mod",
    )(A_x.reshape(NCH, CH, SEG, D), A_mem0.reshape(M, D), A_Wq, A_Wk, A_Wv, A_Wo.reshape(H * DH, D),
      B_w_r, B_w_gate.T, B_w_up.T, B_w_down)
    return out.reshape(1, S, D)
```

```python
import math

import jax
import jax.numpy as jnp
from jax import lax
import jax.experimental.pallas as pl
import jax.experimental.pallas.tpu as pltpu

bf16 = jnp.bfloat16
f32 = jnp.float32
u32 = jnp.uint32
i32 = jnp.int32

S = 2048
D = 640
H = 32
DH = 128
NP = H // 2
NU = NP * 3
M = 8
SEG = 32
NSEG = S // SEG
F = 1728
C = 8
CH = 4
NCH = NSEG // CH
NJ = D // 128
EPS = 1e-5
NEG = -1e30
LOG2E = math.log2(math.e)
CEXP = (DH ** -0.5) * LOG2E
NT = (((1,), (1,)), ((), ()))

LAG_B, POS_B = 1, 3
LAG_D, POS_D = 3, 6
KMAJ = (5, 5, 4, 5)
MORDS = ((0, 1, 2), (1, 0, 2), (1, 0, 2), (1, 0, 2))
EBS = ((0, 6, 12, 20, 22, 32), (0, 8, 16, 21, 23, 32), (0, 8, 12, 17, 23, 32), (0, 6, 12, 20, 28))
EPOS = ((2, 4), (4, 4), (1, 3), (4, 4))
HL = EBS[CH - 1][-1]

NPL = 4
UPL = 8
U0 = 9
CPL = NCH // NPL
SPL = NSEG // NPL
HEAD_GROUPS = (("p0",), ("w0", "p1"), ("w1", "p2", "p3"), ("w2", "w3", "w4"),
               ("mem0", "wr", "w5", "w6", "w7", "w8"))
HOLD = (0, 0, 0, 2, 2)
LOOP_GROUPS = tuple(
    tuple("w%d" % u for u in range(U0 + i * UPL, U0 + (i + 1) * UPL)) + ("x%d" % i,) for i in range(NPL))
TAIL_GROUPS = (tuple("w%d" % u for u in range(U0 + NPL * UPL, NU)) + ("f0", "f1", "f2"),
               tuple("o%d" % j for j in range(NJ)))
GROUPS = HEAD_GROUPS + LOOP_GROUPS + TAIL_GROUPS
TIE_LAG = 6
LN_NUM, LN_DEN = 6, 7
FFN_SKIP = 14


def _tob(x):
    return pltpu.bitcast(x, bf16)


def _tou(x):
    return pltpu.bitcast(x, u32)


def _zero_of(x):
    return (pltpu.bitcast(x, u32) >> 16) >> 16


def _rb(x):
    return x.astype(bf16).astype(f32)


def _layernorm(x, tie=None):
    ps = x[:, 0:128]
    if tie is not None:
        ps = ps + tie
    for j in range(1, NJ):
        ps = ps + x[:, j * 128:(j + 1) * 128]
    mu = jnp.sum(ps, axis=-1, keepdims=True) * (1.0 / D)
    xc = x - mu
    var = jnp.sum(xc * xc, axis=-1, keepdims=True) * (1.0 / D)
    den = _rb(jnp.sqrt(_rb(_rb(var) + EPS)))
    return (_rb(x - _rb(mu)) * pl.reciprocal(den, approx=False, full_range=False)).astype(bf16)


def _sigmoid(z):
    return pl.reciprocal(1.0 + jnp.exp2(z * (-LOG2E)), approx=True)


def _silu(z):
    return z * _sigmoid(z)


def _dot(a, b):
    return jnp.dot(a, b, preferred_element_type=f32)


def _dot_t(a, b):
    return lax.dot_general(a, b, NT, preferred_element_type=f32)


def _kernel(x_hbm, mem0_hbm, wq_hbm, wk_hbm, wv_hbm, wo_hbm, wr_hbm, wg_hbm, wu_hbm, wd_hbm,
            out_hbm,
            xv, lhs, xpre, zbuf, raw, wqkv, wo, pre, wg, wu, wd, outv, mask_ref,
            accv, ocv, rds, wr8, mem0_v, wr_v, sem, sem_out):
    w32 = [w.bitcast(u32) for w in (wq_hbm, wk_hbm, wv_hbm)]
    wo32 = wo_hbm.bitcast(u32)

    def src_dst(name):
        if name == "mem0":
            return mem0_hbm, mem0_v
        if name == "wr":
            return wr_hbm, wr_v
        k, n = name[0], int(name[1:])
        if k == "x":
            idx = (pl.ds(n * CPL, CPL), slice(None), pl.ds(8, SEG - 8), slice(None))
            return x_hbm.at[idx], xv.at[idx]
        if k == "p":
            idx = (pl.ds(n * 4, 4), slice(None), pl.ds(0, 8), slice(None))
            return x_hbm.at[idx], xv.at[idx]
        if k == "w":
            return w32[n % 3].at[:, n // 3, :], raw.at[n]
        if k == "f":
            return ((wg_hbm, wg), (wu_hbm, wu), (wd_hbm, wd))[n]
        return wo32.at[:, pl.ds(n * 128, 128)], wo.at[n]

    cps = [[pltpu.make_async_copy(*src_dst(nm), sem.at[gi]) for nm in grp]
           for gi, grp in enumerate(GROUPS)]
    for grp in cps:
        for cp in grp:
            cp.start()

    def head_pos(i):
        head = jnp.where(i < 32, 0, jnp.where(i < 64, 1, jnp.where(i < 72, 0, 1)))
        j = i & 31
        pos = jnp.where(i < 64, jnp.where(j < 8, j, j + 8), 8 + (i & 7))
        return head, pos

    hr, pr = head_pos(lax.broadcasted_iota(i32, (80, 80), 0))
    hc, pc = head_pos(lax.broadcasted_iota(i32, (80, 80), 1))
    mask_ref[...] = jnp.where((hr == hc) & ((pr < M) | (pr >= pc)), 1.0, 0.0).astype(f32)

    st = {}
    lane8 = lax.broadcasted_iota(i32, (8, 128), 1)
    sub8 = lax.broadcasted_iota(i32, (8, 128), 0)

    def ln_pre(b):
        xb = xv[b * 4:(b + 1) * 4, :, 0:8, :].astype(f32).reshape(128, D)
        xpre[b] = _tou(_layernorm(xb))

    def repack(u):
        ev = raw[u, pl.ds(0, D // 2, stride=2), :]
        od = raw[u, pl.ds(1, D // 2, stride=2), :]
        ws = ((ev & jnp.uint32(0xFFFF)) | (od << 16), (ev >> 16) | (od & jnp.uint32(0xFFFF0000)))
        wqkv[2 * u] = ws[0]
        wqkv[2 * u + 1] = ws[1]
        return ws

    def pre_dots(u, b, hook, ws=None):
        xu = xpre[b]
        res = []
        for hh in range(2):
            tie = hook()
            xt = xu
            if tie is not None:
                top = jnp.concatenate([xu[0:8, 0:128] ^ tie, xu[0:8, 128:]], axis=1)
                xt = jnp.concatenate([top, xu[8:]], axis=0)
            w = wqkv[2 * u + hh] if ws is None else ws[hh]
            res.append(_dot(_tob(xt), _tob(w)))
            st["after"] = res[-1][0:8]
        parts = []
        for k in range(16):
            parts += [res[0][k * 8:(k + 1) * 8], res[1][k * 8:(k + 1) * 8]]
        pre[u, b * 4:(b + 1) * 4] = _tou(jnp.concatenate(parts, axis=0).astype(bf16)).reshape(4, CH * 8, 128)

    def score(i, gl, xn32):
        zbuf[i * CPL + gl // 16, (gl % 16) * 8:(gl % 16) * 8 + 8, :] = xn32
        rc = jnp.sum(xn32 * st["wr"], axis=-1, keepdims=True)
        st["rd"] = jnp.where(lane8 == gl, rc, st["rd"])

    def ln_group(i, s, k):
        tie = None
        if st["after"] is not None:
            tie = pltpu.bitcast(_zero_of(st["after"]), f32)
        xn = _layernorm(xv[i * CPL + s // CH, s % CH, k * 8:(k + 1) * 8, :].astype(f32), tie)
        score(i, s * 4 + k, xn.astype(f32))
        if k == 1 and s % 2 == 0:
            xp = _tob(xpre[i, s * 4:s * 4 + 8, :]).astype(f32)
            score(i, s * 4, xp[0:8])
            score(i, s * 4 + 4, xp[8:16])
        if k == 2:
            st["xn2"] = xn
        else:
            r0 = (s % CH) * 16 + (k // 2) * 8
            pair = jnp.concatenate([xn if k == 1 else st["xn2"], xn], axis=0)
            lhs[i * CPL + s // CH, r0:r0 + 8, :] = _tou(pair)
        return _zero_of(st["rd"])

    def topk():
        rd = _rb(rds[...].reshape(NPL * 8, 128))
        rd = jnp.where(rd == 0.0, 0.0, rd)
        bits = pltpu.bitcast(rd, i32)
        mono = jnp.where(bits < 0, bits ^ jnp.int32(0x7FFFFFFF), bits)
        rowid = jnp.concatenate([lane8 * 8 + sub8 + i * SPL * SEG for i in range(NPL)], axis=0)
        key = ((((mono >> 16) + 32768) << 11) | (S - 1 - rowid)) | jnp.int32(0x20000000)
        key = jnp.where(jnp.concatenate([lane8] * NPL, axis=0) < SPL * 4, pltpu.bitcast(key, f32), 0.0)
        row8 = lax.broadcasted_iota(i32, (8, 1), 0)
        ksel = jnp.zeros((8, 1), f32)
        for t in range(C):
            km = jnp.max(jnp.max(key, axis=0, keepdims=True), axis=1, keepdims=True)
            key = jnp.where(key == km, 0.0, key)
            ksel = jnp.where(row8 == t, km, ksel)
        ksel = pltpu.bitcast(ksel, i32)
        iv = S - 1 - (ksel & (S - 1))
        idxs = [iv[t, 0] for t in range(C)]
        xs = jnp.concatenate([zbuf[i_ >> 7, pl.ds(i_ & 127, 1), :] for i_ in idxs], axis=0)
        hi16 = (((ksel >> 11) & 65535) - 32768) << 16
        rbits = jnp.where(hi16 < 0, hi16 ^ jnp.int32(0x7FFF0000), hi16)
        return idxs, xs, _rb(_sigmoid(pltpu.bitcast(rbits, f32)))

    def ffn_tasks(idxs, xs, rsel):
        cols = [(k * 128, min(F, (k + 1) * 128)) for k in range(pl.cdiv(F, 128))]
        xsb = xs.astype(bf16)
        hid = []
        tmp = {}

        def gate(a, b):
            tmp["g"] = _rb(_dot_t(xsb, wg[a:b, :]))

        def up(a, b):
            hid.append((_rb(_silu(tmp["g"])) * _rb(_dot_t(xsb, wu[a:b, :]))).astype(bf16))

        def down(k):
            t = _dot(hid[k], wd[cols[k][0]:cols[k][1], :])
            tmp["y"] = t if k == 0 else t + tmp["y"]

        def fin():
            zs = _rb(xs + _rb(_rb(tmp["y"]) * rsel))
            for t in range(C):
                zbuf[idxs[t] >> 7, pl.ds(idxs[t] & 127, 1), :] = zs[t:t + 1]

        tasks = []
        for a, b in cols:
            tasks += [lambda a=a, b=b: gate(a, b), lambda a=a, b=b: up(a, b)]
        tasks += [lambda k=k: down(k) for k in range(len(cols))]
        return tasks + [fin]

    def run_region(work, side=(), tasks=(), skip=0):
        side, tasks = list(side), list(tasks)
        ties = []
        st["after"] = None
        cnt = {"dot": 0, "credit": 0}

        def hook():
            di = cnt["dot"]
            cnt["dot"] += 1
            if tasks and di >= skip:
                tasks.pop(0)()
            tie = None
            if ties and ties[0][0] <= di:
                tie = ties.pop(0)[1]
            if side and di + TIE_LAG < 2 * len(work):
                cnt["credit"] += LN_NUM
                if cnt["credit"] >= LN_DEN:
                    cnt["credit"] -= LN_DEN
                    ties.append((di + TIE_LAG, ln_group(*side.pop(0))))
            return tie

        for u, b, *ws in work:
            pre_dots(u, b, hook, *ws)
        assert not ties and not side and not tasks

    pending = []
    units, blocks = [], []
    for gi, grp in enumerate(HEAD_GROUPS):
        for cp in cps[gi]:
            cp.wait()
        for u in [int(nm[1:]) for nm in grp if nm[0] == "w" and nm != "wr"]:
            repack(u)
            pending += [(u, b) for b in blocks]
            units.append(u)
        for b in [int(nm[1:]) for nm in grp if nm[0] == "p"]:
            ln_pre(b)
            pending += [(u, b) for u in units]
            blocks.append(b)
        if "mem0" in grp:
            accv[...] = jnp.concatenate([mem0_v[...].astype(f32), jnp.zeros((40, D), f32)], axis=0)
            ocv[...] = jnp.zeros(ocv.shape, f32)
            wr8[...] = jnp.broadcast_to(wr_v[...].astype(f32).reshape(1, D), (8, D))
        n = len(pending) - HOLD[gi]
        work, pending = pending[:n], pending[n:]
        run_region(work)
    assert pending == [(U0 - 1, 2), (U0 - 1, 3)]

    def pro_body(i, carry):
        ub = U0 + i * UPL
        for k in range(UPL):
            pltpu.make_async_copy(w32[0].at[:, 0, :], raw.at[ub + k], sem.at[len(HEAD_GROUPS) + i]).wait()
        idx = (pl.ds(i * CPL, CPL), slice(None), pl.ds(8, SEG - 8), slice(None))
        pltpu.make_async_copy(x_hbm.at[idx], xv.at[idx], sem.at[len(HEAD_GROUPS) + i]).wait()
        ws = [None] + [repack(ub + k) for k in range(UPL)]
        work = [(ub - 1 + k // 4, k % 4, ws[k // 4]) for k in range(2, 2 + 4 * UPL)]
        st["wr"] = wr8[...]
        st["rd"] = jnp.zeros((8, 128), f32)
        run_region(work, side=[(i, s, k) for s in range(SPL) for k in (1, 2, 3)])
        rds[i] = st["rd"]
        return carry

    lax.fori_loop(0, NPL, pro_body, 0)

    for cp in cps[-2]:
        cp.wait()
    ub = U0 + NPL * UPL
    for u in range(ub, NU):
        repack(u)
    run_region([(ub - 1 + k // 4, k % 4) for k in range(2, 4 + 4 * (NU - ub))],
               tasks=ffn_tasks(*topk()), skip=FFN_SKIP)
    for cp in cps[-1]:
        cp.wait()

    sub4 = lax.broadcasted_iota(i32, (8, D), 0) < 4
    ost = {}

    def finalize(ci, sl, r0, r1, sv, c0=0, c1=D):
        xr = xv[ci, sl, r0:r1, c0:c1].astype(f32)
        g = _silu(zbuf[ci, sl * SEG + r0:sl * SEG + r1, c0:c1])
        outv[ci, sl, r0:r1, c0:c1] = (xr + sv * g).astype(bf16)

    def finish(ci, sl, acc):
        acc = jnp.concatenate(acc, axis=1)
        finalize(ci, sl, 8, SEG, acc[8:32])
        if sl % 2 == 1:
            finalize(ci, sl, 0, 8, acc[32:40])
            finalize(ci, sl - 1, 0, 8, acc[40:48])
        return _tou(acc[0:16].astype(bf16))

    def finish_last(ci):
        o2 = ocv[...].astype(bf16)
        acc = [_dot(o2, _tob(wo[j, HL * 64:, :])) + accv[:, j * 128:(j + 1) * 128] for j in range(NJ)]
        return finish(ci, CH - 1, acc)

    def step(ci, sl, mem):
        xu = lhs[ci, sl * 16:(sl + 1) * 16, :]
        x = _tob(jnp.concatenate([jnp.where(sub4, mem, xu[0:8]), xu[8:16]], axis=0))
        mord, eb = MORDS[sl], EBS[sl]
        sd = {}
        oc = {}

        early = {}
        for k in range(NJ):
            for d in range(KMAJ[sl]):
                key = (d // 6, mord[(d % 6) // 2], d % 2)
                w = _tob(wqkv[2 * (key[0] * 3 + key[1]) + key[2], k * 64:(k + 1) * 64, :])
                t = _dot(x[:, k * 128:(k + 1) * 128], w)
                early[key] = t if k == 0 else t + early[key]

        def project(p, m, hh):
            u = p * 3 + m
            outs = sd.setdefault(p, [None, None, None])
            r = early[p, m, hh] if (p, m, hh) in early else _dot(x, _tob(wqkv[2 * u + hh]))
            if hh == 0:
                outs[m] = r
            else:
                pb = _tob(pre[u, ci, sl * 8:(sl + 1) * 8, :]).astype(f32)
                outs[m] = jnp.concatenate([outs[m], r, pb], axis=0).astype(bf16)

        def scores(p):
            if not 0 <= p < NP:
                return
            sc = jnp.where(mask_ref[...] > 0.5, _dot_t(sd[p][0], sd[p][1]), NEG)
            e = jnp.exp2((sc - jnp.max(sc, axis=-1, keepdims=True)) * CEXP)
            l = jnp.sum(e, axis=-1, keepdims=True)
            sd[p][0] = (e * pl.reciprocal(l, approx=True)).astype(bf16)

        def attend(p):
            if not 0 <= p < NP:
                return
            o = _dot(sd[p][0], sd[p][2])
            for hh in range(2):
                rows = [o[hh * 32:(hh + 1) * 32]]
                first = o[64 + hh * 8:72 + hh * 8]
                if sl % 2 == 0:
                    ost[2 * p + hh] = first
                else:
                    rows += [first, ost[2 * p + hh]]
                oc[2 * p + hh] = jnp.concatenate(rows, axis=0)

        for slot in range(NP):
            for di in range(7):
                if di == POS_B:
                    scores(slot - LAG_B)
                if di == POS_D:
                    attend(slot - LAG_D)
                if di < 6:
                    project(slot, mord[di // 2], di % 2)
        acc = [None] * NJ
        for i in range(len(eb) - 1):
            h0, h1 = eb[i], eb[i + 1]
            o2 = jnp.concatenate([oc[h] for h in range(h0, h1)], axis=1).astype(bf16)
            for j in range(NJ):
                t = _dot(o2, _tob(wo[j, h0 * 64:h1 * 64, :]))
                acc[j] = t if acc[j] is None else t + acc[j]
                if j == EPOS[sl][0]:
                    scores(NP + i - LAG_B)
                if j == EPOS[sl][1]:
                    attend(NP + i - LAG_D)
        if sl == CH - 1:
            accv[...] = jnp.concatenate(acc, axis=1)
            ocv[...] = jnp.concatenate([oc[h] for h in range(HL, H)], axis=1)
            return None
        return finish(ci, sl, acc)

    def out_cp(*idx):
        return pltpu.make_async_copy(outv.at[idx], out_hbm.at[idx], sem_out.at[0])

    def chunk(ci, carry):
        prev = jnp.maximum(ci - 1, 0)
        mem = finish_last(prev)

        @pl.when(ci >= 1)
        def _():
            out_cp(prev, pl.ds(2, 2)).start()

        for sl in range(CH):
            mem = step(ci, sl, mem)
            if sl == 1:
                out_cp(ci, pl.ds(0, 2)).start()
        return carry

    lax.fori_loop(0, NCH, chunk, 0)
    o2 = ocv[...].astype(bf16)
    for j in range(NJ):
        c0, c1 = j * 128, (j + 1) * 128
        t = _dot(o2, _tob(wo[j, HL * 64:, :])) + accv[:, c0:c1]
        finalize(NCH - 1, CH - 1, 8, SEG, t[8:32], c0, c1)
        finalize(NCH - 1, CH - 1, 0, 8, t[32:40], c0, c1)
        finalize(NCH - 1, CH - 2, 0, 8, t[40:48], c0, c1)
        out_cp(NCH - 1, pl.ds(2, 2), slice(None), pl.ds(c0, 128)).start()
    pltpu.make_async_copy(outv, out_hbm, sem_out.at[0]).wait()


@jax.jit
def pallas_recurrent_scan__memory_aug_recurrent_mem_tr__moe_arch_mod__prompt_kernel(
    A_x, A_mem0, A_Wq, A_Wk, A_Wv, A_Wo, A_seg_len, B_x, B_w_r, B_w_gate, B_w_up, B_w_down,
):
    hbm = pl.BlockSpec(memory_space=pltpu.MemorySpace.HBM)
    out = pl.pallas_call(
        _kernel,
        out_shape=jax.ShapeDtypeStruct((NCH, CH, SEG, D), bf16),
        in_specs=[hbm] * 10,
        out_specs=hbm,
        scratch_shapes=[
            pltpu.VMEM((NCH, CH, SEG, D), bf16),
            pltpu.VMEM((NCH, CH * 16, D), u32),
            pltpu.VMEM((4, 64, D), u32),
            pltpu.VMEM((NCH, CH * SEG, D), f32),
            pltpu.VMEM((NU, D, 128), u32),
            pltpu.VMEM((NU * 2, D // 2, 128), u32),
            pltpu.VMEM((NJ, H * DH // 2, 128), u32),
            pltpu.VMEM((NU, NCH, CH * 8, 128), u32),
            pltpu.VMEM((F, D), bf16),
            pltpu.VMEM((F, D), bf16),
            pltpu.VMEM((F, D), bf16),
            pltpu.VMEM((NCH, CH, SEG, D), bf16),
            pltpu.VMEM((80, 80), f32),
            pltpu.VMEM((48, D), f32),
            pltpu.VMEM((48, (H - HL) * DH), f32),
            pltpu.VMEM((NPL, 8, 128), f32),
            pltpu.VMEM((8, D), f32),
            pltpu.VMEM((M, D), bf16),
            pltpu.VMEM((D,), bf16),
            pltpu.SemaphoreType.DMA((len(GROUPS),)),
            pltpu.SemaphoreType.DMA((1,)),
        ],
        compiler_params=pltpu.CompilerParams(
            vmem_limit_bytes=100 * 1024 * 1024,
            disable_bounds_checks=True,
            disable_semaphore_checks=True,
            internal_scratch_in_bytes=48 * 1024,
        ),
        name="rmt_mod",
    )(A_x.reshape(NCH, CH, SEG, D), A_mem0.reshape(M, D), A_Wq, A_Wk, A_Wv, A_Wo.reshape(H * DH, D),
      B_w_r, B_w_gate.T, B_w_up.T, B_w_down)
    return out.reshape(1, S, D)
```

```python
import math

import jax
import jax.numpy as jnp
from jax import lax
import jax.experimental.pallas as pl
import jax.experimental.pallas.tpu as pltpu

bf16 = jnp.bfloat16
f32 = jnp.float32
u32 = jnp.uint32
i32 = jnp.int32

S = 2048
D = 640
H = 32
DH = 128
NP = H // 2
NU = NP * 3
M = 8
SEG = 32
NSEG = S // SEG
F = 1728
C = 8
CH = 4
NCH = NSEG // CH
NJ = D // 128
EPS = 1e-5
NEG = -1e30
LOG2E = math.log2(math.e)
CEXP = (DH ** -0.5) * LOG2E
NT = (((1,), (1,)), ((), ()))

LAG_B, POS_B = 1, 6
LAG_D, POS_D = 3, 4
POS_B0 = (6, 6, 5, 5)
KMAJ = (6, 4, 4, 5)
MORDS = ((1, 0, 2), (1, 0, 2), (0, 1, 2), (1, 0, 2))
EBS = ((0, 6, 12, 20, 22, 32), (0, 9, 14, 18, 22, 27, 32), (0, 8, 14, 17, 23, 32), (0, 8, 14, 19, 25, 28))
EPOS = ((3, 4), (2, 3), (1, 3), (4, 2))
HL = EBS[CH - 1][-1]
NV2 = (8, 2)
VGB = ((0, 5, 11, 16), (0, 5, 11, 17, 24))
LAG_V = 11
TIE_KT = (3, 0, 0, 0, 0, 3)
TIE_W, TIE_E = 2, 3
E_RATE, E_SKIP = 0.6, 4
OO, FO = 192, 224

NPL = 4
UPL = 8
U0 = 9
CPL = NCH // NPL
SPL = NSEG // NPL
HEAD_GROUPS = (("p0",), ("w0", "p1"), ("w1", "p2", "p3"), ("w2", "w3", "w4"),
               ("mem0", "wr", "w5", "w6", "w7", "w8"))
HOLD = (0, 0, 0, 2, 2)
LOOP_GROUPS = tuple(
    tuple("w%d" % u for u in range(U0 + i * UPL, U0 + (i + 1) * UPL)) + ("x%d" % i,) for i in range(NPL))
TAIL_GROUPS = (tuple("w%d" % u for u in range(U0 + NPL * UPL, NU)) + ("f0", "f1", "f2"),
               tuple("o%d" % j for j in range(NJ)))
GROUPS = HEAD_GROUPS + LOOP_GROUPS + TAIL_GROUPS
TIE_LAG = 6
LN_NUM, LN_DEN = 6, 7
FFN_SKIP = 14


def _tob(x):
    return pltpu.bitcast(x, bf16)


def _tou(x):
    return pltpu.bitcast(x, u32)


def _zero_of(x):
    return (pltpu.bitcast(x, u32) >> 16) >> 16


def _rb(x):
    return x.astype(bf16).astype(f32)


def _layernorm(x, tie=None):
    ps = x[:, 0:128]
    if tie is not None:
        ps = ps + tie
    for j in range(1, NJ):
        ps = ps + x[:, j * 128:(j + 1) * 128]
    mu = jnp.sum(ps, axis=-1, keepdims=True) * (1.0 / D)
    xc = x - mu
    var = jnp.sum(xc * xc, axis=-1, keepdims=True) * (1.0 / D)
    den = _rb(jnp.sqrt(_rb(_rb(var) + EPS)))
    return (_rb(x - _rb(mu)) * pl.reciprocal(den, approx=False, full_range=False)).astype(bf16)


def _sigmoid(z):
    return pl.reciprocal(1.0 + jnp.exp2(z * (-LOG2E)), approx=True)


def _silu(z):
    return z * _sigmoid(z)


def _dot(a, b):
    return jnp.dot(a, b, preferred_element_type=f32)


def _dot_t(a, b):
    return lax.dot_general(a, b, NT, preferred_element_type=f32)


def _kernel(x_hbm, mem0_hbm, wq_hbm, wk_hbm, wv_hbm, wo_hbm, wr_hbm, wg_hbm, wu_hbm, wd_hbm,
            out_hbm,
            xv, lhs, xpre, zbuf, raw, wqkv, wo, pre, stg, sst, wg, wu, wd, outv, mask_ref,
            accv, ocv, rds, wr8, mem0_v, wr_v, sem, sem_out):
    w32 = [w.bitcast(u32) for w in (wq_hbm, wk_hbm, wv_hbm)]
    wo32 = wo_hbm.bitcast(u32)

    def src_dst(name):
        if name == "mem0":
            return mem0_hbm, mem0_v
        if name == "wr":
            return wr_hbm, wr_v
        k, n = name[0], int(name[1:])
        if k == "x":
            idx = (pl.ds(n * CPL, CPL), slice(None), pl.ds(8, SEG - 8), slice(None))
            return x_hbm.at[idx], xv.at[idx]
        if k == "p":
            idx = (pl.ds(n * 4, 4), slice(None), pl.ds(0, 8), slice(None))
            return x_hbm.at[idx], xv.at[idx]
        if k == "w":
            return w32[n % 3].at[:, n // 3, :], raw.at[n]
        if k == "f":
            return ((wg_hbm, wg), (wu_hbm, wu), (wd_hbm, wd))[n]
        return wo32.at[:, pl.ds(n * 128, 128)], wo.at[n]

    cps = [[pltpu.make_async_copy(*src_dst(nm), sem.at[gi]) for nm in grp]
           for gi, grp in enumerate(GROUPS)]
    for grp in cps:
        for cp in grp:
            cp.start()

    def head_pos(i):
        head = jnp.where(i < 32, 0, jnp.where(i < 64, 1, jnp.where(i < 72, 0, 1)))
        j = i & 31
        pos = jnp.where(i < 64, jnp.where(j < 8, j, j + 8), 8 + (i & 7))
        return head, pos

    hr, pr = head_pos(lax.broadcasted_iota(i32, (64, 80), 0))
    hc, pc = head_pos(lax.broadcasted_iota(i32, (64, 80), 1))
    mask_ref[...] = jnp.where((hr == hc) & ((pr < M) | (pr >= pc)), 1.0, 0.0).astype(f32)

    st = {}
    lane8 = lax.broadcasted_iota(i32, (8, 128), 1)
    sub8 = lax.broadcasted_iota(i32, (8, 128), 0)

    def ln_pre(b):
        xb = xv[b * 4:(b + 1) * 4, :, 0:8, :].astype(f32).reshape(128, D)
        xpre[b] = _tou(_layernorm(xb))

    def repack(u):
        ev = raw[u, pl.ds(0, D // 2, stride=2), :]
        od = raw[u, pl.ds(1, D // 2, stride=2), :]
        ws = ((ev & jnp.uint32(0xFFFF)) | (od << 16), (ev >> 16) | (od & jnp.uint32(0xFFFF0000)))
        wqkv[2 * u] = ws[0]
        wqkv[2 * u + 1] = ws[1]
        return ws

    def pre_dots(u, b, hook, ws=None):
        xu = xpre[b]
        res = []
        for hh in range(2):
            tie = hook()
            xt = xu
            if tie is not None:
                top = jnp.concatenate([xu[0:8, 0:128] ^ tie, xu[0:8, 128:]], axis=1)
                xt = jnp.concatenate([top, xu[8:]], axis=0)
            w = wqkv[2 * u + hh] if ws is None else ws[hh]
            res.append(_dot(_tob(xt), _tob(w)))
            st["after"] = res[-1][0:8]
        parts = []
        for k in range(16):
            parts += [res[0][k * 8:(k + 1) * 8], res[1][k * 8:(k + 1) * 8]]
        pre[u, b * 4:(b + 1) * 4] = jnp.concatenate(parts, axis=0).reshape(4, CH * 16, 128)

    def score(i, gl, xn32):
        zbuf[i * CPL + gl // 16, (gl % 16) * 8:(gl % 16) * 8 + 8, :] = xn32
        rc = jnp.sum(xn32 * st["wr"], axis=-1, keepdims=True)
        st["rd"] = jnp.where(lane8 == gl, rc, st["rd"])

    def ln_group(i, s, k):
        tie = None
        if st["after"] is not None:
            tie = pltpu.bitcast(_zero_of(st["after"]), f32)
        xn = _layernorm(xv[i * CPL + s // CH, s % CH, k * 8:(k + 1) * 8, :].astype(f32), tie)
        score(i, s * 4 + k, xn.astype(f32))
        if k == 1 and s % 2 == 0:
            xp = _tob(xpre[i, s * 4:s * 4 + 8, :]).astype(f32)
            score(i, s * 4, xp[0:8])
            score(i, s * 4 + 4, xp[8:16])
        if k == 2:
            st["xn2"] = xn
        else:
            r0 = (s % CH) * 16 + (k // 2) * 8
            pair = jnp.concatenate([xn if k == 1 else st["xn2"], xn], axis=0)
            lhs[i * CPL + s // CH, r0:r0 + 8, :] = _tou(pair)
        return _zero_of(st["rd"])

    def topk():
        rd = _rb(rds[...].reshape(NPL * 8, 128))
        rd = jnp.where(rd == 0.0, 0.0, rd)
        bits = pltpu.bitcast(rd, i32)
        mono = jnp.where(bits < 0, bits ^ jnp.int32(0x7FFFFFFF), bits)
        rowid = jnp.concatenate([lane8 * 8 + sub8 + i * SPL * SEG for i in range(NPL)], axis=0)
        key = ((((mono >> 16) + 32768) << 11) | (S - 1 - rowid)) | jnp.int32(0x20000000)
        key = jnp.where(jnp.concatenate([lane8] * NPL, axis=0) < SPL * 4, pltpu.bitcast(key, f32), 0.0)
        row8 = lax.broadcasted_iota(i32, (8, 1), 0)
        ksel = jnp.zeros((8, 1), f32)
        for t in range(C):
            km = jnp.max(jnp.max(key, axis=0, keepdims=True), axis=1, keepdims=True)
            key = jnp.where(key == km, 0.0, key)
            ksel = jnp.where(row8 == t, km, ksel)
        ksel = pltpu.bitcast(ksel, i32)
        iv = S - 1 - (ksel & (S - 1))
        idxs = [iv[t, 0] for t in range(C)]
        xs = jnp.concatenate([zbuf[i_ >> 7, pl.ds(i_ & 127, 1), :] for i_ in idxs], axis=0)
        hi16 = (((ksel >> 11) & 65535) - 32768) << 16
        rbits = jnp.where(hi16 < 0, hi16 ^ jnp.int32(0x7FFF0000), hi16)
        return idxs, xs, _rb(_sigmoid(pltpu.bitcast(rbits, f32)))

    def ffn_tasks(idxs, xs, rsel):
        cols = [(k * 128, min(F, (k + 1) * 128)) for k in range(pl.cdiv(F, 128))]
        xsb = xs.astype(bf16)
        hid = []
        tmp = {}

        def gate(a, b):
            tmp["g"] = _rb(_dot_t(xsb, wg[a:b, :]))

        def up(a, b):
            hid.append((_rb(_silu(tmp["g"])) * _rb(_dot_t(xsb, wu[a:b, :]))).astype(bf16))

        def down(k):
            t = _dot(hid[k], wd[cols[k][0]:cols[k][1], :])
            tmp["y"] = t if k == 0 else t + tmp["y"]

        def fin():
            zs = _rb(xs + _rb(_rb(tmp["y"]) * rsel))
            for t in range(C):
                zbuf[idxs[t] >> 7, pl.ds(idxs[t] & 127, 1), :] = zs[t:t + 1]

        tasks = []
        for a, b in cols:
            tasks += [lambda a=a, b=b: gate(a, b), lambda a=a, b=b: up(a, b)]
        tasks += [lambda k=k: down(k) for k in range(len(cols))]
        return tasks + [fin]

    def run_region(work, side=(), tasks=(), skip=0):
        side, tasks = list(side), list(tasks)
        ties = []
        st["after"] = None
        cnt = {"dot": 0, "credit": 0}

        def hook():
            di = cnt["dot"]
            cnt["dot"] += 1
            if tasks and di >= skip:
                tasks.pop(0)()
            tie = None
            if ties and ties[0][0] <= di:
                tie = ties.pop(0)[1]
            if side and di + TIE_LAG < 2 * len(work):
                cnt["credit"] += LN_NUM
                if cnt["credit"] >= LN_DEN:
                    cnt["credit"] -= LN_DEN
                    ties.append((di + TIE_LAG, ln_group(*side.pop(0))))
            return tie

        for u, b, *ws in work:
            pre_dots(u, b, hook, *ws)
        assert not ties and not side and not tasks

    pending = []
    units, blocks = [], []
    for gi, grp in enumerate(HEAD_GROUPS):
        for cp in cps[gi]:
            cp.wait()
        for u in [int(nm[1:]) for nm in grp if nm[0] == "w" and nm != "wr"]:
            repack(u)
            pending += [(u, b) for b in blocks]
            units.append(u)
        for b in [int(nm[1:]) for nm in grp if nm[0] == "p"]:
            ln_pre(b)
            pending += [(u, b) for u in units]
            blocks.append(b)
        if "mem0" in grp:
            accv[...] = jnp.concatenate([mem0_v[...].astype(f32), jnp.zeros((40, D), f32)], axis=0)
            ocv[...] = jnp.zeros(ocv.shape, f32)
            wr8[:, 0:D] = jnp.broadcast_to(wr_v[...].astype(f32).reshape(1, D), (8, D))
        n = len(pending) - HOLD[gi]
        work, pending = pending[:n], pending[n:]
        run_region(work)
    assert pending == [(U0 - 1, 2), (U0 - 1, 3)]

    def pro_body(i, carry):
        ub = U0 + i * UPL
        for k in range(UPL):
            pltpu.make_async_copy(w32[0].at[:, 0, :], raw.at[ub + k], sem.at[len(HEAD_GROUPS) + i]).wait()
        idx = (pl.ds(i * CPL, CPL), slice(None), pl.ds(8, SEG - 8), slice(None))
        pltpu.make_async_copy(x_hbm.at[idx], xv.at[idx], sem.at[len(HEAD_GROUPS) + i]).wait()
        ws = [None] + [repack(ub + k) for k in range(UPL)]
        work = [(ub - 1 + k // 4, k % 4, ws[k // 4]) for k in range(2, 2 + 4 * UPL)]
        st["wr"] = wr8[:, 0:D]
        st["rd"] = jnp.zeros((8, 128), f32)
        run_region(work, side=[(i, s, k) for s in range(SPL) for k in (1, 2, 3)])
        rds[i] = st["rd"]
        return carry

    lax.fori_loop(0, NPL, pro_body, 0)

    for cp in cps[-2]:
        cp.wait()
    ub = U0 + NPL * UPL
    for u in range(ub, NU):
        repack(u)
    run_region([(ub - 1 + k // 4, k % 4) for k in range(2, 4 + 4 * (NU - ub))],
               tasks=ffn_tasks(*topk()), skip=FFN_SKIP)
    for cp in cps[-1]:
        cp.wait()

    sub4 = lax.broadcasted_iota(i32, (8, D), 0) < 4

    def finalize(ci, sl, r0, r1, sv, c0=0, c1=D):
        xr = xv[ci, sl, r0:r1, c0:c1].astype(f32)
        g = _silu(zbuf[ci, sl * SEG + r0:sl * SEG + r1, c0:c1])
        outv[ci, sl, r0:r1, c0:c1] = (xr + sv * g).astype(bf16)

    def finish(ci, sl, acc):
        acc = jnp.concatenate(acc, axis=1)
        finalize(ci, sl, 8, SEG, acc[8:32])
        if sl % 2 == 1:
            finalize(ci, sl, 0, 8, acc[32:40])
            finalize(ci, sl - 1, 0, 8, acc[40:48])
        return _tou(acc[0:16].astype(bf16))

    def finish_last(ci):
        o2 = ocv[...].astype(bf16)
        acc = [_dot(o2, _tob(wo[j, HL * 64:, :])) + accv[:, j * 128:(j + 1) * 128] for j in range(NJ)]
        return finish(ci, CH - 1, acc)

    vq = []
    clock = [0]

    def vnext():
        ready = [i for i, t in enumerate(vq) if t[0] <= clock[0]]
        if not ready:
            return None
        return vq.pop(min(ready, key=lambda i: (vq[i][2], i)))[1]()

    def vforce(deadline):
        for t in [t for t in vq if t[2] <= deadline]:
            vq.remove(t)
            t[1]()

    def tied(w, g):
        tie = vnext()
        if tie is None:
            return w
        return jnp.concatenate([w[0:g * 8], w[g * 8:g * 8 + 8] ^ tie, w[g * 8 + 8:]], axis=0)

    def step(ci, sl, mem):
        xu = lhs[ci, sl * 16:(sl + 1) * 16, :]
        x = _tob(jnp.concatenate([jnp.where(sub4, mem, xu[0:8]), xu[8:16]], axis=0))
        mord, eb, odd = MORDS[sl], EBS[sl], sl % 2
        probs = {}
        vs = {}

        early = {}
        for k in range(NJ):
            clock[0] += 1
            for d in range(KMAJ[sl]):
                key = (d // 6, mord[(d % 6) // 2], d % 2)
                w = wqkv[2 * (key[0] * 3 + key[1]) + key[2], k * 64:(k + 1) * 64, :]
                if d == 0 and odd:
                    w = tied(w, TIE_W)
                t = _dot(x[:, k * 128:(k + 1) * 128], _tob(w))
                early[key] = t if k == 0 else t + early[key]

        def slot_of(p, m, hh):
            return ((odd * NP + p) * 3 + m) * 2 + hh

        def project(p, di):
            m, hh = mord[di // 2], di % 2
            if (p, m, hh) in early:
                r = early[p, m, hh]
            else:
                clock[0] += 1
                r = _dot(x, _tob(tied(wqkv[2 * (p * 3 + m) + hh], TIE_KT[di] * 8 + TIE_W)))
            stg[slot_of(p, m, hh)] = r

        def mxu_rows(p, a):
            if p < NV2[odd]:
                return jnp.concatenate([a[0:8], a[32:40], a[16:32], a[48:64]], axis=0)
            return a

        def operand(p, m):
            a = jnp.concatenate([stg[slot_of(p, m, hh)] for hh in range(2)], axis=0)
            if m == 0:
                return mxu_rows(p, a).astype(bf16)
            return jnp.concatenate([a, pre[p * 3 + m, ci, sl * 16:(sl + 1) * 16, :]], axis=0).astype(bf16)

        def vpu_rows(p, hh, lv, g):
            gb = VGB[lv]
            r0 = sl * 16 + hh * 8

            def row(m, i):
                if 8 <= i < 16:
                    return pre[p * 3 + m, ci, pl.ds(r0 + i - 8, 8, stride=0), :]
                return stg[slot_of(p, m, hh), pl.ds(i if i < 8 else i - 8, 8, stride=0), :]

            if g == 0:
                q = pre[p * 3, ci, r0:r0 + 8, :] if lv == 0 else stg[slot_of(p, 0, hh), 8:16, :]
                vs[p, hh, lv] = (q * CEXP, None, None, None)
            q, m_old, l, o = vs[p, hh, lv]
            ss = []
            for i in range(gb[g], gb[g + 1]):
                s = jnp.sum(q * row(1, i), axis=-1, keepdims=True)
                if i > 8 + 8 * lv:
                    s = jnp.where(sub8[:, 0:1] >= i - 8 - 8 * lv, s, NEG)
                ss.append(s)
            mx = ss[0] if m_old is None else jnp.maximum(m_old, ss[0])
            for s in ss[1:]:
                mx = jnp.maximum(mx, s)
            if m_old is not None:
                alpha = jnp.exp2(m_old - mx)
                l, o = l * alpha, o * alpha
            for i, s in enumerate(ss):
                e = jnp.exp2(s - mx)
                ev = e * row(2, gb[g] + i)
                l, o = (e, ev) if l is None else (l + e, o + ev)
            if g == len(gb) - 2:
                o = o * pl.reciprocal(l, approx=True)
                if lv == 0:
                    stg[FO + 2 * p + hh, (1 - odd) * 8:(2 - odd) * 8, :] = o
                else:
                    stg[OO + 2 * p + hh, 8:16, :] = o
            vs[p, hh, lv] = (q, mx, l, o)
            return _zero_of(o)

        def scores(p):
            if not 0 <= p < NP:
                return
            sc = jnp.where(mxu_rows(p, mask_ref[...]) > 0.5, _dot_t(operand(p, 0), operand(p, 1)), NEG)
            n = sc.shape[0]
            mx = jnp.max(sc, axis=-1, keepdims=True)
            sst[p % 2, 0:n] = sc
            e = jnp.exp2((sst[p % 2, 0:n] - mx) * CEXP)
            l = jnp.sum(e, axis=-1, keepdims=True)
            sst[2 + p % 2, 0:n] = e
            probs[p] = (sst[2 + p % 2, 0:n] * pl.reciprocal(l, approx=True)).astype(bf16)

        def attend(p):
            if not 0 <= p < NP:
                return
            o = _dot(probs[p], operand(p, 2))
            for hh in range(2):
                if p < NV2[odd]:
                    stg[OO + 2 * p + hh, 0:8, :] = o[hh * 8:hh * 8 + 8]
                    stg[OO + 2 * p + hh, 16:32, :] = o[16 + hh * 16:32 + hh * 16]
                else:
                    stg[OO + 2 * p + hh] = o[hh * 32:(hh + 1) * 32]

        def oheads(h0, h1):
            vforce((sl, h1 - 1))
            if not odd:
                return jnp.concatenate([stg[OO + h] for h in range(h0, h1)], axis=1)
            return jnp.concatenate([jnp.concatenate([stg[OO + h], stg[FO + h, 0:16, :]], axis=0)
                                    for h in range(h0, h1)], axis=1)

        for slot in range(NP):
            for di in range(7):
                if di == (POS_B0[sl] if slot == LAG_B else POS_B):
                    scores(slot - LAG_B)
                if di == POS_D:
                    attend(slot - LAG_D)
                if di < 6:
                    project(slot, di)
            for hh in range(2):
                for lv in ((1, 0) if slot < NV2[odd] else (0,)):
                    for g in range(len(VGB[lv]) - 1):
                        vq.append((clock[0] + LAG_V, lambda a=(slot, hh, lv, g): vpu_rows(*a),
                                   (sl if lv == 1 else sl | 1, 2 * slot + hh)))
        tiles, credit = 0, 0.0
        acc = [None] * NJ
        for i in range(len(eb) - 1):
            h0, h1 = eb[i], eb[i + 1]
            o2 = oheads(h0, h1).astype(bf16)
            for j in range(NJ):
                ws = []
                for h in range(h0, h1):
                    tiles += 1
                    if tiles % (3 if odd else 5) == 0:
                        clock[0] += 1
                    w = wo[j, h * 64:(h + 1) * 64, :]
                    if odd and tiles > E_SKIP:
                        credit += E_RATE
                        if credit >= 1.0:
                            credit -= 1.0
                            w = tied(w, TIE_E)
                    ws.append(w)
                t = _dot(o2, _tob(jnp.concatenate(ws, axis=0)))
                acc[j] = t if acc[j] is None else t + acc[j]
                if j == EPOS[sl][0]:
                    scores(NP + i - LAG_B)
                if j == EPOS[sl][1]:
                    attend(NP + i - LAG_D)
        if sl == CH - 1:
            accv[...] = jnp.concatenate(acc, axis=1)
            ocv[...] = oheads(HL, H)
            assert not vq
            return None
        return finish(ci, sl, acc)

    def out_cp(*idx):
        return pltpu.make_async_copy(outv.at[idx], out_hbm.at[idx], sem_out.at[0])

    def chunk(ci, carry):
        prev = jnp.maximum(ci - 1, 0)
        mem = finish_last(prev)

        @pl.when(ci >= 1)
        def _():
            out_cp(prev, pl.ds(2, 2)).start()

        for sl in range(CH):
            mem = step(ci, sl, mem)
            if sl == 1:
                out_cp(ci, pl.ds(0, 2)).start()
        return carry

    lax.fori_loop(0, NCH, chunk, 0)
    o2 = ocv[...].astype(bf16)
    for j in range(NJ):
        c0, c1 = j * 128, (j + 1) * 128
        t = _dot(o2, _tob(wo[j, HL * 64:, :])) + accv[:, c0:c1]
        finalize(NCH - 1, CH - 1, 8, SEG, t[8:32], c0, c1)
        finalize(NCH - 1, CH - 1, 0, 8, t[32:40], c0, c1)
        finalize(NCH - 1, CH - 2, 0, 8, t[40:48], c0, c1)
        out_cp(NCH - 1, pl.ds(2, 2), slice(None), pl.ds(c0, 128)).start()
    pltpu.make_async_copy(outv, out_hbm, sem_out.at[0]).wait()


@jax.jit
def pallas_recurrent_scan__memory_aug_recurrent_mem_tr__moe_arch_mod__prompt_kernel(
    A_x, A_mem0, A_Wq, A_Wk, A_Wv, A_Wo, A_seg_len, B_x, B_w_r, B_w_gate, B_w_up, B_w_down,
):
    hbm = pl.BlockSpec(memory_space=pltpu.MemorySpace.HBM)
    out = pl.pallas_call(
        _kernel,
        out_shape=jax.ShapeDtypeStruct((NCH, CH, SEG, D), bf16),
        in_specs=[hbm] * 10,
        out_specs=hbm,
        scratch_shapes=[
            pltpu.VMEM((NCH, CH, SEG, D), bf16),
            pltpu.VMEM((NCH, CH * 16, D), u32),
            pltpu.VMEM((4, 64, D), u32),
            pltpu.VMEM((NCH, CH * SEG, D), f32),
            pltpu.VMEM((NU, D, 128), u32),
            pltpu.VMEM((NU * 2, D // 2, 128), u32),
            pltpu.VMEM((NJ, H * DH // 2, 128), u32),
            pltpu.VMEM((NU, NCH, CH * 16, 128), f32),
            pltpu.VMEM((256, 32, 128), f32),
            pltpu.VMEM((4, 64, 80), f32),
            pltpu.VMEM((F, D), bf16),
            pltpu.VMEM((F, D), bf16),
            pltpu.VMEM((F, D), bf16),
            pltpu.VMEM((NCH, CH, SEG, D), bf16),
            pltpu.VMEM((64, 80), f32),
            pltpu.VMEM((48, D), f32),
            pltpu.VMEM((48, (H - HL) * DH), f32),
            pltpu.VMEM((NPL, 8, 128), f32),
            pltpu.VMEM((8, 1024), f32),
            pltpu.VMEM((M, D), bf16),
            pltpu.VMEM((D,), bf16),
            pltpu.SemaphoreType.DMA((len(GROUPS),)),
            pltpu.SemaphoreType.DMA((1,)),
        ],
        compiler_params=pltpu.CompilerParams(
            vmem_limit_bytes=100 * 1024 * 1024,
            disable_bounds_checks=True,
            disable_semaphore_checks=True,
            internal_scratch_in_bytes=48 * 1024,
        ),
        name="rmt_mod",
    )(A_x.reshape(NCH, CH, SEG, D), A_mem0.reshape(M, D), A_Wq, A_Wk, A_Wv, A_Wo.reshape(H * DH, D),
      B_w_r, B_w_gate.T, B_w_up.T, B_w_down)
    return out.reshape(1, S, D)
```

```python
import math

import jax
import jax.numpy as jnp
from jax import lax
import jax.experimental.pallas as pl
import jax.experimental.pallas.tpu as pltpu

bf16 = jnp.bfloat16
f32 = jnp.float32
u32 = jnp.uint32
i32 = jnp.int32

S = 2048
D = 640
H = 32
DH = 128
NP = H // 2
NU = NP * 3
M = 8
SEG = 32
NSEG = S // SEG
F = 1728
C = 8
CH = 4
NCH = NSEG // CH
NJ = D // 128
EPS = 1e-5
NEG = -1e30
LOG2E = math.log2(math.e)
CEXP = (DH ** -0.5) * LOG2E
NT = (((1,), (1,)), ((), ()))

LAG_B, POS_B = 1, 6
LAG_D, POS_D = 3, 4
POS_B0 = (6, 6, 4, 5)
KMAJ = (5, 4, 4, 5)
MORDS = ((1, 0, 2), (1, 0, 2), (1, 0, 2), (1, 0, 2))
EBS = ((0, 6, 12, 20, 22, 32), (0, 9, 14, 18, 22, 27, 32), (0, 8, 15, 17, 20, 32), (0, 8, 14, 19, 23, 28))
EPOS = ((4, 2), (2, 3), (1, 3), (4, 2))
HL = EBS[CH - 1][-1]
NV2 = (8, 2)
VGB = ((0, 5, 11, 16), (0, 5, 11, 17, 24))
LAG_V = 11
TIE_KT = ((3, 0, 0, 0, 0, 3), (0, 0, 4, 0, 0, 3))
TIE_W, TIE_E = 2, 7
E_RATE, E_SKIP = 0.6, 0

NPL = 4
UPL = 8
U0 = 9
CPL = NCH // NPL
SPL = NSEG // NPL
HEAD_GROUPS = (("p0",), ("w0", "p1"), ("w1", "p2", "p3"), ("w2", "w3", "w4"),
               ("mem0", "wr", "w5", "w6", "w7", "w8"))
HOLD = (0, 0, 0, 2, 2)
LOOP_GROUPS = tuple(
    tuple("w%d" % u for u in range(U0 + i * UPL, U0 + (i + 1) * UPL)) + ("x%d" % i,) for i in range(NPL))
TAIL_GROUPS = (tuple("w%d" % u for u in range(U0 + NPL * UPL, NU)) + ("f0", "f1", "f2"),
               tuple("o%d" % j for j in range(NJ)))
GROUPS = HEAD_GROUPS + LOOP_GROUPS + TAIL_GROUPS
TIE_LAG = 6
LN_NUM, LN_DEN = 6, 7
FFN_SKIP = 14


def _tob(x):
    return pltpu.bitcast(x, bf16)


def _tou(x):
    return pltpu.bitcast(x, u32)


def _zero_of(x):
    return (pltpu.bitcast(x, u32) >> 16) >> 16


def _rb(x):
    return x.astype(bf16).astype(f32)


def _layernorm(x, tie=None):
    ps = x[:, 0:128]
    if tie is not None:
        ps = ps + tie
    for j in range(1, NJ):
        ps = ps + x[:, j * 128:(j + 1) * 128]
    mu = jnp.sum(ps, axis=-1, keepdims=True) * (1.0 / D)
    xc = x - mu
    var = jnp.sum(xc * xc, axis=-1, keepdims=True) * (1.0 / D)
    den = _rb(jnp.sqrt(_rb(_rb(var) + EPS)))
    return (_rb(x - _rb(mu)) * pl.reciprocal(den, approx=False, full_range=False)).astype(bf16)


def _sigmoid(z):
    return pl.reciprocal(1.0 + jnp.exp2(z * (-LOG2E)), approx=True)


def _silu(z):
    return z * _sigmoid(z)


def _dot(a, b):
    return jnp.dot(a, b, preferred_element_type=f32)


def _dot_t(a, b):
    return lax.dot_general(a, b, NT, preferred_element_type=f32)


def _kernel(x_hbm, mem0_hbm, wq_hbm, wk_hbm, wv_hbm, wo_hbm, wr_hbm, wg_hbm, wu_hbm, wd_hbm,
            out_hbm,
            xv, lhs, xpre, zbuf, raw, wqkv, wo, pre, stg, sst, wg, wu, wd, outv, mask_ref,
            accv, ocv, rds, wr8, mem0_v, wr_v, sem, sem_out):
    w32 = [w.bitcast(u32) for w in (wq_hbm, wk_hbm, wv_hbm)]
    wo32 = wo_hbm.bitcast(u32)

    def src_dst(name):
        if name == "mem0":
            return mem0_hbm, mem0_v
        if name == "wr":
            return wr_hbm, wr_v
        k, n = name[0], int(name[1:])
        if k == "x":
            idx = (pl.ds(n * CPL, CPL), slice(None), pl.ds(8, SEG - 8), slice(None))
            return x_hbm.at[idx], xv.at[idx]
        if k == "p":
            idx = (pl.ds(n * 4, 4), slice(None), pl.ds(0, 8), slice(None))
            return x_hbm.at[idx], xv.at[idx]
        if k == "w":
            return w32[n % 3].at[:, n // 3, :], raw.at[n]
        if k == "f":
            return ((wg_hbm, wg), (wu_hbm, wu), (wd_hbm, wd))[n]
        return wo32.at[:, pl.ds(n * 128, 128)], wo.at[n]

    cps = [[pltpu.make_async_copy(*src_dst(nm), sem.at[gi]) for nm in grp]
           for gi, grp in enumerate(GROUPS)]
    for grp in cps:
        for cp in grp:
            cp.start()

    rr = lax.broadcasted_iota(i32, (64, 80), 0)
    hr = jnp.where(rr < 32, 0, 1)
    pr = jnp.where((rr & 31) < 8, rr & 31, (rr & 31) + 8)
    cc = lax.broadcasted_iota(i32, (64, 80), 1)
    hc = jnp.where(cc < 40, 0, 1)
    pc = cc - 40 * hc
    mask_ref[...] = jnp.where((hr == hc) & ((pr < M) | (pr >= pc)), 1.0, 0.0).astype(f32)

    st = {}
    lane8 = lax.broadcasted_iota(i32, (8, 128), 1)
    sub8 = lax.broadcasted_iota(i32, (8, 128), 0)

    def ln_pre(b):
        xb = xv[b * 4:(b + 1) * 4, :, 0:8, :].astype(f32).reshape(128, D)
        xpre[b] = _tou(_layernorm(xb))

    def repack(u):
        ev = raw[u, pl.ds(0, D // 2, stride=2), :]
        od = raw[u, pl.ds(1, D // 2, stride=2), :]
        ws = ((ev & jnp.uint32(0xFFFF)) | (od << 16), (ev >> 16) | (od & jnp.uint32(0xFFFF0000)))
        wqkv[2 * u] = ws[0]
        wqkv[2 * u + 1] = ws[1]
        return ws

    def pre_dots(u, b, hook, ws=None):
        xu = xpre[b]
        res = []
        for hh in range(2):
            tie = hook()
            xt = xu
            if tie is not None:
                top = jnp.concatenate([xu[0:8, 0:128] ^ tie, xu[0:8, 128:]], axis=1)
                xt = jnp.concatenate([top, xu[8:]], axis=0)
            w = wqkv[2 * u + hh] if ws is None else ws[hh]
            res.append(_dot(_tob(xt), _tob(w)))
            st["after"] = res[-1][0:8]
        parts = []
        for k in range(16):
            parts += [res[0][k * 8:(k + 1) * 8], res[1][k * 8:(k + 1) * 8]]
        pre[u, b * 4:(b + 1) * 4] = jnp.concatenate(parts, axis=0).reshape(4, CH * 16, 128)

    def score(i, gl, xn32):
        zbuf[i * CPL + gl // 16, (gl % 16) * 8:(gl % 16) * 8 + 8, :] = xn32
        rc = jnp.sum(xn32 * st["wr"], axis=-1, keepdims=True)
        st["rd"] = jnp.where(lane8 == gl, rc, st["rd"])

    def ln_group(i, s, k):
        tie = None
        if st["after"] is not None:
            tie = pltpu.bitcast(_zero_of(st["after"]), f32)
        xn = _layernorm(xv[i * CPL + s // CH, s % CH, k * 8:(k + 1) * 8, :].astype(f32), tie)
        score(i, s * 4 + k, xn.astype(f32))
        if k == 1 and s % 2 == 0:
            xp = _tob(xpre[i, s * 4:s * 4 + 8, :]).astype(f32)
            score(i, s * 4, xp[0:8])
            score(i, s * 4 + 4, xp[8:16])
        if k == 2:
            st["xn2"] = xn
        else:
            r0 = (s % CH) * 16 + (k // 2) * 8
            pair = jnp.concatenate([xn if k == 1 else st["xn2"], xn], axis=0)
            lhs[i * CPL + s // CH, r0:r0 + 8, :] = _tou(pair)
        return _zero_of(st["rd"])

    def topk():
        rd = _rb(rds[...].reshape(NPL * 8, 128))
        rd = jnp.where(rd == 0.0, 0.0, rd)
        bits = pltpu.bitcast(rd, i32)
        mono = jnp.where(bits < 0, bits ^ jnp.int32(0x7FFFFFFF), bits)
        rowid = jnp.concatenate([lane8 * 8 + sub8 + i * SPL * SEG for i in range(NPL)], axis=0)
        key = ((((mono >> 16) + 32768) << 11) | (S - 1 - rowid)) | jnp.int32(0x20000000)
        key = jnp.where(jnp.concatenate([lane8] * NPL, axis=0) < SPL * 4, pltpu.bitcast(key, f32), 0.0)
        row8 = lax.broadcasted_iota(i32, (8, 1), 0)
        ksel = jnp.zeros((8, 1), f32)
        for t in range(C):
            km = jnp.max(jnp.max(key, axis=0, keepdims=True), axis=1, keepdims=True)
            key = jnp.where(key == km, 0.0, key)
            ksel = jnp.where(row8 == t, km, ksel)
        ksel = pltpu.bitcast(ksel, i32)
        iv = S - 1 - (ksel & (S - 1))
        idxs = [iv[t, 0] for t in range(C)]
        xs = jnp.concatenate([zbuf[i_ >> 7, pl.ds(i_ & 127, 1), :] for i_ in idxs], axis=0)
        hi16 = (((ksel >> 11) & 65535) - 32768) << 16
        rbits = jnp.where(hi16 < 0, hi16 ^ jnp.int32(0x7FFF0000), hi16)
        return idxs, xs, _rb(_sigmoid(pltpu.bitcast(rbits, f32)))

    def ffn_tasks(idxs, xs, rsel):
        cols = [(k * 128, min(F, (k + 1) * 128)) for k in range(pl.cdiv(F, 128))]
        xsb = xs.astype(bf16)
        hid = []
        tmp = {}

        def gate(a, b):
            tmp["g"] = _rb(_dot_t(xsb, wg[a:b, :]))

        def up(a, b):
            hid.append((_rb(_silu(tmp["g"])) * _rb(_dot_t(xsb, wu[a:b, :]))).astype(bf16))

        def down(k):
            t = _dot(hid[k], wd[cols[k][0]:cols[k][1], :])
            tmp["y"] = t if k == 0 else t + tmp["y"]

        def fin():
            zs = _rb(xs + _rb(_rb(tmp["y"]) * rsel))
            for t in range(C):
                zbuf[idxs[t] >> 7, pl.ds(idxs[t] & 127, 1), :] = zs[t:t + 1]

        tasks = []
        for a, b in cols:
            tasks += [lambda a=a, b=b: gate(a, b), lambda a=a, b=b: up(a, b)]
        tasks += [lambda k=k: down(k) for k in range(len(cols))]
        return tasks + [fin]

    def run_region(work, side=(), tasks=(), skip=0):
        side, tasks = list(side), list(tasks)
        ties = []
        st["after"] = None
        cnt = {"dot": 0, "credit": 0}

        def hook():
            di = cnt["dot"]
            cnt["dot"] += 1
            if tasks and di >= skip:
                tasks.pop(0)()
            tie = None
            if ties and ties[0][0] <= di:
                tie = ties.pop(0)[1]
            if side and di + TIE_LAG < 2 * len(work):
                cnt["credit"] += LN_NUM
                if cnt["credit"] >= LN_DEN:
                    cnt["credit"] -= LN_DEN
                    ties.append((di + TIE_LAG, ln_group(*side.pop(0))))
            return tie

        for u, b, *ws in work:
            pre_dots(u, b, hook, *ws)
        assert not ties and not side and not tasks

    pending = []
    units, blocks = [], []
    for gi, grp in enumerate(HEAD_GROUPS):
        for cp in cps[gi]:
            cp.wait()
        for u in [int(nm[1:]) for nm in grp if nm[0] == "w" and nm != "wr"]:
            repack(u)
            pending += [(u, b) for b in blocks]
            units.append(u)
        for b in [int(nm[1:]) for nm in grp if nm[0] == "p"]:
            ln_pre(b)
            pending += [(u, b) for u in units]
            blocks.append(b)
        if "mem0" in grp:
            accv[...] = jnp.concatenate([mem0_v[...].astype(f32), jnp.zeros((40, D), f32)], axis=0)
            ocv[...] = jnp.zeros(ocv.shape, f32)
            wr8[:, 0:D] = jnp.broadcast_to(wr_v[...].astype(f32).reshape(1, D), (8, D))
        n = len(pending) - HOLD[gi]
        work, pending = pending[:n], pending[n:]
        run_region(work)
    assert pending == [(U0 - 1, 2), (U0 - 1, 3)]

    def pro_body(i, carry):
        ub = U0 + i * UPL
        for k in range(UPL):
            pltpu.make_async_copy(w32[0].at[:, 0, :], raw.at[ub + k], sem.at[len(HEAD_GROUPS) + i]).wait()
        idx = (pl.ds(i * CPL, CPL), slice(None), pl.ds(8, SEG - 8), slice(None))
        pltpu.make_async_copy(x_hbm.at[idx], xv.at[idx], sem.at[len(HEAD_GROUPS) + i]).wait()
        ws = [None] + [repack(ub + k) for k in range(UPL)]
        work = [(ub - 1 + k // 4, k % 4, ws[k // 4]) for k in range(2, 2 + 4 * UPL)]
        st["wr"] = wr8[:, 0:D]
        st["rd"] = jnp.zeros((8, 128), f32)
        run_region(work, side=[(i, s, k) for s in range(SPL) for k in (1, 2, 3)])
        rds[i] = st["rd"]
        return carry

    lax.fori_loop(0, NPL, pro_body, 0)

    for cp in cps[-2]:
        cp.wait()
    ub = U0 + NPL * UPL
    for u in range(ub, NU):
        repack(u)
    run_region([(ub - 1 + k // 4, k % 4) for k in range(2, 4 + 4 * (NU - ub))],
               tasks=ffn_tasks(*topk()), skip=FFN_SKIP)
    for cp in cps[-1]:
        cp.wait()

    sub4 = lax.broadcasted_iota(i32, (8, D), 0) < 4

    def finalize(ci, sl, r0, r1, sv, c0=0, c1=D):
        xr = xv[ci, sl, r0:r1, c0:c1].astype(f32)
        g = _silu(zbuf[ci, sl * SEG + r0:sl * SEG + r1, c0:c1])
        outv[ci, sl, r0:r1, c0:c1] = (xr + sv * g).astype(bf16)

    def finish(ci, sl, acc):
        acc = jnp.concatenate(acc, axis=1)
        finalize(ci, sl, 8, SEG, acc[8:32])
        if sl % 2 == 1:
            finalize(ci, sl, 0, 8, acc[32:40])
            finalize(ci, sl - 1, 0, 8, acc[40:48])
        return _tou(acc[0:16].astype(bf16))

    def finish_last(ci):
        o2 = ocv[...].astype(bf16)
        acc = [_dot(o2, _tob(wo[j, HL * 64:, :])) + accv[:, j * 128:(j + 1) * 128] for j in range(NJ)]
        return finish(ci, CH - 1, acc)

    vq = []
    clock = [0]

    def vnext():
        ready = [i for i, t in enumerate(vq) if t[0] <= clock[0]]
        if not ready:
            return None
        return vq.pop(min(ready, key=lambda i: (vq[i][2], i)))[1]()

    def vforce(deadline):
        for t in [t for t in vq if t[2] <= deadline]:
            vq.remove(t)
            t[1]()

    def tied(w, g):
        tie = vnext()
        if tie is None:
            return w
        parts = [w[0:g * 8], w[g * 8:g * 8 + 8] ^ tie, w[g * 8 + 8:]]
        return jnp.concatenate([t for t in parts if t.shape[0]], axis=0)

    def orow(h, r0, n):
        r0 += 240 + (h % 2) * 32 if h < H else 304 + (h % 2) * 16
        return ((h % H) // 2, slice(r0, r0 + n), slice(None))

    def step(ci, sl, mem):
        xu = lhs[ci, sl * 16:(sl + 1) * 16, :]
        x = _tob(jnp.concatenate([jnp.where(sub4, mem, xu[0:8]), xu[8:16]], axis=0))
        mord, eb, odd = MORDS[sl], EBS[sl], sl % 2
        probs = {}
        vs = {}

        early = {}
        for k in range(NJ):
            clock[0] += 1
            for d in range(KMAJ[sl]):
                key = (d // 6, mord[(d % 6) // 2], d % 2)
                w = wqkv[2 * (key[0] * 3 + key[1]) + key[2], k * 64:(k + 1) * 64, :]
                if d == 3 and odd:
                    w = tied(w, TIE_W)
                t = _dot(x[:, k * 128:(k + 1) * 128], _tob(w))
                early[key] = t if k == 0 else t + early[key]

        def slot_of(p, m, hh):
            return m * 2 + hh

        def project(p, di):
            m, hh = mord[di // 2], di % 2
            if (p, m, hh) in early:
                r = early[p, m, hh]
            else:
                clock[0] += 1
                r = _dot(x, _tob(tied(wqkv[2 * (p * 3 + m) + hh], TIE_KT[odd][di] * 8 + TIE_W)))
            b0 = slot_of(p, m, hh) * 40
            stg[odd * NP + p, b0:b0 + 8, :] = r[0:8]
            stg[odd * NP + p, b0 + 16:b0 + 40, :] = r[8:32]
            if m > 0:
                stg[odd * NP + p, b0 + 8:b0 + 16, :] = pre[p * 3 + m, ci, sl * 16 + hh * 8:sl * 16 + hh * 8 + 8, :]

        def mxu_rows(p, a):
            if p < NV2[odd]:
                return jnp.concatenate([a[0:8], a[32:40], a[16:32], a[48:64]], axis=0)
            return a

        def operand(p, m):
            b0 = slot_of(p, m, 0) * 40
            if m > 0:
                a = stg[odd * NP + p, b0:b0 + 80, :]
            else:
                a = mxu_rows(p, jnp.concatenate([stg[odd * NP + p, b0:b0 + 8, :], stg[odd * NP + p, b0 + 16:b0 + 48, :],
                                                 stg[odd * NP + p, b0 + 56:b0 + 80, :]], axis=0))
            return a.astype(bf16)

        def vpu_rows(p, hh, lv, g):
            gb = VGB[lv]
            r0 = sl * 16 + hh * 8

            def row(m, i):
                b0 = slot_of(p, m, hh) * 40 + 8 + 8 * lv - i
                return stg[odd * NP + p, b0:b0 + 8, :]

            if g == 0:
                q = pre[p * 3, ci, r0:r0 + 8, :] if lv == 0 else row(0, 0)
                vs[p, hh, lv] = (q * CEXP, None, None, None)
            q, m_old, l, o = vs[p, hh, lv]
            i0, n = gb[g], gb[g + 1] - gb[g]

            def rows(m):
                return jnp.concatenate([row(m, i0 + i) for i in range(n)], axis=0).reshape(n, 8, 128)

            s = jnp.sum(q[None] * rows(1), axis=-1, keepdims=True)
            if i0 + n > 9 + 8 * lv:
                ok = (lax.broadcasted_iota(i32, (n, 8, 1), 1)
                      >= lax.broadcasted_iota(i32, (n, 8, 1), 0) + (i0 - 8 - 8 * lv))
                s = jnp.where(ok, s, NEG)
            mx = jnp.max(s, axis=0)
            if m_old is not None:
                mx = jnp.maximum(mx, m_old)
            e = jnp.exp2(s - mx[None])
            el, ev = jnp.sum(e, axis=0), jnp.sum(e * rows(2), axis=0)
            if m_old is None:
                l, o = el, ev
            else:
                alpha = jnp.exp2(m_old - mx)
                l, o = l * alpha + el, o * alpha + ev
            if g == len(gb) - 2:
                o = o * pl.reciprocal(l, approx=True)
                if lv == 0:
                    stg[orow(H + 2 * p + hh, (1 - odd) * 8, 8)] = o
                else:
                    stg[orow(2 * p + hh, 8, 8)] = o
            vs[p, hh, lv] = (q, mx, l, o)
            return _zero_of(o)

        def scores(p):
            if not 0 <= p < NP:
                return
            sc = jnp.where(mxu_rows(p, mask_ref[...]) > 0.5, _dot_t(operand(p, 0), operand(p, 1)), NEG)
            n = sc.shape[0]
            mx = jnp.max(sc, axis=-1, keepdims=True)
            sst[p % 2, 0:n] = sc
            e = jnp.exp2((sst[p % 2, 0:n] - mx) * CEXP)
            l = jnp.sum(e, axis=-1, keepdims=True)
            sst[2 + p % 2, 0:n] = e
            probs[p] = (sst[2 + p % 2, 0:n] * pl.reciprocal(l, approx=True)).astype(bf16)

        def attend(p):
            if not 0 <= p < NP:
                return
            o = _dot(probs[p], operand(p, 2))
            for hh in range(2):
                if p < NV2[odd]:
                    stg[orow(2 * p + hh, 0, 8)] = o[hh * 8:hh * 8 + 8]
                    stg[orow(2 * p + hh, 16, 16)] = o[16 + hh * 16:32 + hh * 16]
                else:
                    stg[orow(2 * p + hh, 0, 32)] = o[hh * 32:(hh + 1) * 32]

        def oheads(h0, h1):
            vforce((sl, h1 - 1))
            if not odd:
                return jnp.concatenate([stg[orow(h, 0, 32)] for h in range(h0, h1)], axis=1)
            return jnp.concatenate([jnp.concatenate([stg[orow(h, 0, 32)], stg[orow(H + h, 0, 16)]], axis=0)
                                    for h in range(h0, h1)], axis=1)

        for slot in range(NP):
            for di in range(7):
                if di == (POS_B0[sl] if slot == LAG_B else POS_B):
                    scores(slot - LAG_B)
                if di == POS_D:
                    attend(slot - LAG_D)
                if di < 6:
                    project(slot, di)
            for hh in range(2):
                for lv in ((1, 0) if slot < NV2[odd] else (0,)):
                    for g in range(len(VGB[lv]) - 1):
                        vq.append((clock[0] + LAG_V, lambda a=(slot, hh, lv, g): vpu_rows(*a),
                                   (sl if lv == 1 else sl | 1, 2 * slot + hh)))
        tiles, credit = 0, 0.0
        acc = [None] * NJ
        for i in range(len(eb) - 1):
            h0, h1 = eb[i], eb[i + 1]
            o2 = oheads(h0, h1).astype(bf16)
            for j in range(NJ):
                ws = []
                for h in range(h0, h1):
                    tiles += 1
                    if tiles % (3 if odd else 5) == 0:
                        clock[0] += 1
                    w = wo[j, h * 64:(h + 1) * 64, :]
                    if odd and tiles > E_SKIP:
                        credit += E_RATE
                        if credit >= 1.0:
                            credit -= 1.0
                            w = tied(w, TIE_E)
                    ws.append(w)
                t = _dot(o2, _tob(jnp.concatenate(ws, axis=0)))
                acc[j] = t if acc[j] is None else t + acc[j]
                if j == EPOS[sl][0]:
                    scores(NP + i - LAG_B)
                if j == EPOS[sl][1]:
                    attend(NP + i - LAG_D)
        if sl == CH - 1:
            accv[...] = jnp.concatenate(acc, axis=1)
            ocv[...] = oheads(HL, H)
            assert not vq
            return None
        return finish(ci, sl, acc)

    def out_cp(*idx):
        return pltpu.make_async_copy(outv.at[idx], out_hbm.at[idx], sem_out.at[0])

    def chunk(ci, carry):
        prev = jnp.maximum(ci - 1, 0)
        mem = finish_last(prev)

        @pl.when(ci >= 1)
        def _():
            out_cp(prev, pl.ds(2, 2)).start()

        for sl in range(CH):
            mem = step(ci, sl, mem)
            if sl == 1:
                out_cp(ci, pl.ds(0, 2)).start()
        return carry

    lax.fori_loop(0, NCH, chunk, 0)
    o2 = ocv[...].astype(bf16)
    for j in range(NJ):
        c0, c1 = j * 128, (j + 1) * 128
        t = _dot(o2, _tob(wo[j, HL * 64:, :])) + accv[:, c0:c1]
        finalize(NCH - 1, CH - 1, 8, SEG, t[8:32], c0, c1)
        finalize(NCH - 1, CH - 1, 0, 8, t[32:40], c0, c1)
        finalize(NCH - 1, CH - 2, 0, 8, t[40:48], c0, c1)
        out_cp(NCH - 1, pl.ds(2, 2), slice(None), pl.ds(c0, 128)).start()
    pltpu.make_async_copy(outv, out_hbm, sem_out.at[0]).wait()


@jax.jit
def pallas_recurrent_scan__memory_aug_recurrent_mem_tr__moe_arch_mod__prompt_kernel(
    A_x, A_mem0, A_Wq, A_Wk, A_Wv, A_Wo, A_seg_len, B_x, B_w_r, B_w_gate, B_w_up, B_w_down,
):
    hbm = pl.BlockSpec(memory_space=pltpu.MemorySpace.HBM)
    out = pl.pallas_call(
        _kernel,
        out_shape=jax.ShapeDtypeStruct((NCH, CH, SEG, D), bf16),
        in_specs=[hbm] * 10,
        out_specs=hbm,
        scratch_shapes=[
            pltpu.VMEM((NCH, CH, SEG, D), bf16),
            pltpu.VMEM((NCH, CH * 16, D), u32),
            pltpu.VMEM((4, 64, D), u32),
            pltpu.VMEM((NCH, CH * SEG, D), f32),
            pltpu.VMEM((NU, D, 128), u32),
            pltpu.VMEM((NU * 2, D // 2, 128), u32),
            pltpu.VMEM((NJ, H * DH // 2, 128), u32),
            pltpu.VMEM((NU, NCH, CH * 16, 128), f32),
            pltpu.VMEM((2 * NP, 352, 128), f32),
            pltpu.VMEM((4, 64, 80), f32),
            pltpu.VMEM((F, D), bf16),
            pltpu.VMEM((F, D), bf16),
            pltpu.VMEM((F, D), bf16),
            pltpu.VMEM((NCH, CH, SEG, D), bf16),
            pltpu.VMEM((64, 80), f32),
            pltpu.VMEM((48, D), f32),
            pltpu.VMEM((48, (H - HL) * DH), f32),
            pltpu.VMEM((NPL, 8, 128), f32),
            pltpu.VMEM((8, 1024), f32),
            pltpu.VMEM((M, D), bf16),
            pltpu.VMEM((D,), bf16),
            pltpu.SemaphoreType.DMA((len(GROUPS),)),
            pltpu.SemaphoreType.DMA((1,)),
        ],
        compiler_params=pltpu.CompilerParams(
            vmem_limit_bytes=100 * 1024 * 1024,
            disable_bounds_checks=True,
            disable_semaphore_checks=True,
            internal_scratch_in_bytes=48 * 1024,
        ),
        name="rmt_mod",
    )(A_x.reshape(NCH, CH, SEG, D), A_mem0.reshape(M, D), A_Wq, A_Wk, A_Wv, A_Wo.reshape(H * DH, D),
      B_w_r, B_w_gate.T, B_w_up.T, B_w_down)
    return out.reshape(1, S, D)
```

```python
import math

import jax
import jax.numpy as jnp
from jax import lax
import jax.experimental.pallas as pl
import jax.experimental.pallas.tpu as pltpu

bf16 = jnp.bfloat16
f32 = jnp.float32
u32 = jnp.uint32
i32 = jnp.int32

S = 2048
D = 640
H = 32
DH = 128
NP = H // 2
NU = NP * 3
M = 8
SEG = 32
NSEG = S // SEG
F = 1728
C = 8
CH = 4
NCH = NSEG // CH
NJ = D // 128
EPS = 1e-5
NEG = -1e30
LOG2E = math.log2(math.e)
CEXP = (DH ** -0.5) * LOG2E
NT = (((1,), (1,)), ((), ()))

LAG_B, POS_B = 1, 6
LAG_D, POS_D = 3, 4
POS_B0 = (6, 6, 5, 5)
KMAJ = (4, 4, 4, 5)
MORDS = ((1, 0, 2), (1, 0, 2), (1, 0, 2), (1, 0, 2))
EBS = ((0, 6, 12, 20, 21, 32), (0, 9, 14, 18, 22, 27, 32), (0, 8, 15, 17, 25, 32), (0, 8, 14, 19, 23, 28))
EPOS = ((4, 2), (2, 3), (4, 4), (4, 2))
HL = EBS[CH - 1][-1]
NV2 = (8, 2)
VGB = ((0, 5, 11, 16), (0, 5, 11, 17, 24))
LAG_V = 11
TIE_KT = ((3, 0, 0, 0, 0, 3), (0, 0, 4, 0, 0, 3))
TIE_W, TIE_E = 2, 7
E_RATE, E_SKIP = 0.6, 0

NPL = 4
UPL = 8
U0 = 9
CPL = NCH // NPL
SPL = NSEG // NPL
HEAD_GROUPS = (("p0",), ("w0", "p1"), ("w1", "p2", "p3"), ("w2", "w3", "w4"),
               ("mem0", "wr", "w5", "w6", "w7", "w8"))
HOLD = (0, 0, 0, 2, 2)
LOOP_GROUPS = tuple(
    tuple("w%d" % u for u in range(U0 + i * UPL, U0 + (i + 1) * UPL)) + ("x%d" % i,) for i in range(NPL))
TAIL_GROUPS = (tuple("w%d" % u for u in range(U0 + NPL * UPL, NU)) + ("f0", "f1", "f2"),
               tuple("o%d" % j for j in range(NJ)))
GROUPS = HEAD_GROUPS + LOOP_GROUPS + TAIL_GROUPS
TIE_LAG = 6
LN_NUM, LN_DEN = 6, 7
FFN_SKIP = 16


def _tob(x):
    return pltpu.bitcast(x, bf16)


def _tou(x):
    return pltpu.bitcast(x, u32)


def _zero_of(x):
    return (pltpu.bitcast(x, u32) >> 16) >> 16


def _rb(x):
    return x.astype(bf16).astype(f32)


def _layernorm(x, tie=None):
    ps = x[:, 0:128]
    if tie is not None:
        ps = ps + tie
    for j in range(1, NJ):
        ps = ps + x[:, j * 128:(j + 1) * 128]
    mu = jnp.sum(ps, axis=-1, keepdims=True) * (1.0 / D)
    xc = x - mu
    var = jnp.sum(xc * xc, axis=-1, keepdims=True) * (1.0 / D)
    den = _rb(jnp.sqrt(_rb(_rb(var) + EPS)))
    return (_rb(x - _rb(mu)) * pl.reciprocal(den, approx=False, full_range=False)).astype(bf16)


def _sigmoid(z):
    return pl.reciprocal(1.0 + jnp.exp2(z * (-LOG2E)), approx=True)


def _silu(z):
    return z * _sigmoid(z)


def _dot(a, b):
    return jnp.dot(a, b, preferred_element_type=f32)


def _dot_t(a, b):
    return lax.dot_general(a, b, NT, preferred_element_type=f32)


def _kernel(x_hbm, mem0_hbm, wq_hbm, wk_hbm, wv_hbm, wo_hbm, wr_hbm, wg_hbm, wu_hbm, wd_hbm,
            out_hbm,
            xv, lhs, xpre, zbuf, raw, wqkv, wo, pre, stg, sst, wg, wu, wd, outv, mask_ref,
            accv, ocv, rds, wr8, mem0_v, wr_v, sem, sem_out):
    w32 = [w.bitcast(u32) for w in (wq_hbm, wk_hbm, wv_hbm)]
    wo32 = wo_hbm.bitcast(u32)

    def src_dst(name):
        if name == "mem0":
            return mem0_hbm, mem0_v
        if name == "wr":
            return wr_hbm, wr_v
        k, n = name[0], int(name[1:])
        if k == "x":
            idx = (pl.ds(n * CPL, CPL), slice(None), pl.ds(8, SEG - 8), slice(None))
            return x_hbm.at[idx], xv.at[idx]
        if k == "p":
            idx = (pl.ds(n * 4, 4), slice(None), pl.ds(0, 8), slice(None))
            return x_hbm.at[idx], xv.at[idx]
        if k == "w":
            return w32[n % 3].at[:, n // 3, :], raw.at[n]
        if k == "f":
            return ((wg_hbm, wg), (wu_hbm, wu), (wd_hbm, wd))[n]
        return wo32.at[:, pl.ds(n * 128, 128)], wo.at[n]

    cps = [[pltpu.make_async_copy(*src_dst(nm), sem.at[gi]) for nm in grp]
           for gi, grp in enumerate(GROUPS)]
    for grp in cps:
        for cp in grp:
            cp.start()

    rr = lax.broadcasted_iota(i32, (64, 80), 0)
    hr = jnp.where(rr < 32, 0, 1)
    pr = jnp.where((rr & 31) < 8, rr & 31, (rr & 31) + 8)
    cc = lax.broadcasted_iota(i32, (64, 80), 1)
    hc = jnp.where(cc < 40, 0, 1)
    pc = cc - 40 * hc
    mask_ref[...] = jnp.where((hr == hc) & ((pr < M) | (pr >= pc)), 1.0, 0.0).astype(f32)

    st = {}
    lane8 = lax.broadcasted_iota(i32, (8, 128), 1)
    sub8 = lax.broadcasted_iota(i32, (8, 128), 0)

    def ln_pre(b):
        xb = xv[b * 4:(b + 1) * 4, :, 0:8, :].astype(f32).reshape(128, D)
        xpre[b] = _tou(_layernorm(xb))

    def repack(u):
        ev = raw[u, pl.ds(0, D // 2, stride=2), :]
        od = raw[u, pl.ds(1, D // 2, stride=2), :]
        ws = ((ev & jnp.uint32(0xFFFF)) | (od << 16), (ev >> 16) | (od & jnp.uint32(0xFFFF0000)))
        wqkv[2 * u] = ws[0]
        wqkv[2 * u + 1] = ws[1]
        return ws

    def pre_dots(u, b, hook, ws=None):
        xu = xpre[b]
        res = []
        for hh in range(2):
            tie = hook()
            xt = xu
            if tie is not None:
                top = jnp.concatenate([xu[0:8, 0:128] ^ tie, xu[0:8, 128:]], axis=1)
                xt = jnp.concatenate([top, xu[8:]], axis=0)
            w = wqkv[2 * u + hh] if ws is None else ws[hh]
            res.append(_dot(_tob(xt), _tob(w)))
            st["after"] = res[-1][0:8]
        parts = []
        for k in range(16):
            parts += [res[0][k * 8:(k + 1) * 8], res[1][k * 8:(k + 1) * 8]]
        pre[u, b * 4:(b + 1) * 4] = jnp.concatenate(parts, axis=0).reshape(4, CH * 16, 128)

    def score(i, gl, xn32):
        zbuf[i * CPL + gl // 16, (gl % 16) * 8:(gl % 16) * 8 + 8, :] = xn32
        rc = jnp.sum(xn32 * st["wr"], axis=-1, keepdims=True)
        st["rd"] = jnp.where(lane8 == gl, rc, st["rd"])

    def ln_group(i, s, k):
        tie = None
        if st["after"] is not None:
            tie = pltpu.bitcast(_zero_of(st["after"]), f32)
        xn = _layernorm(xv[i * CPL + s // CH, s % CH, k * 8:(k + 1) * 8, :].astype(f32), tie)
        score(i, s * 4 + k, xn.astype(f32))
        if k == 1 and s % 2 == 0:
            xp = _tob(xpre[i, s * 4:s * 4 + 8, :]).astype(f32)
            score(i, s * 4, xp[0:8])
            score(i, s * 4 + 4, xp[8:16])
        if k == 2:
            st["xn2"] = xn
        else:
            r0 = (s % CH) * 16 + (k // 2) * 8
            pair = jnp.concatenate([xn if k == 1 else st["xn2"], xn], axis=0)
            lhs[i * CPL + s // CH, r0:r0 + 8, :] = _tou(pair)
        return _zero_of(st["rd"])

    def topk():
        rd = _rb(rds[...].reshape(NPL * 8, 128))
        rd = jnp.where(rd == 0.0, 0.0, rd)
        bits = pltpu.bitcast(rd, i32)
        mono = jnp.where(bits < 0, bits ^ jnp.int32(0x7FFFFFFF), bits)
        rowid = jnp.concatenate([lane8 * 8 + sub8 + i * SPL * SEG for i in range(NPL)], axis=0)
        key = ((((mono >> 16) + 32768) << 11) | (S - 1 - rowid)) | jnp.int32(0x20000000)
        key = jnp.where(jnp.concatenate([lane8] * NPL, axis=0) < SPL * 4, pltpu.bitcast(key, f32), 0.0)
        row8 = lax.broadcasted_iota(i32, (8, 1), 0)
        ksel = jnp.zeros((8, 1), f32)
        for t in range(C):
            km = jnp.max(jnp.max(key, axis=0, keepdims=True), axis=1, keepdims=True)
            key = jnp.where(key == km, 0.0, key)
            ksel = jnp.where(row8 == t, km, ksel)
        ksel = pltpu.bitcast(ksel, i32)
        iv = S - 1 - (ksel & (S - 1))
        idxs = [iv[t, 0] for t in range(C)]
        xs = jnp.concatenate([zbuf[i_ >> 7, pl.ds(i_ & 127, 1), :] for i_ in idxs], axis=0)
        hi16 = (((ksel >> 11) & 65535) - 32768) << 16
        rbits = jnp.where(hi16 < 0, hi16 ^ jnp.int32(0x7FFF0000), hi16)
        return idxs, xs, _rb(_sigmoid(pltpu.bitcast(rbits, f32)))

    def ffn_tasks(idxs, xs, rsel):
        cols = [(k * 128, min(F, (k + 1) * 128)) for k in range(pl.cdiv(F, 128))]
        xsb = xs.astype(bf16)
        hid = []
        tmp = {}

        def gate(a, b):
            tmp["g"] = _rb(_dot_t(xsb, wg[a:b, :]))

        def up(a, b):
            hid.append((_rb(_silu(tmp["g"])) * _rb(_dot_t(xsb, wu[a:b, :]))).astype(bf16))

        def down(k):
            t = _dot(hid[k], wd[cols[k][0]:cols[k][1], :])
            tmp["y"] = t if k == 0 else t + tmp["y"]

        def fin():
            zs = _rb(xs + _rb(_rb(tmp["y"]) * rsel))
            for t in range(C):
                zbuf[idxs[t] >> 7, pl.ds(idxs[t] & 127, 1), :] = zs[t:t + 1]

        tasks = []
        for a, b in cols:
            tasks += [lambda a=a, b=b: gate(a, b), lambda a=a, b=b: up(a, b)]
        tasks += [lambda k=k: down(k) for k in range(len(cols))]
        return tasks + [fin]

    def run_region(work, side=(), tasks=(), skip=0):
        side, tasks = list(side), list(tasks)
        ties = []
        st["after"] = None
        cnt = {"dot": 0, "credit": 0}

        def hook():
            di = cnt["dot"]
            cnt["dot"] += 1
            if tasks and di >= skip:
                tasks.pop(0)()
            tie = None
            if ties and ties[0][0] <= di:
                tie = ties.pop(0)[1]
            if side and di + TIE_LAG < 2 * len(work):
                cnt["credit"] += LN_NUM
                if cnt["credit"] >= LN_DEN:
                    cnt["credit"] -= LN_DEN
                    ties.append((di + TIE_LAG, ln_group(*side.pop(0))))
            return tie

        for u, b, *ws in work:
            pre_dots(u, b, hook, *ws)
        assert not ties and not side and not tasks

    pending = []
    units, blocks = [], []
    for gi, grp in enumerate(HEAD_GROUPS):
        for cp in cps[gi]:
            cp.wait()
        for u in [int(nm[1:]) for nm in grp if nm[0] == "w" and nm != "wr"]:
            repack(u)
            pending += [(u, b) for b in blocks]
            units.append(u)
        for b in [int(nm[1:]) for nm in grp if nm[0] == "p"]:
            ln_pre(b)
            pending += [(u, b) for u in units]
            blocks.append(b)
        if "mem0" in grp:
            accv[...] = jnp.concatenate([mem0_v[...].astype(f32), jnp.zeros((40, D), f32)], axis=0)
            ocv[...] = jnp.zeros(ocv.shape, f32)
            wr8[:, 0:D] = jnp.broadcast_to(wr_v[...].astype(f32).reshape(1, D), (8, D))
        n = len(pending) - HOLD[gi]
        work, pending = pending[:n], pending[n:]
        run_region(work)
    assert pending == [(U0 - 1, 2), (U0 - 1, 3)]

    def pro_body(i, carry):
        ub = U0 + i * UPL
        for k in range(UPL):
            pltpu.make_async_copy(w32[0].at[:, 0, :], raw.at[ub + k], sem.at[len(HEAD_GROUPS) + i]).wait()
        idx = (pl.ds(i * CPL, CPL), slice(None), pl.ds(8, SEG - 8), slice(None))
        pltpu.make_async_copy(x_hbm.at[idx], xv.at[idx], sem.at[len(HEAD_GROUPS) + i]).wait()
        ws = [None] + [repack(ub + k) for k in range(UPL)]
        work = [(ub - 1 + k // 4, k % 4, ws[k // 4]) for k in range(2, 2 + 4 * UPL)]
        st["wr"] = wr8[:, 0:D]
        st["rd"] = jnp.zeros((8, 128), f32)
        run_region(work, side=[(i, s, k) for s in range(SPL) for k in (1, 2, 3)])
        rds[i] = st["rd"]
        return carry

    lax.fori_loop(0, NPL, pro_body, 0)

    for cp in cps[-2]:
        cp.wait()
    ub = U0 + NPL * UPL
    for u in range(ub, NU):
        repack(u)
    run_region([(ub - 1 + k // 4, k % 4) for k in range(2, 4 + 4 * (NU - ub))],
               tasks=ffn_tasks(*topk()), skip=FFN_SKIP)
    for cp in cps[-1]:
        cp.wait()

    sub4 = lax.broadcasted_iota(i32, (8, D), 0) < 4

    def finalize(ci, sl, r0, r1, sv, c0=0, c1=D):
        xr = xv[ci, sl, r0:r1, c0:c1].astype(f32)
        g = _silu(zbuf[ci, sl * SEG + r0:sl * SEG + r1, c0:c1])
        outv[ci, sl, r0:r1, c0:c1] = (xr + sv * g).astype(bf16)

    def finish(ci, sl, acc):
        acc = jnp.concatenate(acc, axis=1)
        finalize(ci, sl, 8, SEG, acc[8:32])
        if sl % 2 == 1:
            finalize(ci, sl, 0, 8, acc[32:40])
            finalize(ci, sl - 1, 0, 8, acc[40:48])
        return _tou(acc[0:16].astype(bf16))

    def finish_last(ci):
        o2 = ocv[...].astype(bf16)
        acc = [_dot(o2, _tob(wo[j, HL * 64:, :])) + accv[:, j * 128:(j + 1) * 128] for j in range(NJ)]
        return finish(ci, CH - 1, acc)

    vq = []
    clock = [0]

    def vnext():
        ready = [i for i, t in enumerate(vq) if t[0] <= clock[0]]
        if not ready:
            return None
        return vq.pop(min(ready, key=lambda i: (vq[i][2], i)))[1]()

    def vforce(deadline):
        for t in [t for t in vq if t[2] <= deadline]:
            vq.remove(t)
            t[1]()

    def tied(w, g):
        tie = vnext()
        if tie is None:
            return w
        parts = [w[0:g * 8], w[g * 8:g * 8 + 8] ^ tie, w[g * 8 + 8:]]
        return jnp.concatenate([t for t in parts if t.shape[0]], axis=0)

    def orow(h, r0, n):
        r0 += 240 + (h % 2) * 32 if h < H else 304 + (h % 2) * 16
        return ((h % H) // 2, slice(r0, r0 + n), slice(None))

    def step(ci, sl, mem):
        xu = lhs[ci, sl * 16:(sl + 1) * 16, :]
        x = _tob(jnp.concatenate([jnp.where(sub4, mem, xu[0:8]), xu[8:16]], axis=0))
        mord, eb, odd = MORDS[sl], EBS[sl], sl % 2
        probs = {}
        vs = {}

        early = {}
        for k in range(NJ):
            clock[0] += 1
            for d in range(KMAJ[sl]):
                key = (d // 6, mord[(d % 6) // 2], d % 2)
                w = wqkv[2 * (key[0] * 3 + key[1]) + key[2], k * 64:(k + 1) * 64, :]
                if d == 3 and odd:
                    w = tied(w, TIE_W)
                t = _dot(x[:, k * 128:(k + 1) * 128], _tob(w))
                early[key] = t if k == 0 else t + early[key]

        def slot_of(p, m, hh):
            return m * 2 + hh

        def project(p, di):
            m, hh = mord[di // 2], di % 2
            if (p, m, hh) in early:
                r = early[p, m, hh]
            else:
                clock[0] += 1
                r = _dot(x, _tob(tied(wqkv[2 * (p * 3 + m) + hh], TIE_KT[odd][di] * 8 + TIE_W)))
            b0 = slot_of(p, m, hh) * 40
            stg[odd * NP + p, b0:b0 + 8, :] = r[0:8]
            stg[odd * NP + p, b0 + 16:b0 + 40, :] = r[8:32]
            if m > 0:
                stg[odd * NP + p, b0 + 8:b0 + 16, :] = pre[p * 3 + m, ci, sl * 16 + hh * 8:sl * 16 + hh * 8 + 8, :]

        def mxu_rows(p, a):
            if p < NV2[odd]:
                return jnp.concatenate([a[0:8], a[32:40], a[16:32], a[48:64]], axis=0)
            return a

        def operand(p, m):
            b0 = slot_of(p, m, 0) * 40
            if m > 0:
                a = stg[odd * NP + p, b0:b0 + 80, :]
            else:
                a = mxu_rows(p, jnp.concatenate([stg[odd * NP + p, b0:b0 + 8, :], stg[odd * NP + p, b0 + 16:b0 + 48, :],
                                                 stg[odd * NP + p, b0 + 56:b0 + 80, :]], axis=0))
            return a.astype(bf16)

        def vpu_rows(p, hh, lv, g):
            gb = VGB[lv]
            r0 = sl * 16 + hh * 8

            def row(m, i):
                b0 = slot_of(p, m, hh) * 40 + 8 + 8 * lv - i
                return stg[odd * NP + p, b0:b0 + 8, :]

            if g == 0:
                q = pre[p * 3, ci, r0:r0 + 8, :] if lv == 0 else row(0, 0)
                vs[p, hh, lv] = (q * CEXP, None, None, None)
            q, m_old, l, o = vs[p, hh, lv]
            i0, n = gb[g], gb[g + 1] - gb[g]

            def rows(m):
                return jnp.concatenate([row(m, i0 + i) for i in range(n)], axis=0).reshape(n, 8, 128)

            s = jnp.sum(q[None] * rows(1), axis=-1, keepdims=True)
            if i0 + n > 9 + 8 * lv:
                ok = (lax.broadcasted_iota(i32, (n, 8, 1), 1)
                      >= lax.broadcasted_iota(i32, (n, 8, 1), 0) + (i0 - 8 - 8 * lv))
                s = jnp.where(ok, s, NEG)
            mx = jnp.max(s, axis=0)
            if m_old is not None:
                mx = jnp.maximum(mx, m_old)
            e = jnp.exp2(s - mx[None])
            el, ev = jnp.sum(e, axis=0), jnp.sum(e * rows(2), axis=0)
            if m_old is None:
                l, o = el, ev
            else:
                alpha = jnp.exp2(m_old - mx)
                l, o = l * alpha + el, o * alpha + ev
            if g == len(gb) - 2:
                o = o * pl.reciprocal(l, approx=True)
                if lv == 0:
                    stg[orow(H + 2 * p + hh, (1 - odd) * 8, 8)] = o
                else:
                    stg[orow(2 * p + hh, 8, 8)] = o
            vs[p, hh, lv] = (q, mx, l, o)
            return _zero_of(o)

        def scores(p):
            if not 0 <= p < NP:
                return
            sc = jnp.where(mxu_rows(p, mask_ref[...]) > 0.5, _dot_t(operand(p, 0), operand(p, 1)), NEG)
            n = sc.shape[0]
            mx = jnp.max(sc, axis=-1, keepdims=True)
            sst[p % 2, 0:n] = sc
            e = jnp.exp2((sst[p % 2, 0:n] - mx) * CEXP)
            l = jnp.sum(e, axis=-1, keepdims=True)
            sst[2 + p % 2, 0:n] = e
            probs[p] = (sst[2 + p % 2, 0:n] * pl.reciprocal(l, approx=True)).astype(bf16)

        def attend(p):
            if not 0 <= p < NP:
                return
            o = _dot(probs[p], operand(p, 2))
            for hh in range(2):
                if p < NV2[odd]:
                    stg[orow(2 * p + hh, 0, 8)] = o[hh * 8:hh * 8 + 8]
                    stg[orow(2 * p + hh, 16, 16)] = o[16 + hh * 16:32 + hh * 16]
                else:
                    stg[orow(2 * p + hh, 0, 32)] = o[hh * 32:(hh + 1) * 32]

        def oheads(h0, h1):
            vforce((sl, h1 - 1))
            if not odd:
                return jnp.concatenate([stg[orow(h, 0, 32)] for h in range(h0, h1)], axis=1)
            return jnp.concatenate([jnp.concatenate([stg[orow(h, 0, 32)], stg[orow(H + h, 0, 16)]], axis=0)
                                    for h in range(h0, h1)], axis=1)

        for slot in range(NP):
            for di in range(7):
                if di == (POS_B0[sl] if slot == LAG_B else POS_B):
                    scores(slot - LAG_B)
                if di == POS_D:
                    attend(slot - LAG_D)
                if di < 6:
                    project(slot, di)
            for hh in range(2):
                for lv in ((1, 0) if slot < NV2[odd] else (0,)):
                    for g in range(len(VGB[lv]) - 1):
                        vq.append((clock[0] + LAG_V, lambda a=(slot, hh, lv, g): vpu_rows(*a),
                                   (sl if lv == 1 else sl | 1, 2 * slot + hh)))
        tiles, credit = 0, 0.0
        acc = [None] * NJ
        for i in range(len(eb) - 1):
            h0, h1 = eb[i], eb[i + 1]
            o2 = oheads(h0, h1).astype(bf16)
            for j in range(NJ):
                ws = []
                for h in range(h0, h1):
                    tiles += 1
                    if tiles % (3 if odd else 5) == 0:
                        clock[0] += 1
                    w = wo[j, h * 64:(h + 1) * 64, :]
                    if odd and tiles > E_SKIP:
                        credit += E_RATE
                        if credit >= 1.0:
                            credit -= 1.0
                            w = tied(w, TIE_E)
                    ws.append(w)
                t = _dot(o2, _tob(jnp.concatenate(ws, axis=0)))
                acc[j] = t if acc[j] is None else t + acc[j]
                if j == EPOS[sl][0]:
                    scores(NP + i - LAG_B)
                if j == EPOS[sl][1]:
                    attend(NP + i - LAG_D)
        if sl == CH - 1:
            accv[...] = jnp.concatenate(acc, axis=1)
            ocv[...] = oheads(HL, H)
            assert not vq
            return None
        return finish(ci, sl, acc)

    def out_cp(*idx):
        return pltpu.make_async_copy(outv.at[idx], out_hbm.at[idx], sem_out.at[0])

    def chunk(ci, carry):
        prev = jnp.maximum(ci - 1, 0)
        mem = finish_last(prev)

        @pl.when(ci >= 1)
        def _():
            out_cp(prev, pl.ds(2, 2)).start()

        for sl in range(CH):
            mem = step(ci, sl, mem)
            if sl == 1:
                out_cp(ci, pl.ds(0, 2)).start()
        return carry

    lax.fori_loop(0, NCH, chunk, 0)
    o2 = ocv[...].astype(bf16)
    for j in range(NJ):
        c0, c1 = j * 128, (j + 1) * 128
        t = _dot(o2, _tob(wo[j, HL * 64:, :])) + accv[:, c0:c1]
        finalize(NCH - 1, CH - 1, 8, SEG, t[8:32], c0, c1)
        finalize(NCH - 1, CH - 1, 0, 8, t[32:40], c0, c1)
        finalize(NCH - 1, CH - 2, 0, 8, t[40:48], c0, c1)
        out_cp(NCH - 1, pl.ds(2, 2), slice(None), pl.ds(c0, 128)).start()
    pltpu.make_async_copy(outv, out_hbm, sem_out.at[0]).wait()


@jax.jit
def pallas_recurrent_scan__memory_aug_recurrent_mem_tr__moe_arch_mod__prompt_kernel(
    A_x, A_mem0, A_Wq, A_Wk, A_Wv, A_Wo, A_seg_len, B_x, B_w_r, B_w_gate, B_w_up, B_w_down,
):
    hbm = pl.BlockSpec(memory_space=pltpu.MemorySpace.HBM)
    out = pl.pallas_call(
        _kernel,
        out_shape=jax.ShapeDtypeStruct((NCH, CH, SEG, D), bf16),
        in_specs=[hbm] * 10,
        out_specs=hbm,
        scratch_shapes=[
            pltpu.VMEM((NCH, CH, SEG, D), bf16),
            pltpu.VMEM((NCH, CH * 16, D), u32),
            pltpu.VMEM((4, 64, D), u32),
            pltpu.VMEM((NCH, CH * SEG, D), f32),
            pltpu.VMEM((NU, D, 128), u32),
            pltpu.VMEM((NU * 2, D // 2, 128), u32),
            pltpu.VMEM((NJ, H * DH // 2, 128), u32),
            pltpu.VMEM((NU, NCH, CH * 16, 128), f32),
            pltpu.VMEM((2 * NP, 352, 128), f32),
            pltpu.VMEM((4, 64, 80), f32),
            pltpu.VMEM((F, D), bf16),
            pltpu.VMEM((F, D), bf16),
            pltpu.VMEM((F, D), bf16),
            pltpu.VMEM((NCH, CH, SEG, D), bf16),
            pltpu.VMEM((64, 80), f32),
            pltpu.VMEM((48, D), f32),
            pltpu.VMEM((48, (H - HL) * DH), f32),
            pltpu.VMEM((NPL, 8, 128), f32),
            pltpu.VMEM((8, 1024), f32),
            pltpu.VMEM((M, D), bf16),
            pltpu.VMEM((D,), bf16),
            pltpu.SemaphoreType.DMA((len(GROUPS),)),
            pltpu.SemaphoreType.DMA((1,)),
        ],
        compiler_params=pltpu.CompilerParams(
            vmem_limit_bytes=100 * 1024 * 1024,
            disable_bounds_checks=True,
            disable_semaphore_checks=True,
            internal_scratch_in_bytes=48 * 1024,
        ),
        name="rmt_mod",
    )(A_x.reshape(NCH, CH, SEG, D), A_mem0.reshape(M, D), A_Wq, A_Wk, A_Wv, A_Wo.reshape(H * DH, D),
      B_w_r, B_w_gate.T, B_w_up.T, B_w_down)
    return out.reshape(1, S, D)
```

```python
import math

import jax
import jax.numpy as jnp
from jax import lax
import jax.experimental.pallas as pl
import jax.experimental.pallas.tpu as pltpu

bf16 = jnp.bfloat16
f32 = jnp.float32
u32 = jnp.uint32
i32 = jnp.int32

S = 2048
D = 640
H = 32
DH = 128
NP = H // 2
NU = NP * 3
M = 8
SEG = 32
NSEG = S // SEG
F = 1728
C = 8
CH = 4
NCH = NSEG // CH
NJ = D // 128
EPS = 1e-5
NEG = -1e30
LOG2E = math.log2(math.e)
CEXP = (DH ** -0.5) * LOG2E
NT = (((1,), (1,)), ((), ()))

LAG_B, POS_B = 1, 6
LAG_D, POS_D = 3, 4
POS_B0 = (6, 6, 5, 5)
KMAJ = (4, 4, 4, 5)
MORDS = ((1, 0, 2), (1, 0, 2), (1, 0, 2), (1, 0, 2))
EBS = ((0, 6, 12, 20, 21, 32), (0, 9, 14, 18, 22, 27, 32), (0, 8, 15, 17, 25, 32), (0, 8, 14, 19, 23, 28))
EPOS = ((4, 2), (2, 3), (4, 4), (4, 2))
HL = EBS[CH - 1][-1]
NV2 = (8, 2)
VGB = ((0, 5, 11, 16), (0, 5, 11, 17, 24))
LAG_V = 11
TIE_KT = ((3, 0, 0, 0, 0, 3), (0, 0, 4, 0, 0, 3))
TIE_W, TIE_E = 2, 7
E_RATE, E_SKIP = 0.6, 0

NPL = 4
UPL = 8
U0 = 9
CPL = NCH // NPL
SPL = NSEG // NPL
HEAD_GROUPS = (("p0",), ("w0", "p1"), ("w1", "p2", "p3"), ("w2", "w3", "w4"),
               ("mem0", "wr", "w5", "w6", "w7", "w8"))
HOLD = (0, 0, 0, 2, 2)
LOOP_GROUPS = tuple(
    tuple("w%d" % u for u in range(U0 + i * UPL, U0 + (i + 1) * UPL)) + ("x%d" % i,) for i in range(NPL))
TAIL_GROUPS = (tuple("w%d" % u for u in range(U0 + NPL * UPL, NU)) + ("f0", "f1", "f2"),
               tuple("o%d" % j for j in range(NJ)))
GROUPS = HEAD_GROUPS + LOOP_GROUPS + TAIL_GROUPS
TIE_LAG = 6
LN_NUM, LN_DEN = 6, 7
FFN_SKIP = 16


def _tob(x):
    return pltpu.bitcast(x, bf16)


def _tou(x):
    return pltpu.bitcast(x, u32)


def _zero_of(x):
    return (pltpu.bitcast(x, u32) >> 16) >> 16


def _rb(x):
    return x.astype(bf16).astype(f32)


def _layernorm(x, tie=None):
    ps = x[:, 0:128]
    if tie is not None:
        ps = ps + tie
    for j in range(1, NJ):
        ps = ps + x[:, j * 128:(j + 1) * 128]
    mu = jnp.sum(ps, axis=-1, keepdims=True) * (1.0 / D)
    xc = x - mu
    var = jnp.sum(xc * xc, axis=-1, keepdims=True) * (1.0 / D)
    den = _rb(jnp.sqrt(_rb(_rb(var) + EPS)))
    return (_rb(x - _rb(mu)) * pl.reciprocal(den, approx=False, full_range=False)).astype(bf16)


def _sigmoid(z):
    return pl.reciprocal(1.0 + jnp.exp2(z * (-LOG2E)), approx=True)


def _silu(z):
    return z * _sigmoid(z)


def _dot(a, b):
    return jnp.dot(a, b, preferred_element_type=f32)


def _dot_t(a, b):
    return lax.dot_general(a, b, NT, preferred_element_type=f32)


def _kernel(x_hbm, mem0_hbm, wq_hbm, wk_hbm, wv_hbm, wo_hbm, wr_hbm, wg_hbm, wu_hbm, wd_hbm,
            out_hbm,
            xv, lhs, xpre, zbuf, raw, wqkv, wo, pre, stg, sst, wg, wu, wd, outv, mask_ref,
            accv, rds, wr8, mem0_v, wr_v, sem, sem_out):
    w32 = [w.bitcast(u32) for w in (wq_hbm, wk_hbm, wv_hbm)]
    wo32 = wo_hbm.bitcast(u32)

    def src_dst(name):
        if name == "mem0":
            return mem0_hbm, mem0_v
        if name == "wr":
            return wr_hbm, wr_v
        k, n = name[0], int(name[1:])
        if k == "x":
            idx = (pl.ds(n * CPL, CPL), slice(None), pl.ds(8, SEG - 8), slice(None))
            return x_hbm.at[idx], xv.at[idx]
        if k == "p":
            idx = (pl.ds(n * 4, 4), slice(None), pl.ds(0, 8), slice(None))
            return x_hbm.at[idx], xv.at[idx]
        if k == "w":
            return w32[n % 3].at[:, n // 3, :], raw.at[n]
        if k == "f":
            return ((wg_hbm, wg), (wu_hbm, wu), (wd_hbm, wd))[n]
        return wo32.at[:, pl.ds(n * 128, 128)], wo.at[n]

    cps = [[pltpu.make_async_copy(*src_dst(nm), sem.at[gi]) for nm in grp]
           for gi, grp in enumerate(GROUPS)]
    for grp in cps:
        for cp in grp:
            cp.start()

    rr = lax.broadcasted_iota(i32, (64, 80), 0)
    hr = jnp.where(rr < 32, 0, 1)
    pr = jnp.where((rr & 31) < 8, rr & 31, (rr & 31) + 8)
    cc = lax.broadcasted_iota(i32, (64, 80), 1)
    hc = jnp.where(cc < 40, 0, 1)
    pc = cc - 40 * hc
    mask_ref[...] = jnp.where((hr == hc) & ((pr < M) | (pr >= pc)), 1.0, 0.0).astype(f32)

    def orow(h, r0, n):
        r0 += 240 + (h % 2) * 32 if h < H else 304 + (h % 2) * 16
        return ((h % H) // 2, slice(r0, r0 + n), slice(None))

    def o48(h0, h1):
        return jnp.concatenate([jnp.concatenate([stg[orow(h, 0, 32)], stg[orow(H + h, 0, 16)]], axis=0)
                                for h in range(h0, h1)], axis=1)

    st = {}
    lane8 = lax.broadcasted_iota(i32, (8, 128), 1)
    sub8 = lax.broadcasted_iota(i32, (8, 128), 0)

    def ln_pre(b):
        xb = xv[b * 4:(b + 1) * 4, :, 0:8, :].astype(f32).reshape(128, D)
        xpre[b] = _tou(_layernorm(xb))

    def repack(u):
        ev = raw[u, pl.ds(0, D // 2, stride=2), :]
        od = raw[u, pl.ds(1, D // 2, stride=2), :]
        ws = ((ev & jnp.uint32(0xFFFF)) | (od << 16), (ev >> 16) | (od & jnp.uint32(0xFFFF0000)))
        wqkv[2 * u] = ws[0]
        wqkv[2 * u + 1] = ws[1]
        return ws

    def pre_dots(u, b, hook, ws=None):
        xu = xpre[b]
        res = []
        for hh in range(2):
            tie = hook()
            xt = xu
            if tie is not None:
                top = jnp.concatenate([xu[0:8, 0:128] ^ tie, xu[0:8, 128:]], axis=1)
                xt = jnp.concatenate([top, xu[8:]], axis=0)
            w = wqkv[2 * u + hh] if ws is None else ws[hh]
            res.append(_dot(_tob(xt), _tob(w)))
            st["after"] = res[-1][0:8]
        parts = []
        for k in range(16):
            parts += [res[0][k * 8:(k + 1) * 8], res[1][k * 8:(k + 1) * 8]]
        pre[u, b * 4:(b + 1) * 4] = jnp.concatenate(parts, axis=0).reshape(4, CH * 16, 128)

    def score(i, gl, xn32):
        zbuf[i * CPL + gl // 16, (gl % 16) * 8:(gl % 16) * 8 + 8, :] = xn32
        rc = jnp.sum(xn32 * st["wr"], axis=-1, keepdims=True)
        st["rd"] = jnp.where(lane8 == gl, rc, st["rd"])

    def ln_group(i, s, k):
        tie = None
        if st["after"] is not None:
            tie = pltpu.bitcast(_zero_of(st["after"]), f32)
        xn = _layernorm(xv[i * CPL + s // CH, s % CH, k * 8:(k + 1) * 8, :].astype(f32), tie)
        score(i, s * 4 + k, xn.astype(f32))
        if k == 1 and s % 2 == 0:
            xp = _tob(xpre[i, s * 4:s * 4 + 8, :]).astype(f32)
            score(i, s * 4, xp[0:8])
            score(i, s * 4 + 4, xp[8:16])
        if k == 2:
            st["xn2"] = xn
        else:
            r0 = (s % CH) * 16 + (k // 2) * 8
            pair = jnp.concatenate([xn if k == 1 else st["xn2"], xn], axis=0)
            lhs[i * CPL + s // CH, r0:r0 + 8, :] = _tou(pair)
        return _zero_of(st["rd"])

    def topk():
        rd = _rb(rds[...].reshape(NPL * 8, 128))
        rd = jnp.where(rd == 0.0, 0.0, rd)
        bits = pltpu.bitcast(rd, i32)
        mono = jnp.where(bits < 0, bits ^ jnp.int32(0x7FFFFFFF), bits)
        rowid = jnp.concatenate([lane8 * 8 + sub8 + i * SPL * SEG for i in range(NPL)], axis=0)
        key = ((((mono >> 16) + 32768) << 11) | (S - 1 - rowid)) | jnp.int32(0x20000000)
        key = jnp.where(jnp.concatenate([lane8] * NPL, axis=0) < SPL * 4, pltpu.bitcast(key, f32), 0.0)
        row8 = lax.broadcasted_iota(i32, (8, 1), 0)
        ksel = jnp.zeros((8, 1), f32)
        for t in range(C):
            km = jnp.max(jnp.max(key, axis=0, keepdims=True), axis=1, keepdims=True)
            key = jnp.where(key == km, 0.0, key)
            ksel = jnp.where(row8 == t, km, ksel)
        ksel = pltpu.bitcast(ksel, i32)
        iv = S - 1 - (ksel & (S - 1))
        idxs = [iv[t, 0] for t in range(C)]
        xs = jnp.concatenate([zbuf[i_ >> 7, pl.ds(i_ & 127, 1), :] for i_ in idxs], axis=0)
        hi16 = (((ksel >> 11) & 65535) - 32768) << 16
        rbits = jnp.where(hi16 < 0, hi16 ^ jnp.int32(0x7FFF0000), hi16)
        return idxs, xs, _rb(_sigmoid(pltpu.bitcast(rbits, f32)))

    def ffn_tasks(idxs, xs, rsel):
        cols = [(k * 128, min(F, (k + 1) * 128)) for k in range(pl.cdiv(F, 128))]
        xsb = xs.astype(bf16)
        hid = []
        tmp = {}

        def gate(a, b):
            tmp["g"] = _rb(_dot_t(xsb, wg[a:b, :]))

        def up(a, b):
            hid.append((_rb(_silu(tmp["g"])) * _rb(_dot_t(xsb, wu[a:b, :]))).astype(bf16))

        def down(k):
            t = _dot(hid[k], wd[cols[k][0]:cols[k][1], :])
            tmp["y"] = t if k == 0 else t + tmp["y"]

        def fin():
            zs = _rb(xs + _rb(_rb(tmp["y"]) * rsel))
            for t in range(C):
                zbuf[idxs[t] >> 7, pl.ds(idxs[t] & 127, 1), :] = zs[t:t + 1]

        tasks = []
        for a, b in cols:
            tasks += [lambda a=a, b=b: gate(a, b), lambda a=a, b=b: up(a, b)]
        tasks += [lambda k=k: down(k) for k in range(len(cols))]
        return tasks + [fin]

    def run_region(work, side=(), tasks=(), skip=0):
        side, tasks = list(side), list(tasks)
        ties = []
        st["after"] = None
        cnt = {"dot": 0, "credit": 0}

        def hook():
            di = cnt["dot"]
            cnt["dot"] += 1
            if tasks and di >= skip:
                tasks.pop(0)()
            tie = None
            if ties and ties[0][0] <= di:
                tie = ties.pop(0)[1]
            if side and di + TIE_LAG < 2 * len(work):
                cnt["credit"] += LN_NUM
                if cnt["credit"] >= LN_DEN:
                    cnt["credit"] -= LN_DEN
                    ties.append((di + TIE_LAG, ln_group(*side.pop(0))))
            return tie

        for u, b, *ws in work:
            pre_dots(u, b, hook, *ws)
        assert not ties and not side and not tasks

    pending = []
    units, blocks = [], []
    for gi, grp in enumerate(HEAD_GROUPS):
        for cp in cps[gi]:
            cp.wait()
        for u in [int(nm[1:]) for nm in grp if nm[0] == "w" and nm != "wr"]:
            repack(u)
            pending += [(u, b) for b in blocks]
            units.append(u)
        for b in [int(nm[1:]) for nm in grp if nm[0] == "p"]:
            ln_pre(b)
            pending += [(u, b) for u in units]
            blocks.append(b)
        if "mem0" in grp:
            accv[...] = jnp.concatenate([mem0_v[...].astype(f32), jnp.zeros((40, D), f32)], axis=0)
            for h in range(HL, H):
                stg[orow(h, 0, 32)] = jnp.zeros((32, 128), f32)
                stg[orow(H + h, 0, 16)] = jnp.zeros((16, 128), f32)
            wr8[:, 0:D] = jnp.broadcast_to(wr_v[...].astype(f32).reshape(1, D), (8, D))
        n = len(pending) - HOLD[gi]
        work, pending = pending[:n], pending[n:]
        run_region(work)
    assert pending == [(U0 - 1, 2), (U0 - 1, 3)]

    def pro_body(i, carry):
        ub = U0 + i * UPL
        for k in range(UPL):
            pltpu.make_async_copy(w32[0].at[:, 0, :], raw.at[ub + k], sem.at[len(HEAD_GROUPS) + i]).wait()
        idx = (pl.ds(i * CPL, CPL), slice(None), pl.ds(8, SEG - 8), slice(None))
        pltpu.make_async_copy(x_hbm.at[idx], xv.at[idx], sem.at[len(HEAD_GROUPS) + i]).wait()
        ws = [None] + [repack(ub + k) for k in range(UPL)]
        work = [(ub - 1 + k // 4, k % 4, ws[k // 4]) for k in range(2, 2 + 4 * UPL)]
        st["wr"] = wr8[:, 0:D]
        st["rd"] = jnp.zeros((8, 128), f32)
        run_region(work, side=[(i, s, k) for s in range(SPL) for k in (1, 2, 3)])
        rds[i] = st["rd"]
        return carry

    lax.fori_loop(0, NPL, pro_body, 0)

    for cp in cps[-2]:
        cp.wait()
    ub = U0 + NPL * UPL
    for u in range(ub, NU):
        repack(u)
    run_region([(ub - 1 + k // 4, k % 4) for k in range(2, 4 + 4 * (NU - ub))],
               tasks=ffn_tasks(*topk()), skip=FFN_SKIP)
    for cp in cps[-1]:
        cp.wait()

    sub4 = lax.broadcasted_iota(i32, (8, D), 0) < 4

    def finalize(ci, sl, r0, r1, sv, c0=0, c1=D):
        xr = xv[ci, sl, r0:r1, c0:c1].astype(f32)
        g = _silu(zbuf[ci, sl * SEG + r0:sl * SEG + r1, c0:c1])
        outv[ci, sl, r0:r1, c0:c1] = (xr + sv * g).astype(bf16)

    def finish(ci, sl, acc):
        acc = jnp.concatenate(acc, axis=1)
        finalize(ci, sl, 8, SEG, acc[8:32])
        if sl % 2 == 1:
            finalize(ci, sl, 0, 8, acc[32:40])
            finalize(ci, sl - 1, 0, 8, acc[40:48])
        return _tou(acc[0:16].astype(bf16))

    def finish_last(ci):
        o2 = o48(HL, H).astype(bf16)
        acc = [_dot(o2, _tob(wo[j, HL * 64:, :])) + accv[:, j * 128:(j + 1) * 128] for j in range(NJ)]
        return finish(ci, CH - 1, acc)

    vq = []
    clock = [0]

    def vnext():
        ready = [i for i, t in enumerate(vq) if t[0] <= clock[0]]
        if not ready:
            return None
        return vq.pop(min(ready, key=lambda i: (vq[i][2], i)))[1]()

    def vforce(deadline):
        for t in [t for t in vq if t[2] <= deadline]:
            vq.remove(t)
            t[1]()

    def tied(w, g):
        tie = vnext()
        if tie is None:
            return w
        parts = [w[0:g * 8], w[g * 8:g * 8 + 8] ^ tie, w[g * 8 + 8:]]
        return jnp.concatenate([t for t in parts if t.shape[0]], axis=0)

    def step(ci, sl, mem):
        xu = lhs[ci, sl * 16:(sl + 1) * 16, :]
        x = _tob(jnp.concatenate([jnp.where(sub4, mem, xu[0:8]), xu[8:16]], axis=0))
        mord, eb, odd = MORDS[sl], EBS[sl], sl % 2
        probs = {}
        vs = {}
        attended = set()

        early = {}
        for k in range(NJ):
            clock[0] += 1
            for d in range(KMAJ[sl]):
                key = (d // 6, mord[(d % 6) // 2], d % 2)
                w = wqkv[2 * (key[0] * 3 + key[1]) + key[2], k * 64:(k + 1) * 64, :]
                if d == 3 and odd:
                    w = tied(w, TIE_W)
                t = _dot(x[:, k * 128:(k + 1) * 128], _tob(w))
                early[key] = t if k == 0 else t + early[key]

        def slot_of(p, m, hh):
            return m * 2 + hh

        def project(p, di):
            m, hh = mord[di // 2], di % 2
            if (p, m, hh) in early:
                r = early[p, m, hh]
            else:
                clock[0] += 1
                r = _dot(x, _tob(tied(wqkv[2 * (p * 3 + m) + hh], TIE_KT[odd][di] * 8 + TIE_W)))
            b0 = slot_of(p, m, hh) * 40
            stg[odd * NP + p, b0:b0 + 8, :] = r[0:8]
            stg[odd * NP + p, b0 + 16:b0 + 40, :] = r[8:32]
            if m > 0:
                stg[odd * NP + p, b0 + 8:b0 + 16, :] = pre[p * 3 + m, ci, sl * 16 + hh * 8:sl * 16 + hh * 8 + 8, :]

        def mxu_rows(p, a):
            if p < NV2[odd]:
                return jnp.concatenate([a[0:8], a[32:40], a[16:32], a[48:64]], axis=0)
            return a

        def operand(p, m):
            b0 = slot_of(p, m, 0) * 40
            if m > 0:
                a = stg[odd * NP + p, b0:b0 + 80, :]
            else:
                a = mxu_rows(p, jnp.concatenate([stg[odd * NP + p, b0:b0 + 8, :], stg[odd * NP + p, b0 + 16:b0 + 48, :],
                                                 stg[odd * NP + p, b0 + 56:b0 + 80, :]], axis=0))
            return a.astype(bf16)

        def vpu_rows(p, hh, lv, g):
            gb = VGB[lv]
            r0 = sl * 16 + hh * 8

            def row(m, i):
                b0 = slot_of(p, m, hh) * 40 + 8 + 8 * lv - i
                return stg[odd * NP + p, b0:b0 + 8, :]

            if g == 0:
                q = pre[p * 3, ci, r0:r0 + 8, :] if lv == 0 else row(0, 0)
                vs[p, hh, lv] = (q * CEXP, None, None, None)
            q, m_old, l, o = vs[p, hh, lv]
            i0, n = gb[g], gb[g + 1] - gb[g]

            def rows(m):
                return jnp.concatenate([row(m, i0 + i) for i in range(n)], axis=0).reshape(n, 8, 128)

            s = jnp.sum(q[None] * rows(1), axis=-1, keepdims=True)
            if i0 + n > 9 + 8 * lv:
                ok = (lax.broadcasted_iota(i32, (n, 8, 1), 1)
                      >= lax.broadcasted_iota(i32, (n, 8, 1), 0) + (i0 - 8 - 8 * lv))
                s = jnp.where(ok, s, NEG)
            mx = jnp.max(s, axis=0)
            if m_old is not None:
                mx = jnp.maximum(mx, m_old)
            e = jnp.exp2(s - mx[None])
            el, ev = jnp.sum(e, axis=0), jnp.sum(e * rows(2), axis=0)
            if m_old is None:
                l, o = el, ev
            else:
                alpha = jnp.exp2(m_old - mx)
                l, o = l * alpha + el, o * alpha + ev
            if g == len(gb) - 2:
                o = o * pl.reciprocal(l, approx=True)
                if lv == 0:
                    stg[orow(H + 2 * p + hh, (1 - odd) * 8, 8)] = o
                else:
                    stg[orow(2 * p + hh, 8, 8)] = o
            vs[p, hh, lv] = (q, mx, l, o)
            return _zero_of(o)

        def scores(p):
            if not 0 <= p < NP:
                return
            sc = jnp.where(mxu_rows(p, mask_ref[...]) > 0.5, _dot_t(operand(p, 0), operand(p, 1)), NEG)
            n = sc.shape[0]
            mx = jnp.max(sc, axis=-1, keepdims=True)
            sst[p % 2, 0:n] = sc
            e = jnp.exp2((sst[p % 2, 0:n] - mx) * CEXP)
            l = jnp.sum(e, axis=-1, keepdims=True)
            sst[2 + p % 2, 0:n] = e
            probs[p] = (sst[2 + p % 2, 0:n] * pl.reciprocal(l, approx=True)).astype(bf16)

        def attend(p):
            if not 0 <= p < NP:
                return
            o = _dot(probs[p], operand(p, 2))
            attended.add(p)
            for hh in range(2):
                if p < NV2[odd]:
                    stg[orow(2 * p + hh, 0, 8)] = o[hh * 8:hh * 8 + 8]
                    stg[orow(2 * p + hh, 16, 16)] = o[16 + hh * 16:32 + hh * 16]
                else:
                    stg[orow(2 * p + hh, 0, 32)] = o[hh * 32:(hh + 1) * 32]

        def oheads(h0, h1):
            assert (h1 - 1) // 2 in attended
            vforce((sl, h1 - 1))
            if not odd:
                return jnp.concatenate([stg[orow(h, 0, 32)] for h in range(h0, h1)], axis=1)
            return o48(h0, h1)

        for slot in range(NP):
            for di in range(7):
                if di == (POS_B0[sl] if slot == LAG_B else POS_B):
                    scores(slot - LAG_B)
                if di == POS_D:
                    attend(slot - LAG_D)
                if di < 6:
                    project(slot, di)
            for hh in range(2):
                for lv in ((1, 0) if slot < NV2[odd] else (0,)):
                    for g in range(len(VGB[lv]) - 1):
                        vq.append((clock[0] + LAG_V, lambda a=(slot, hh, lv, g): vpu_rows(*a),
                                   (sl if lv == 1 else sl | 1, 2 * slot + hh)))
        tiles, credit = 0, 0.0
        acc = [None] * NJ
        for i in range(len(eb) - 1):
            h0, h1 = eb[i], eb[i + 1]
            o2 = oheads(h0, h1).astype(bf16)
            for j in range(NJ):
                ws = []
                for h in range(h0, h1):
                    tiles += 1
                    if tiles % (3 if odd else 5) == 0:
                        clock[0] += 1
                    w = wo[j, h * 64:(h + 1) * 64, :]
                    if odd and tiles > E_SKIP:
                        credit += E_RATE
                        if credit >= 1.0:
                            credit -= 1.0
                            w = tied(w, TIE_E)
                    ws.append(w)
                t = _dot(o2, _tob(jnp.concatenate(ws, axis=0)))
                acc[j] = t if acc[j] is None else t + acc[j]
                if j == EPOS[sl][0]:
                    scores(NP + i - LAG_B)
                if j == EPOS[sl][1]:
                    attend(NP + i - LAG_D)
        if sl == CH - 1:
            accv[...] = jnp.concatenate(acc, axis=1)
            vforce((sl, H))
            assert not vq and len(attended) == NP
            return None
        return finish(ci, sl, acc)

    def out_cp(*idx):
        return pltpu.make_async_copy(outv.at[idx], out_hbm.at[idx], sem_out.at[0])

    def chunk(ci, carry):
        prev = jnp.maximum(ci - 1, 0)
        mem = finish_last(prev)

        @pl.when(ci >= 1)
        def _():
            out_cp(prev, pl.ds(2, 2)).start()

        for sl in range(CH):
            mem = step(ci, sl, mem)
            if sl == 1:
                out_cp(ci, pl.ds(0, 2)).start()
        return carry

    lax.fori_loop(0, NCH, chunk, 0)
    o2 = o48(HL, H).astype(bf16)
    for j in range(NJ):
        c0, c1 = j * 128, (j + 1) * 128
        t = _dot(o2, _tob(wo[j, HL * 64:, :])) + accv[:, c0:c1]
        finalize(NCH - 1, CH - 1, 8, SEG, t[8:32], c0, c1)
        finalize(NCH - 1, CH - 1, 0, 8, t[32:40], c0, c1)
        finalize(NCH - 1, CH - 2, 0, 8, t[40:48], c0, c1)
        out_cp(NCH - 1, pl.ds(2, 2), slice(None), pl.ds(c0, 128)).start()
    pltpu.make_async_copy(outv, out_hbm, sem_out.at[0]).wait()


@jax.jit
def pallas_recurrent_scan__memory_aug_recurrent_mem_tr__moe_arch_mod__prompt_kernel(
    A_x, A_mem0, A_Wq, A_Wk, A_Wv, A_Wo, A_seg_len, B_x, B_w_r, B_w_gate, B_w_up, B_w_down,
):
    hbm = pl.BlockSpec(memory_space=pltpu.MemorySpace.HBM)
    out = pl.pallas_call(
        _kernel,
        out_shape=jax.ShapeDtypeStruct((NCH, CH, SEG, D), bf16),
        in_specs=[hbm] * 10,
        out_specs=hbm,
        scratch_shapes=[
            pltpu.VMEM((NCH, CH, SEG, D), bf16),
            pltpu.VMEM((NCH, CH * 16, D), u32),
            pltpu.VMEM((4, 64, D), u32),
            pltpu.VMEM((NCH, CH * SEG, D), f32),
            pltpu.VMEM((NU, D, 128), u32),
            pltpu.VMEM((NU * 2, D // 2, 128), u32),
            pltpu.VMEM((NJ, H * DH // 2, 128), u32),
            pltpu.VMEM((NU, NCH, CH * 16, 128), f32),
            pltpu.VMEM((2 * NP, 352, 128), f32),
            pltpu.VMEM((4, 64, 80), f32),
            pltpu.VMEM((F, D), bf16),
            pltpu.VMEM((F, D), bf16),
            pltpu.VMEM((F, D), bf16),
            pltpu.VMEM((NCH, CH, SEG, D), bf16),
            pltpu.VMEM((64, 80), f32),
            pltpu.VMEM((48, D), f32),
            pltpu.VMEM((NPL, 8, 128), f32),
            pltpu.VMEM((8, 1024), f32),
            pltpu.VMEM((M, D), bf16),
            pltpu.VMEM((D,), bf16),
            pltpu.SemaphoreType.DMA((len(GROUPS),)),
            pltpu.SemaphoreType.DMA((1,)),
        ],
        compiler_params=pltpu.CompilerParams(
            vmem_limit_bytes=100 * 1024 * 1024,
            disable_bounds_checks=True,
            disable_semaphore_checks=True,
            internal_scratch_in_bytes=48 * 1024,
        ),
        name="rmt_mod",
    )(A_x.reshape(NCH, CH, SEG, D), A_mem0.reshape(M, D), A_Wq, A_Wk, A_Wv, A_Wo.reshape(H * DH, D),
      B_w_r, B_w_gate.T, B_w_up.T, B_w_down)
    return out.reshape(1, S, D)
```

```python
import math

import jax
import jax.numpy as jnp
from jax import lax
import jax.experimental.pallas as pl
import jax.experimental.pallas.tpu as pltpu

bf16 = jnp.bfloat16
f32 = jnp.float32
u32 = jnp.uint32
i32 = jnp.int32

S = 2048
D = 640
H = 32
DH = 128
NP = H // 2
NU = NP * 3
M = 8
SEG = 32
NSEG = S // SEG
F = 1728
C = 8
CH = 4
NCH = NSEG // CH
NJ = D // 128
EPS = 1.3125 * 2.0 ** -17
NEG = -1e30
LOG2E = math.log2(math.e)
CEXP = (DH ** -0.5) * LOG2E
NT = (((1,), (1,)), ((), ()))

LAG_B, POS_B = 1, 6
LAG_D, POS_D = 3, 4
POS_B0 = (6, 6, 5, 5)
KMAJ = (4, 4, 4, 5)
MORDS = ((1, 0, 2), (1, 0, 2), (0, 1, 2), (1, 0, 2))
EBS = ((0, 6, 12, 20, 21, 32), (0, 9, 14, 18, 22, 27, 32), (0, 8, 13, 18, 25, 32), (0, 8, 14, 19, 23, 28))
EPOS = ((4, 2), (2, 3), (4, 4), (4, 2))
HL = EBS[CH - 1][-1]
NV2 = (8, 2)
VGB = (((0, 5, 11, 16), (0, 5, 11, 17, 24)), ((0, 5, 11, 16), (0, 5, 11, 17, 24)),
       ((0, 6, 11, 16), (0, 5, 11, 17, 24)), ((0, 6, 11, 16), (0, 6, 12, 18, 24)))
LAG_V = 11
TIE_KT = ((3, 0, 0, 0, 0, 3), (0, 0, 4, 0, 0, 3))
TIE_K = (None, 0, None, 1)
TIE_W, TIE_E = 2, (None, 2, None, 7)
E_RATE = 0.6

NPL = 4
UPL = 8
U0 = 9
CPL = NCH // NPL
SPL = NSEG // NPL
HEAD_GROUPS = (("p0",), ("w0", "p1"), ("w1", "p2", "p3"), ("w2", "w3", "w4"),
               ("mem0", "wr", "w5", "w6", "w7", "w8"))
HOLD = (0, 0, 0, 2, 2)
LOOP_GROUPS = tuple(
    tuple("w%d" % u for u in range(U0 + i * UPL, U0 + (i + 1) * UPL)) + ("x%d" % i,) for i in range(NPL))
TAIL_GROUPS = (tuple("w%d" % u for u in range(U0 + NPL * UPL, NU)) + ("f0", "f1", "f2"),
               tuple("o%d" % j for j in range(NJ)))
GROUPS = HEAD_GROUPS + LOOP_GROUPS + TAIL_GROUPS
TIE_LAG = 6
LN_NUM, LN_DEN = 6, 7
FFN_SKIP = 16


def _tob(x):
    return pltpu.bitcast(x, bf16)


def _tou(x):
    return pltpu.bitcast(x, u32)


def _zero_of(x):
    return (pltpu.bitcast(x, u32) >> 16) >> 16


def _rb(x):
    return x.astype(bf16).astype(f32)


def _layernorm(x, tie=None):
    ps = x[:, 0:128]
    if tie is not None:
        ps = ps + tie
    for j in range(1, NJ):
        ps = ps + x[:, j * 128:(j + 1) * 128]
    mu = jnp.sum(ps, axis=-1, keepdims=True) * (1.0 / D)
    xc = x - mu
    var = jnp.sum(xc * xc, axis=-1, keepdims=True) * (1.0 / D)
    den = _rb(jnp.sqrt(_rb(_rb(var) + EPS)))
    return (_rb(x - _rb(mu)) * pl.reciprocal(den, approx=False, full_range=False)).astype(bf16)


def _sigmoid(z):
    return pl.reciprocal(1.0 + jnp.exp2(z * (-LOG2E)), approx=True)


def _silu(z):
    return z * _sigmoid(z)


def _dot(a, b):
    return jnp.dot(a, b, preferred_element_type=f32)


def _dot_t(a, b):
    return lax.dot_general(a, b, NT, preferred_element_type=f32)


def _kernel(x_hbm, mem0_hbm, wq_hbm, wk_hbm, wv_hbm, wo_hbm, wr_hbm, wg_hbm, wu_hbm, wd_hbm,
            out_hbm,
            xv, lhs, xpre, zbuf, raw, wqkv, wo, pre, stg, sst, wg, wu, wd, outv, mask_ref,
            accv, rds, wr8, mem0_v, wr_v, sem, sem_out):
    w32 = [w.bitcast(u32) for w in (wq_hbm, wk_hbm, wv_hbm)]
    wo32 = wo_hbm.bitcast(u32)

    def src_dst(name):
        if name == "mem0":
            return mem0_hbm, mem0_v
        if name == "wr":
            return wr_hbm, wr_v
        k, n = name[0], int(name[1:])
        if k == "x":
            idx = (pl.ds(n * CPL, CPL), slice(None), pl.ds(8, SEG - 8), slice(None))
            return x_hbm.at[idx], xv.at[idx]
        if k == "p":
            idx = (pl.ds(n * 4, 4), slice(None), pl.ds(0, 8), slice(None))
            return x_hbm.at[idx], xv.at[idx]
        if k == "w":
            return w32[n % 3].at[:, n // 3, :], raw.at[n]
        if k == "f":
            return ((wg_hbm, wg), (wu_hbm, wu), (wd_hbm, wd))[n]
        return wo32.at[:, pl.ds(n * 128, 128)], wo.at[n]

    cps = [[pltpu.make_async_copy(*src_dst(nm), sem.at[gi]) for nm in grp]
           for gi, grp in enumerate(GROUPS)]
    for grp in cps:
        for cp in grp:
            cp.start()

    rr = lax.broadcasted_iota(i32, (64, 80), 0)
    hr = jnp.where(rr < 32, 0, 1)
    pr = jnp.where((rr & 31) < 8, rr & 31, (rr & 31) + 8)
    cc = lax.broadcasted_iota(i32, (64, 80), 1)
    hc = jnp.where(cc < 40, 0, 1)
    pc = cc - 40 * hc
    mask_ref[...] = jnp.where((hr == hc) & ((pr < M) | (pr >= pc)), 1.0, 0.0).astype(f32)

    def orow(h, r0, n):
        r0 += 240 + (h % 2) * 32 if h < H else 304 + (h % 2) * 16
        return ((h % H) // 2, slice(r0, r0 + n), slice(None))

    def o48(h0, h1):
        return jnp.concatenate([jnp.concatenate([stg[orow(h, 0, 32)], stg[orow(H + h, 0, 16)]], axis=0)
                                for h in range(h0, h1)], axis=1)

    st = {}
    lane8 = lax.broadcasted_iota(i32, (8, 128), 1)
    sub8 = lax.broadcasted_iota(i32, (8, 128), 0)

    def ln_pre(b):
        xb = xv[b * 4:(b + 1) * 4, :, 0:8, :].astype(f32).reshape(128, D)
        xpre[b] = _tou(_layernorm(xb))

    def repack(u):
        ev = raw[u, pl.ds(0, D // 2, stride=2), :]
        od = raw[u, pl.ds(1, D // 2, stride=2), :]
        ws = ((ev & jnp.uint32(0xFFFF)) | (od << 16), (ev >> 16) | (od & jnp.uint32(0xFFFF0000)))
        wqkv[2 * u] = ws[0]
        wqkv[2 * u + 1] = ws[1]
        return ws

    def pre_dots(u, b, hook, ws=None):
        xu = xpre[b]
        res = []
        for hh in range(2):
            tie = hook()
            xt = xu
            if tie is not None:
                top = jnp.concatenate([xu[0:8, 0:128] ^ tie, xu[0:8, 128:]], axis=1)
                xt = jnp.concatenate([top, xu[8:]], axis=0)
            w = wqkv[2 * u + hh] if ws is None else ws[hh]
            res.append(_dot(_tob(xt), _tob(w)))
            st["after"] = res[-1][0:8]
        parts = []
        for k in range(16):
            parts += [res[0][k * 8:(k + 1) * 8], res[1][k * 8:(k + 1) * 8]]
        pre[u, b * 4:(b + 1) * 4] = jnp.concatenate(parts, axis=0).reshape(4, CH * 16, 128)

    def score(i, gl, xn32):
        zbuf[i * CPL + gl // 16, (gl % 16) * 8:(gl % 16) * 8 + 8, :] = xn32
        rc = jnp.sum(xn32 * st["wr"], axis=-1, keepdims=True)
        st["rd"] = jnp.where(lane8 == gl, rc, st["rd"])

    def ln_group(i, s, k):
        tie = None
        if st["after"] is not None:
            tie = pltpu.bitcast(_zero_of(st["after"]), f32)
        xn = _layernorm(xv[i * CPL + s // CH, s % CH, k * 8:(k + 1) * 8, :].astype(f32), tie)
        score(i, s * 4 + k, xn.astype(f32))
        if k == 1 and s % 2 == 0:
            xp = _tob(xpre[i, s * 4:s * 4 + 8, :]).astype(f32)
            score(i, s * 4, xp[0:8])
            score(i, s * 4 + 4, xp[8:16])
        if k == 2:
            st["xn2"] = xn
        else:
            r0 = (s % CH) * 16 + (k // 2) * 8
            pair = jnp.concatenate([xn if k == 1 else st["xn2"], xn], axis=0)
            lhs[i * CPL + s // CH, r0:r0 + 8, :] = _tou(pair)
        return _zero_of(st["rd"])

    def topk():
        rd = _rb(rds[...].reshape(NPL * 8, 128))
        rd = jnp.where(rd == 0.0, 0.0, rd)
        bits = pltpu.bitcast(rd, i32)
        mono = jnp.where(bits < 0, bits ^ jnp.int32(0x7FFFFFFF), bits)
        rowid = jnp.concatenate([lane8 * 8 + sub8 + i * SPL * SEG for i in range(NPL)], axis=0)
        key = ((((mono >> 16) + 32768) << 11) | (S - 1 - rowid)) | jnp.int32(0x20000000)
        key = jnp.where(jnp.concatenate([lane8] * NPL, axis=0) < SPL * 4, pltpu.bitcast(key, f32), 0.0)
        row8 = lax.broadcasted_iota(i32, (8, 1), 0)
        ksel = jnp.zeros((8, 1), f32)
        for t in range(C):
            km = jnp.max(jnp.max(key, axis=0, keepdims=True), axis=1, keepdims=True)
            key = jnp.where(key == km, 0.0, key)
            ksel = jnp.where(row8 == t, km, ksel)
        ksel = pltpu.bitcast(ksel, i32)
        iv = S - 1 - (ksel & (S - 1))
        idxs = [iv[t, 0] for t in range(C)]
        xs = jnp.concatenate([zbuf[i_ >> 7, pl.ds(i_ & 127, 1), :] for i_ in idxs], axis=0)
        hi16 = (((ksel >> 11) & 65535) - 32768) << 16
        rbits = jnp.where(hi16 < 0, hi16 ^ jnp.int32(0x7FFF0000), hi16)
        return idxs, xs, _rb(_sigmoid(pltpu.bitcast(rbits, f32)))

    def ffn_tasks(idxs, xs, rsel):
        cols = [(k * 128, min(F, (k + 1) * 128)) for k in range(pl.cdiv(F, 128))]
        xsb = xs.astype(bf16)
        hid = []
        tmp = {}

        def gate(a, b):
            tmp["g"] = _rb(_dot_t(xsb, wg[a:b, :]))

        def up(a, b):
            hid.append((_rb(_silu(tmp["g"])) * _rb(_dot_t(xsb, wu[a:b, :]))).astype(bf16))

        def down(k):
            t = _dot(hid[k], wd[cols[k][0]:cols[k][1], :])
            tmp["y"] = t if k == 0 else t + tmp["y"]

        def fin():
            zs = _rb(xs + _rb(_rb(tmp["y"]) * rsel))
            for t in range(C):
                zbuf[idxs[t] >> 7, pl.ds(idxs[t] & 127, 1), :] = zs[t:t + 1]

        tasks = []
        for a, b in cols:
            tasks += [lambda a=a, b=b: gate(a, b), lambda a=a, b=b: up(a, b)]
        tasks += [lambda k=k: down(k) for k in range(len(cols))]
        return tasks + [fin]

    def run_region(work, side=(), tasks=(), skip=0):
        side, tasks = list(side), list(tasks)
        ties = []
        st["after"] = None
        cnt = {"dot": 0, "credit": 0}

        def hook():
            di = cnt["dot"]
            cnt["dot"] += 1
            if tasks and di >= skip:
                tasks.pop(0)()
            tie = None
            if ties and ties[0][0] <= di:
                tie = ties.pop(0)[1]
            if side and di + TIE_LAG < 2 * len(work):
                cnt["credit"] += LN_NUM
                if cnt["credit"] >= LN_DEN:
                    cnt["credit"] -= LN_DEN
                    ties.append((di + TIE_LAG, ln_group(*side.pop(0))))
            return tie

        for u, b, *ws in work:
            pre_dots(u, b, hook, *ws)
        assert not ties and not side and not tasks

    pending = []
    units, blocks = [], []
    for gi, grp in enumerate(HEAD_GROUPS):
        for cp in cps[gi]:
            cp.wait()
        for u in [int(nm[1:]) for nm in grp if nm[0] == "w" and nm != "wr"]:
            repack(u)
            pending += [(u, b) for b in blocks]
            units.append(u)
        for b in [int(nm[1:]) for nm in grp if nm[0] == "p"]:
            ln_pre(b)
            pending += [(u, b) for u in units]
            blocks.append(b)
        if "mem0" in grp:
            accv[...] = jnp.concatenate([mem0_v[...].astype(f32), jnp.zeros((40, D), f32)], axis=0)
            for h in range(HL, H):
                stg[orow(h, 0, 32)] = jnp.zeros((32, 128), f32)
                stg[orow(H + h, 0, 16)] = jnp.zeros((16, 128), f32)
            wr8[:, 0:D] = jnp.broadcast_to(wr_v[...].astype(f32).reshape(1, D), (8, D))
        n = len(pending) - HOLD[gi]
        work, pending = pending[:n], pending[n:]
        run_region(work)
    assert pending == [(U0 - 1, 2), (U0 - 1, 3)]

    def pro_body(i, carry):
        ub = U0 + i * UPL
        for k in range(UPL):
            pltpu.make_async_copy(w32[0].at[:, 0, :], raw.at[ub + k], sem.at[len(HEAD_GROUPS) + i]).wait()
        idx = (pl.ds(i * CPL, CPL), slice(None), pl.ds(8, SEG - 8), slice(None))
        pltpu.make_async_copy(x_hbm.at[idx], xv.at[idx], sem.at[len(HEAD_GROUPS) + i]).wait()
        ws = [None] + [repack(ub + k) for k in range(UPL)]
        work = [(ub - 1 + k // 4, k % 4, ws[k // 4]) for k in range(2, 2 + 4 * UPL)]
        st["wr"] = wr8[:, 0:D]
        st["rd"] = jnp.zeros((8, 128), f32)
        run_region(work, side=[(i, s, k) for s in range(SPL) for k in (1, 2, 3)])
        rds[i] = st["rd"]
        return carry

    lax.fori_loop(0, NPL, pro_body, 0)

    for cp in cps[-2]:
        cp.wait()
    ub = U0 + NPL * UPL
    for u in range(ub, NU):
        repack(u)
    run_region([(ub - 1 + k // 4, k % 4) for k in range(2, 4 + 4 * (NU - ub))],
               tasks=ffn_tasks(*topk()), skip=FFN_SKIP)
    for cp in cps[-1]:
        cp.wait()

    sub4 = lax.broadcasted_iota(i32, (8, D), 0) < 4

    def finalize(ci, sl, r0, r1, sv, c0=0, c1=D):
        xr = xv[ci, sl, r0:r1, c0:c1].astype(f32)
        g = _silu(zbuf[ci, sl * SEG + r0:sl * SEG + r1, c0:c1])
        outv[ci, sl, r0:r1, c0:c1] = (xr + sv * g).astype(bf16)

    def finish(ci, sl, acc):
        acc = jnp.concatenate(acc, axis=1)
        finalize(ci, sl, 8, SEG, acc[8:32])
        if sl % 2 == 1:
            finalize(ci, sl, 0, 8, acc[32:40])
            finalize(ci, sl - 1, 0, 8, acc[40:48])
        return _tou(acc[0:16].astype(bf16))

    def finish_last(ci):
        o2 = o48(HL, H).astype(bf16)
        acc = [_dot(o2, _tob(wo[j, HL * 64:, :])) + accv[:, j * 128:(j + 1) * 128] for j in range(NJ)]
        return finish(ci, CH - 1, acc)

    vq = []
    clock = [0]

    def vnext():
        ready = [i for i, t in enumerate(vq) if t[0] <= clock[0]]
        if not ready:
            return None
        return vq.pop(min(ready, key=lambda i: (vq[i][2], i)))[1]()

    def vforce(deadline):
        for t in [t for t in vq if t[2] <= deadline]:
            vq.remove(t)
            t[1]()

    def tied(w, g):
        tie = vnext()
        if tie is None:
            return w
        parts = [w[0:g * 8], w[g * 8:g * 8 + 8] ^ tie, w[g * 8 + 8:]]
        return jnp.concatenate([t for t in parts if t.shape[0]], axis=0)

    def step(ci, sl, mem):
        xu = lhs[ci, sl * 16:(sl + 1) * 16, :]
        x = _tob(jnp.concatenate([jnp.where(sub4, mem, xu[0:8]), xu[8:16]], axis=0))
        mord, eb, odd = MORDS[sl], EBS[sl], sl % 2
        probs = {}
        vs = {}
        attended = set()

        early = {}
        for k in range(NJ):
            clock[0] += 1
            for d in range(KMAJ[sl]):
                key = (d // 6, mord[(d % 6) // 2], d % 2)
                w = wqkv[2 * (key[0] * 3 + key[1]) + key[2], k * 64:(k + 1) * 64, :]
                if d == TIE_K[sl]:
                    w = tied(w, TIE_W)
                t = _dot(x[:, k * 128:(k + 1) * 128], _tob(w))
                early[key] = t if k == 0 else t + early[key]

        def slot_of(p, m, hh):
            return m * 2 + hh

        def project(p, di):
            m, hh = mord[di // 2], di % 2
            if (p, m, hh) in early:
                r = early[p, m, hh]
            else:
                clock[0] += 1
                r = _dot(x, _tob(tied(wqkv[2 * (p * 3 + m) + hh], TIE_KT[odd][di] * 8 + TIE_W)))
            b0 = slot_of(p, m, hh) * 40
            stg[odd * NP + p, b0:b0 + 8, :] = r[0:8]
            stg[odd * NP + p, b0 + 16:b0 + 40, :] = r[8:32]
            if m > 0:
                stg[odd * NP + p, b0 + 8:b0 + 16, :] = pre[p * 3 + m, ci, sl * 16 + hh * 8:sl * 16 + hh * 8 + 8, :]

        def mxu_rows(p, a):
            if p < NV2[odd]:
                return jnp.concatenate([a[0:8], a[32:40], a[16:32], a[48:64]], axis=0)
            return a

        def operand(p, m):
            b0 = slot_of(p, m, 0) * 40
            if m > 0:
                a = stg[odd * NP + p, b0:b0 + 80, :]
            else:
                a = mxu_rows(p, jnp.concatenate([stg[odd * NP + p, b0:b0 + 8, :], stg[odd * NP + p, b0 + 16:b0 + 48, :],
                                                 stg[odd * NP + p, b0 + 56:b0 + 80, :]], axis=0))
            return a.astype(bf16)

        def vpu_rows(p, hh, lv, g):
            gb = VGB[sl][lv]
            r0 = sl * 16 + hh * 8

            def row(m, i):
                b0 = slot_of(p, m, hh) * 40 + 8 + 8 * lv - i
                return stg[odd * NP + p, b0:b0 + 8, :]

            if g == 0:
                q = pre[p * 3, ci, r0:r0 + 8, :] if lv == 0 else row(0, 0)
                vs[p, hh, lv] = (q * CEXP, None, None, None)
            q, m_old, l, o = vs[p, hh, lv]
            i0, n = gb[g], gb[g + 1] - gb[g]

            def rows(m):
                return jnp.concatenate([row(m, i0 + i) for i in range(n)], axis=0).reshape(n, 8, 128)

            s = jnp.sum(q[None] * rows(1), axis=-1, keepdims=True)
            if i0 + n > 9 + 8 * lv:
                ok = (lax.broadcasted_iota(i32, (n, 8, 1), 1)
                      >= lax.broadcasted_iota(i32, (n, 8, 1), 0) + (i0 - 8 - 8 * lv))
                s = jnp.where(ok, s, NEG)
            mx = jnp.max(s, axis=0)
            if m_old is not None:
                mx = jnp.maximum(mx, m_old)
            e = jnp.exp2(s - mx[None])
            el, ev = jnp.sum(e, axis=0), jnp.sum(e * rows(2), axis=0)
            if m_old is None:
                l, o = el, ev
            else:
                alpha = jnp.exp2(m_old - mx)
                l, o = l * alpha + el, o * alpha + ev
            if g == len(gb) - 2:
                o = o * pl.reciprocal(l, approx=True)
                if lv == 0:
                    stg[orow(H + 2 * p + hh, (1 - odd) * 8, 8)] = o
                else:
                    stg[orow(2 * p + hh, 8, 8)] = o
            vs[p, hh, lv] = (q, mx, l, o)
            return _zero_of(o)

        def scores(p):
            if not 0 <= p < NP:
                return
            sc = jnp.where(mxu_rows(p, mask_ref[...]) > 0.5, _dot_t(operand(p, 0), operand(p, 1)), NEG)
            n = sc.shape[0]
            mx = jnp.max(sc, axis=-1, keepdims=True)
            sst[p % 2, 0:n] = sc
            e = jnp.exp2((sst[p % 2, 0:n] - mx) * CEXP)
            l = jnp.sum(e, axis=-1, keepdims=True)
            sst[2 + p % 2, 0:n] = e
            probs[p] = (sst[2 + p % 2, 0:n] * pl.reciprocal(l, approx=True)).astype(bf16)

        def attend(p):
            if not 0 <= p < NP:
                return
            o = _dot(probs[p], operand(p, 2))
            attended.add(p)
            for hh in range(2):
                if p < NV2[odd]:
                    stg[orow(2 * p + hh, 0, 8)] = o[hh * 8:hh * 8 + 8]
                    stg[orow(2 * p + hh, 16, 16)] = o[16 + hh * 16:32 + hh * 16]
                else:
                    stg[orow(2 * p + hh, 0, 32)] = o[hh * 32:(hh + 1) * 32]

        def oheads(h0, h1):
            assert (h1 - 1) // 2 in attended
            vforce((sl, h1 - 1))
            if not odd:
                return jnp.concatenate([stg[orow(h, 0, 32)] for h in range(h0, h1)], axis=1)
            return o48(h0, h1)

        for slot in range(NP):
            for di in range(7):
                if di == (POS_B0[sl] if slot == LAG_B else POS_B):
                    scores(slot - LAG_B)
                if di == POS_D:
                    attend(slot - LAG_D)
                if di < 6:
                    project(slot, di)
            for hh in range(2):
                for lv in ((1, 0) if slot < NV2[odd] else (0,)):
                    for g in range(len(VGB[sl][lv]) - 1):
                        vq.append((clock[0] + LAG_V, lambda a=(slot, hh, lv, g): vpu_rows(*a),
                                   (sl if lv == 1 else sl | 1, 2 * slot + hh)))
        tiles, credit = 0, 0.0
        acc = [None] * NJ
        for i in range(len(eb) - 1):
            h0, h1 = eb[i], eb[i + 1]
            o2 = oheads(h0, h1).astype(bf16)
            for j in range(NJ):
                ws = []
                for h in range(h0, h1):
                    tiles += 1
                    if tiles % (3 if odd else 5) == 0:
                        clock[0] += 1
                    w = wo[j, h * 64:(h + 1) * 64, :]
                    if odd:
                        credit += E_RATE
                        if credit >= 1.0:
                            credit -= 1.0
                            w = tied(w, TIE_E[sl])
                    ws.append(w)
                t = _dot(o2, _tob(jnp.concatenate(ws, axis=0)))
                acc[j] = t if acc[j] is None else t + acc[j]
                if j == EPOS[sl][0]:
                    scores(NP + i - LAG_B)
                if j == EPOS[sl][1]:
                    attend(NP + i - LAG_D)
        if sl == CH - 1:
            accv[...] = jnp.concatenate(acc, axis=1)
            vforce((sl, H))
            assert not vq and len(attended) == NP
            return None
        return finish(ci, sl, acc)

    def out_cp(*idx):
        return pltpu.make_async_copy(outv.at[idx], out_hbm.at[idx], sem_out.at[0])

    def chunk(ci, carry):
        prev = jnp.maximum(ci - 1, 0)
        mem = finish_last(prev)

        @pl.when(ci >= 1)
        def _():
            out_cp(prev, pl.ds(2, 2)).start()

        for sl in range(CH):
            mem = step(ci, sl, mem)
            if sl == 1:
                out_cp(ci, pl.ds(0, 2)).start()
        return carry

    lax.fori_loop(0, NCH, chunk, 0)
    o2 = o48(HL, H).astype(bf16)
    for j in range(NJ):
        c0, c1 = j * 128, (j + 1) * 128
        t = _dot(o2, _tob(wo[j, HL * 64:, :])) + accv[:, c0:c1]
        finalize(NCH - 1, CH - 1, 8, SEG, t[8:32], c0, c1)
        finalize(NCH - 1, CH - 1, 0, 8, t[32:40], c0, c1)
        finalize(NCH - 1, CH - 2, 0, 8, t[40:48], c0, c1)
        out_cp(NCH - 1, pl.ds(2, 2), slice(None), pl.ds(c0, 128)).start()
    pltpu.make_async_copy(outv, out_hbm, sem_out.at[0]).wait()


@jax.jit
def pallas_recurrent_scan__memory_aug_recurrent_mem_tr__moe_arch_mod__prompt_kernel(
    A_x, A_mem0, A_Wq, A_Wk, A_Wv, A_Wo, A_seg_len, B_x, B_w_r, B_w_gate, B_w_up, B_w_down,
):
    hbm = pl.BlockSpec(memory_space=pltpu.MemorySpace.HBM)
    out = pl.pallas_call(
        _kernel,
        out_shape=jax.ShapeDtypeStruct((NCH, CH, SEG, D), bf16),
        in_specs=[hbm] * 10,
        out_specs=hbm,
        scratch_shapes=[
            pltpu.VMEM((NCH, CH, SEG, D), bf16),
            pltpu.VMEM((NCH, CH * 16, D), u32),
            pltpu.VMEM((4, 64, D), u32),
            pltpu.VMEM((NCH, CH * SEG, D), f32),
            pltpu.VMEM((NU, D, 128), u32),
            pltpu.VMEM((NU * 2, D // 2, 128), u32),
            pltpu.VMEM((NJ, H * DH // 2, 128), u32),
            pltpu.VMEM((NU, NCH, CH * 16, 128), f32),
            pltpu.VMEM((2 * NP, 352, 128), f32),
            pltpu.VMEM((4, 64, 80), f32),
            pltpu.VMEM((F, D), bf16),
            pltpu.VMEM((F, D), bf16),
            pltpu.VMEM((F, D), bf16),
            pltpu.VMEM((NCH, CH, SEG, D), bf16),
            pltpu.VMEM((64, 80), f32),
            pltpu.VMEM((48, D), f32),
            pltpu.VMEM((NPL, 8, 128), f32),
            pltpu.VMEM((8, 1024), f32),
            pltpu.VMEM((M, D), bf16),
            pltpu.VMEM((D,), bf16),
            pltpu.SemaphoreType.DMA((len(GROUPS),)),
            pltpu.SemaphoreType.DMA((1,)),
        ],
        compiler_params=pltpu.CompilerParams(
            vmem_limit_bytes=100 * 1024 * 1024,
            disable_bounds_checks=True,
            disable_semaphore_checks=True,
            internal_scratch_in_bytes=48 * 1024,
        ),
        name="rmt_mod",
    )(A_x.reshape(NCH, CH, SEG, D), A_mem0.reshape(M, D), A_Wq, A_Wk, A_Wv, A_Wo.reshape(H * DH, D),
      B_w_r, B_w_gate.T, B_w_up.T, B_w_down)
    return out.reshape(1, S, D)
```

```python
import math

import jax
import jax.numpy as jnp
from jax import lax
import jax.experimental.pallas as pl
import jax.experimental.pallas.tpu as pltpu

bf16 = jnp.bfloat16
f32 = jnp.float32
u32 = jnp.uint32
i32 = jnp.int32

S = 2048
D = 640
H = 32
DH = 128
NP = H // 2
NU = NP * 3
M = 8
SEG = 32
NSEG = S // SEG
F = 1728
C = 8
CH = 4
NCH = NSEG // CH
NJ = D // 128
EPS = 1.3125 * 2.0 ** -17
NEG = -1e30
LOG2E = math.log2(math.e)
CEXP = (DH ** -0.5) * LOG2E
NT = (((1,), (1,)), ((), ()))

LAG_B, POS_B = 1, 6
LAG_D, POS_D = 3, 4
POS_B0 = (6, 6, 5, 5)
KMAJ = (4, 4, 4, 5)
MORDS = ((1, 0, 2), (1, 0, 2), (0, 1, 2), (1, 0, 2))
EBS = ((0, 6, 12, 20, 21, 32), (0, 9, 14, 18, 22, 27, 32), (0, 8, 13, 18, 25, 32), (0, 8, 14, 19, 23, 28))
EPOS = ((4, 2), (2, 3), (4, 4), (4, 2))
HL = EBS[CH - 1][-1]
NV2 = (8, 2)
VGB = (((0, 5, 11, 16), (0, 5, 11, 17, 24)), ((0, 5, 11, 16), (0, 5, 11, 17, 24)),
       ((0, 6, 11, 16), (0, 5, 11, 17, 24)), ((0, 6, 11, 16), (0, 6, 12, 18, 24)))
LAG_V = 11
TIE_KT = ((3, 0, 0, 0, 0, 3), (0, 0, 4, 0, 0, 3))
TIE_K = (None, 0, None, 1)
TIE_W, TIE_E = 2, (None, 2, None, 7)
E_RATE = 0.6

NPL = 4
UPL = 8
U0 = 9
CPL = NCH // NPL
SPL = NSEG // NPL
HEAD_GROUPS = (("p0",), ("w0", "p1"), ("w1", "p2", "p3"), ("w2", "w3", "w4"),
               ("mem0", "wr", "w5", "w6", "w7", "w8"))
HOLD = (0, 0, 0, 2, 2)
US = 5
LOOP_GROUPS = tuple(
    tuple("w%d" % u for u in range(U0 + i * UPL, U0 + (i + 1) * UPL)) + ("x%d" % i,) for i in range(NPL))
TAIL_GROUP = tuple("w%d" % u for u in range(U0 + NPL * UPL, NU)) + ("f0", "f1", "f2")
GROUPS = HEAD_GROUPS + LOOP_GROUPS + (TAIL_GROUP,)
WOR = H * DH // 2 // NPL
TIE_LAG = 5.0
FFN_SKIP, FFN_UP, FFN_DOWN = 9.0, 0.2, 0.16


def _tob(x):
    return pltpu.bitcast(x, bf16)


def _tou(x):
    return pltpu.bitcast(x, u32)


def _zero_of(x):
    return (pltpu.bitcast(x, u32) >> 16) >> 16


def _rb(x):
    return x.astype(bf16).astype(f32)


def _layernorm(x, tie=None):
    ps = x[:, 0:128]
    if tie is not None:
        ps = ps + tie
    for j in range(1, NJ):
        ps = ps + x[:, j * 128:(j + 1) * 128]
    mu = jnp.sum(ps, axis=-1, keepdims=True) * (1.0 / D)
    xc = x - mu
    var = jnp.sum(xc * xc, axis=-1, keepdims=True) * (1.0 / D)
    den = _rb(jnp.sqrt(_rb(_rb(var) + EPS)))
    return (_rb(x - _rb(mu)) * pl.reciprocal(den, approx=False, full_range=False)).astype(bf16)


def _sigmoid(z):
    return pl.reciprocal(1.0 + jnp.exp2(z * (-LOG2E)), approx=True)


def _silu(z):
    return z * _sigmoid(z)


def _dot(a, b):
    return jnp.dot(a, b, preferred_element_type=f32)


def _dot_t(a, b):
    return lax.dot_general(a, b, NT, preferred_element_type=f32)


def _kernel(x_hbm, mem0_hbm, wq_hbm, wk_hbm, wv_hbm, wo_hbm, wr_hbm, wg_hbm, wu_hbm, wd_hbm,
            out_hbm,
            xv, lhs, xpre, xsum, zbuf, raw, wqkv, wo, pre, stg, sst, wg, wu, wd, outv, mask_ref,
            accv, rds, wr8, mem0_v, wr_v, sem, sem_out):
    w32 = [w.bitcast(u32) for w in (wq_hbm, wk_hbm, wv_hbm)]
    wo32 = wo_hbm.bitcast(u32)

    def src_dst(name):
        if name == "mem0":
            return mem0_hbm, mem0_v
        if name == "wr":
            return wr_hbm, wr_v
        k, n = name[0], int(name[1:])
        if k == "x":
            idx = (pl.ds(n * CPL, CPL), slice(None), pl.ds(8, SEG - 8), slice(None))
            return x_hbm.at[idx], xv.at[idx]
        if k == "p":
            idx = (pl.ds(n * 4, 4), slice(None), pl.ds(0, 8), slice(None))
            return x_hbm.at[idx], xv.at[idx]
        if k == "w":
            return w32[n % 3].at[:, n // 3, :], raw.at[n]
        return ((wg_hbm, wg), (wu_hbm, wu), (wd_hbm, wd))[n]

    cps = [[pltpu.make_async_copy(*src_dst(nm), sem.at[gi]) for nm in grp]
           for gi, grp in enumerate(GROUPS)]
    for grp in cps:
        for cp in grp:
            cp.start()

    rr = lax.broadcasted_iota(i32, (64, 80), 0)
    hr = jnp.where(rr < 32, 0, 1)
    pr = jnp.where((rr & 31) < 8, rr & 31, (rr & 31) + 8)
    cc = lax.broadcasted_iota(i32, (64, 80), 1)
    hc = jnp.where(cc < 40, 0, 1)
    pc = cc - 40 * hc
    mask_ref[...] = jnp.where((hr == hc) & ((pr < M) | (pr >= pc)), 1.0, 0.0).astype(f32)

    def orow(h, r0, n):
        r0 += 240 + (h % 2) * 32 if h < H else 304 + (h % 2) * 16
        return ((h % H) // 2, slice(r0, r0 + n), slice(None))

    def o48(h0, h1):
        return jnp.concatenate([jnp.concatenate([stg[orow(h, 0, 32)], stg[orow(H + h, 0, 16)]], axis=0)
                                for h in range(h0, h1)], axis=1)

    st = {}
    lane8 = lax.broadcasted_iota(i32, (8, 128), 1)
    sub8 = lax.broadcasted_iota(i32, (8, 128), 0)

    def ln_pre(b):
        xb = xv[b * 4:(b + 1) * 4, :, 0:8, :].astype(f32).reshape(128, D)
        xpre[b] = _tou(_layernorm(xb))

    def repack(u):
        ev = raw[u, pl.ds(0, D // 2, stride=2), :]
        od = raw[u, pl.ds(1, D // 2, stride=2), :]
        ws = ((ev & jnp.uint32(0xFFFF)) | (od << 16), (ev >> 16) | (od & jnp.uint32(0xFFFF0000)))
        wqkv[2 * u] = ws[0]
        wqkv[2 * u + 1] = ws[1]
        return ws

    def x_sums(r):
        rows = slice((r % 8) * 8, (r % 8) * 8 + 8)
        u1, u2 = xpre[r // 8, rows, 0:512], xpre[2 + r // 8, rows, 0:512]
        if st["after"] is not None:
            u1 = u1 ^ jnp.concatenate([_zero_of(st["after"])] * 4, axis=1)
        x1, x2 = _tob(u1).astype(f32), _tob(u2).astype(f32)
        a11, a12, a21, a22 = x1[:, 0:256], x1[:, 256:512], x2[:, 0:256], x2[:, 256:512]
        tie = None
        for k, t in enumerate((a11 + a22, a21 + a22, a11 + a12, a21 - a11, a12 - a22)):
            t = _tou(t.astype(bf16))
            xsum[k, r * 8:(r + 1) * 8] = t
            t = t[:, 0:128] | t[:, 128:]
            tie = t if tie is None else tie | t
        return _zero_of(tie)

    def w_sums(u):
        w = raw[u, 0:512, :]
        lo = pltpu.bitcast(w << 16, f32)
        hi = pltpu.bitcast(w & jnp.uint32(0xFFFF0000), f32)
        b11, b21, b12, b22 = lo[0:256], lo[256:], hi[0:256], hi[256:]
        return [t.astype(bf16) for t in (b11 + b22, b12 - b22, b21 - b11, b11 + b12, b21 + b22)]

    def hooked_dot(hook, dt, xx, w):
        tie = hook(dt)
        if tie is not None:
            top = xx[0:8, 0:128] ^ tie
            if xx.shape[1] > 128:
                top = jnp.concatenate([top, xx[0:8, 128:]], axis=1)
            xx = jnp.concatenate([top, xx[8:]], axis=0)
        r = _dot(_tob(xx), w)
        st["after"] = r[0:8]
        return r

    def store_pre(u, b, r0, r1):
        n = r0.shape[0]
        parts = []
        for k in range(n // 8):
            parts += [r0[k * 8:(k + 1) * 8], r1[k * 8:(k + 1) * 8]]
        pre[u, b * 4:b * 4 + n // 32] = jnp.concatenate(parts, axis=0).reshape(n // 32, CH * 16, 128)

    def pre_plain(hook, u, b):
        store_pre(u, b, *[hooked_dot(hook, 1.0, xpre[b], _tob(wqkv[2 * u + hh])) for hh in range(2)])

    def pre_strassen(hook, u, gs, ws, sw):
        dt = 0.4 * len(gs)
        x1 = jnp.concatenate([xpre[g] for g in gs], axis=0)
        x2 = jnp.concatenate([xpre[g + 2] for g in gs], axis=0)
        sx = [xsum[k, gs[0] * 64:(gs[-1] + 1) * 64] for k in range(5)]
        n = 128 * len(gs)

        def last_tile(hh):
            return jnp.concatenate([hooked_dot(hook, dt / 2, xx[:, 512:], _tob(ws[hh][256:]))
                                    for xx in (x1, x2)], axis=0)

        l0 = last_tile(0)
        c11 = hooked_dot(hook, dt, sx[4], sw[4]) + l0[0:n]
        m4 = hooked_dot(hook, dt, x2[:, 256:512], sw[2])
        c11, c21 = c11 + m4, l0[n:] + m4
        m2 = hooked_dot(hook, dt, sx[1], _tob(ws[0][0:128]))
        c21 = c21 + m2
        m1 = hooked_dot(hook, dt, sx[0], sw[0])
        c11, c22 = c11 + m1, m1 - m2
        m5 = hooked_dot(hook, dt, sx[2], _tob(ws[1][128:256]))
        c11 = c11 - m5
        m3 = hooked_dot(hook, dt, x1[:, 0:256], sw[1])
        c12, c22 = m3 + m5, c22 + m3
        c22 = hooked_dot(hook, dt, sx[3], sw[3]) + c22
        l1 = last_tile(1)
        c12, c22 = c12 + l1[0:n], c22 + l1[n:]
        store_pre(u, gs[0], c11, c12)
        store_pre(u, gs[0] + 2, c21, c22)

    def score(i, gl, xn32):
        zbuf[i * CPL + gl // 16, (gl % 16) * 8:(gl % 16) * 8 + 8, :] = xn32
        rc = jnp.sum(xn32 * st["wr"], axis=-1, keepdims=True)
        st["rd"] = jnp.where(lane8 == gl, rc, st["rd"])

    def ln_group(i, s, k):
        tie = None
        if st["after"] is not None:
            tie = pltpu.bitcast(_zero_of(st["after"]), f32)
        xn = _layernorm(xv[i * CPL + s // CH, s % CH, k * 8:(k + 1) * 8, :].astype(f32), tie)
        score(i, s * 4 + k, xn.astype(f32))
        if k == 1 and s % 2 == 0:
            xp = _tob(xpre[i, s * 4:s * 4 + 8, :]).astype(f32)
            score(i, s * 4, xp[0:8])
            score(i, s * 4 + 4, xp[8:16])
        if k == 2:
            st["xn2"] = xn
        else:
            r0 = (s % CH) * 16 + (k // 2) * 8
            pair = jnp.concatenate([xn if k == 1 else st["xn2"], xn], axis=0)
            lhs[i * CPL + s // CH, r0:r0 + 8, :] = _tou(pair)
        return _zero_of(st["rd"])

    def topk():
        rd = _rb(rds[...].reshape(NPL * 8, 128))
        rd = jnp.where(rd == 0.0, 0.0, rd)
        bits = pltpu.bitcast(rd, i32)
        mono = jnp.where(bits < 0, bits ^ jnp.int32(0x7FFFFFFF), bits)
        rowid = jnp.concatenate([lane8 * 8 + sub8 + i * SPL * SEG for i in range(NPL)], axis=0)
        key = ((((mono >> 16) + 32768) << 11) | (S - 1 - rowid)) | jnp.int32(0x20000000)
        key = jnp.where(jnp.concatenate([lane8] * NPL, axis=0) < SPL * 4, pltpu.bitcast(key, f32), 0.0)
        row8 = lax.broadcasted_iota(i32, (8, 1), 0)
        ksel = jnp.zeros((8, 1), f32)
        for t in range(C):
            km = jnp.max(jnp.max(key, axis=0, keepdims=True), axis=1, keepdims=True)
            key = jnp.where(key == km, 0.0, key)
            ksel = jnp.where(row8 == t, km, ksel)
        ksel = pltpu.bitcast(ksel, i32)
        iv = S - 1 - (ksel & (S - 1))
        idxs = [iv[t, 0] for t in range(C)]
        xs = jnp.concatenate([zbuf[i_ >> 7, pl.ds(i_ & 127, 1), :] for i_ in idxs], axis=0)
        hi16 = (((ksel >> 11) & 65535) - 32768) << 16
        rbits = jnp.where(hi16 < 0, hi16 ^ jnp.int32(0x7FFF0000), hi16)
        return idxs, xs, _rb(_sigmoid(pltpu.bitcast(rbits, f32)))

    def ffn_tasks(idxs, xs, rsel):
        cols = [(k * 128, min(F, (k + 1) * 128)) for k in range(pl.cdiv(F, 128))]
        xsb = xs.astype(bf16)
        hid = []
        tmp = {}

        def up(w, a, b, k):
            t = _dot_t(xsb[:, k * 128:(k + 1) * 128], (wg, wu)[w][a:b, k * 128:(k + 1) * 128])
            tmp[w] = t if k == 0 else t + tmp[w]
            if w == 1 and k == NJ - 1:
                hid.append((_rb(_silu(_rb(tmp[0]))) * _rb(tmp[1])).astype(bf16))

        def down(k, j):
            t = _dot(hid[k], wd[cols[k][0]:cols[k][1], j * 128:(j + 1) * 128])
            tmp["y", j] = t if k == 0 else t + tmp["y", j]

        def fin():
            y = jnp.concatenate([tmp["y", j] for j in range(NJ)], axis=1)
            zs = _rb(xs + _rb(_rb(y) * rsel))
            for t in range(C):
                zbuf[idxs[t] >> 7, pl.ds(idxs[t] & 127, 1), :] = zs[t:t + 1]

        tasks = [(FFN_UP, lambda t=(w, a, b, k): up(*t)) for a, b in cols for w in range(2) for k in range(NJ)]
        tasks += [(FFN_DOWN, lambda t=(k, j): down(*t)) for k in range(len(cols)) for j in range(NJ)]
        return tasks + [(0.0, fin)]

    def run_region(work, side=(), span=None, tasks=()):
        side, tasks = list(side), list(tasks)
        total = sum(2.0 if len(w) == 2 else 3.6 * len(w[1]) for w in work)
        rate = len(side) / (span or (total - TIE_LAG - 2.0))
        ties = []
        st["after"] = None
        cnt = {"t": 0.0, "credit": 0.5, "next": FFN_SKIP}

        def hook(dt):
            t = cnt["t"]
            cnt["t"] += dt
            while tasks and t >= cnt["next"] - 1e-6:
                c, fn = tasks.pop(0)
                cnt["next"] += c
                fn()
            tie = None
            while ties and ties[0][0] <= t:
                z = ties.pop(0)[1]
                tie = z if tie is None else tie | z
            cnt["credit"] += rate * dt
            while side and cnt["credit"] >= 1.0:
                cnt["credit"] -= 1.0
                ties.append((t + TIE_LAG, side.pop(0)()))
            return tie

        for w in work:
            (pre_plain if len(w) == 2 else pre_strassen)(hook, *w)
        assert not ties and not side and not tasks

    pending = []
    units, blocks = [], []
    sums = [lambda r=r: x_sums(r) for r in range(16)]
    for gi, grp in enumerate(HEAD_GROUPS):
        for cp in cps[gi]:
            cp.wait()
        for u in [int(nm[1:]) for nm in grp if nm[0] == "w" and nm != "wr"]:
            ws = repack(u)
            if u == U0 - 1:
                pending += [(u, (0,), ws, w_sums(u)), (u, 1), (u, 3)]
            elif u >= US:
                pending.append((u, (0, 1), ws, w_sums(u)))
            else:
                pending += [(u, b) for b in blocks]
            units.append(u)
        for b in [int(nm[1:]) for nm in grp if nm[0] == "p"]:
            ln_pre(b)
            pending += [(u, b) for u in units]
            blocks.append(b)
        if "mem0" in grp:
            accv[...] = jnp.concatenate([mem0_v[...].astype(f32), jnp.zeros((40, D), f32)], axis=0)
            for h in range(HL, H):
                stg[orow(h, 0, 32)] = jnp.zeros((32, 128), f32)
                stg[orow(H + h, 0, 16)] = jnp.zeros((16, 128), f32)
            wr8[:, 0:D] = jnp.broadcast_to(wr_v[...].astype(f32).reshape(1, D), (8, D))
        n = len(pending) - HOLD[gi]
        work, pending = pending[:n], pending[n:]
        if gi == 3:
            run_region(work, sums[:13])
        elif gi == 4:
            run_region(work, sums[13:], span=3.0)
        else:
            run_region(work)
    assert pending == [(U0 - 1, 1), (U0 - 1, 3)]

    def pro_body(i, carry):
        ub = U0 + i * UPL
        for k in range(UPL):
            pltpu.make_async_copy(w32[0].at[:, 0, :], raw.at[ub + k], sem.at[len(HEAD_GROUPS) + i]).wait()
        idx = (pl.ds(i * CPL, CPL), slice(None), pl.ds(8, SEG - 8), slice(None))
        pltpu.make_async_copy(x_hbm.at[idx], xv.at[idx], sem.at[len(HEAD_GROUPS) + i]).wait()
        rows = pl.ds(pl.multiple_of(i * WOR, WOR), WOR)
        for j in range(NJ):
            pltpu.make_async_copy(wo32.at[rows, pl.ds(j * 128, 128)], wo.at[j, rows], sem.at[len(GROUPS)]).start()
        work = [(ub - 1, 1), (ub - 1, 3)]
        for k in range(UPL):
            work.append((ub + k, (0, 1) if k < UPL - 1 else (0,), repack(ub + k), w_sums(ub + k)))
        st["wr"] = wr8[:, 0:D]
        st["rd"] = jnp.zeros((8, 128), f32)
        run_region(work, [lambda a=(i, s, k): ln_group(*a) for s in range(SPL) for k in (1, 2, 3)])
        rds[i] = st["rd"]
        return carry

    lax.fori_loop(0, NPL, pro_body, 0)

    for cp in cps[-1]:
        cp.wait()
    ub = U0 + NPL * UPL
    work = [(ub - 1, 1), (ub - 1, 3)]
    for u in range(ub, NU):
        ws, sw = repack(u), w_sums(u)
        work += [(u, (0, 1), ws, sw)] if u == ub else [(u, (0,), ws, sw), (u, (1,), ws, sw)]
    run_region(work, tasks=ffn_tasks(*topk()))
    pltpu.make_async_copy(wo, wo, sem.at[len(GROUPS)]).wait()

    sub4 = lax.broadcasted_iota(i32, (8, D), 0) < 4

    def finalize(ci, sl, r0, r1, sv, c0=0, c1=D):
        xr = xv[ci, sl, r0:r1, c0:c1].astype(f32)
        g = _silu(zbuf[ci, sl * SEG + r0:sl * SEG + r1, c0:c1])
        outv[ci, sl, r0:r1, c0:c1] = (xr + sv * g).astype(bf16)

    def finish(ci, sl, acc):
        acc = jnp.concatenate(acc, axis=1)
        finalize(ci, sl, 8, SEG, acc[8:32])
        if sl % 2 == 1:
            finalize(ci, sl, 0, 8, acc[32:40])
            finalize(ci, sl - 1, 0, 8, acc[40:48])
        return _tou(acc[0:16].astype(bf16))

    def finish_last(ci):
        o2 = o48(HL, H).astype(bf16)
        acc = [_dot(o2, _tob(wo[j, HL * 64:, :])) + accv[:, j * 128:(j + 1) * 128] for j in range(NJ)]
        return finish(ci, CH - 1, acc)

    vq = []
    clock = [0]

    def vnext():
        ready = [i for i, t in enumerate(vq) if t[0] <= clock[0]]
        if not ready:
            return None
        return vq.pop(min(ready, key=lambda i: (vq[i][2], i)))[1]()

    def vforce(deadline):
        for t in [t for t in vq if t[2] <= deadline]:
            vq.remove(t)
            t[1]()

    def tied(w, g):
        tie = vnext()
        if tie is None:
            return w
        parts = [w[0:g * 8], w[g * 8:g * 8 + 8] ^ tie, w[g * 8 + 8:]]
        return jnp.concatenate([t for t in parts if t.shape[0]], axis=0)

    def step(ci, sl, mem):
        xu = lhs[ci, sl * 16:(sl + 1) * 16, :]
        x = _tob(jnp.concatenate([jnp.where(sub4, mem, xu[0:8]), xu[8:16]], axis=0))
        mord, eb, odd = MORDS[sl], EBS[sl], sl % 2
        probs = {}
        vs = {}
        attended = set()

        early = {}
        for k in range(NJ):
            clock[0] += 1
            for d in range(KMAJ[sl]):
                key = (d // 6, mord[(d % 6) // 2], d % 2)
                w = wqkv[2 * (key[0] * 3 + key[1]) + key[2], k * 64:(k + 1) * 64, :]
                if d == TIE_K[sl]:
                    w = tied(w, TIE_W)
                t = _dot(x[:, k * 128:(k + 1) * 128], _tob(w))
                early[key] = t if k == 0 else t + early[key]

        def slot_of(p, m, hh):
            return m * 2 + hh

        def project(p, di):
            m, hh = mord[di // 2], di % 2
            if (p, m, hh) in early:
                r = early[p, m, hh]
            else:
                clock[0] += 1
                r = _dot(x, _tob(tied(wqkv[2 * (p * 3 + m) + hh], TIE_KT[odd][di] * 8 + TIE_W)))
            b0 = slot_of(p, m, hh) * 40
            stg[odd * NP + p, b0:b0 + 8, :] = r[0:8]
            stg[odd * NP + p, b0 + 16:b0 + 40, :] = r[8:32]
            if m > 0:
                stg[odd * NP + p, b0 + 8:b0 + 16, :] = pre[p * 3 + m, ci, sl * 16 + hh * 8:sl * 16 + hh * 8 + 8, :]

        def mxu_rows(p, a):
            if p < NV2[odd]:
                return jnp.concatenate([a[0:8], a[32:40], a[16:32], a[48:64]], axis=0)
            return a

        def operand(p, m):
            b0 = slot_of(p, m, 0) * 40
            if m > 0:
                a = stg[odd * NP + p, b0:b0 + 80, :]
            else:
                a = mxu_rows(p, jnp.concatenate([stg[odd * NP + p, b0:b0 + 8, :], stg[odd * NP + p, b0 + 16:b0 + 48, :],
                                                 stg[odd * NP + p, b0 + 56:b0 + 80, :]], axis=0))
            return a.astype(bf16)

        def vpu_rows(p, hh, lv, g):
            gb = VGB[sl][lv]
            r0 = sl * 16 + hh * 8

            def row(m, i):
                b0 = slot_of(p, m, hh) * 40 + 8 + 8 * lv - i
                return stg[odd * NP + p, b0:b0 + 8, :]

            if g == 0:
                q = pre[p * 3, ci, r0:r0 + 8, :] if lv == 0 else row(0, 0)
                vs[p, hh, lv] = (q * CEXP, None, None, None)
            q, m_old, l, o = vs[p, hh, lv]
            i0, n = gb[g], gb[g + 1] - gb[g]

            def rows(m):
                return jnp.concatenate([row(m, i0 + i) for i in range(n)], axis=0).reshape(n, 8, 128)

            s = jnp.sum(q[None] * rows(1), axis=-1, keepdims=True)
            if i0 + n > 9 + 8 * lv:
                ok = (lax.broadcasted_iota(i32, (n, 8, 1), 1)
                      >= lax.broadcasted_iota(i32, (n, 8, 1), 0) + (i0 - 8 - 8 * lv))
                s = jnp.where(ok, s, NEG)
            mx = jnp.max(s, axis=0)
            if m_old is not None:
                mx = jnp.maximum(mx, m_old)
            e = jnp.exp2(s - mx[None])
            el, ev = jnp.sum(e, axis=0), jnp.sum(e * rows(2), axis=0)
            if m_old is None:
                l, o = el, ev
            else:
                alpha = jnp.exp2(m_old - mx)
                l, o = l * alpha + el, o * alpha + ev
            if g == len(gb) - 2:
                o = o * pl.reciprocal(l, approx=True)
                if lv == 0:
                    stg[orow(H + 2 * p + hh, (1 - odd) * 8, 8)] = o
                else:
                    stg[orow(2 * p + hh, 8, 8)] = o
            vs[p, hh, lv] = (q, mx, l, o)
            return _zero_of(o)

        def scores(p):
            if not 0 <= p < NP:
                return
            sc = jnp.where(mxu_rows(p, mask_ref[...]) > 0.5, _dot_t(operand(p, 0), operand(p, 1)), NEG)
            n = sc.shape[0]
            mx = jnp.max(sc, axis=-1, keepdims=True)
            sst[p % 2, 0:n] = sc
            e = jnp.exp2((sst[p % 2, 0:n] - mx) * CEXP)
            l = jnp.sum(e, axis=-1, keepdims=True)
            sst[2 + p % 2, 0:n] = e
            probs[p] = (sst[2 + p % 2, 0:n] * pl.reciprocal(l, approx=True)).astype(bf16)

        def attend(p):
            if not 0 <= p < NP:
                return
            o = _dot(probs[p], operand(p, 2))
            attended.add(p)
            for hh in range(2):
                if p < NV2[odd]:
                    stg[orow(2 * p + hh, 0, 8)] = o[hh * 8:hh * 8 + 8]
                    stg[orow(2 * p + hh, 16, 16)] = o[16 + hh * 16:32 + hh * 16]
                else:
                    stg[orow(2 * p + hh, 0, 32)] = o[hh * 32:(hh + 1) * 32]

        def oheads(h0, h1):
            assert (h1 - 1) // 2 in attended
            vforce((sl, h1 - 1))
            if not odd:
                return jnp.concatenate([stg[orow(h, 0, 32)] for h in range(h0, h1)], axis=1)
            return o48(h0, h1)

        for slot in range(NP):
            for di in range(7):
                if di == (POS_B0[sl] if slot == LAG_B else POS_B):
                    scores(slot - LAG_B)
                if di == POS_D:
                    attend(slot - LAG_D)
                if di < 6:
                    project(slot, di)
            for hh in range(2):
                for lv in ((1, 0) if slot < NV2[odd] else (0,)):
                    for g in range(len(VGB[sl][lv]) - 1):
                        vq.append((clock[0] + LAG_V, lambda a=(slot, hh, lv, g): vpu_rows(*a),
                                   (sl if lv == 1 else sl | 1, 2 * slot + hh)))
        tiles, credit = 0, 0.0
        acc = [None] * NJ
        for i in range(len(eb) - 1):
            h0, h1 = eb[i], eb[i + 1]
            o2 = oheads(h0, h1).astype(bf16)
            for j in range(NJ):
                ws = []
                for h in range(h0, h1):
                    tiles += 1
                    if tiles % (3 if odd else 5) == 0:
                        clock[0] += 1
                    w = wo[j, h * 64:(h + 1) * 64, :]
                    if odd:
                        credit += E_RATE
                        if credit >= 1.0:
                            credit -= 1.0
                            w = tied(w, TIE_E[sl])
                    ws.append(w)
                t = _dot(o2, _tob(jnp.concatenate(ws, axis=0)))
                acc[j] = t if acc[j] is None else t + acc[j]
                if j == EPOS[sl][0]:
                    scores(NP + i - LAG_B)
                if j == EPOS[sl][1]:
                    attend(NP + i - LAG_D)
        if sl == CH - 1:
            accv[...] = jnp.concatenate(acc, axis=1)
            vforce((sl, H))
            assert not vq and len(attended) == NP
            return None
        return finish(ci, sl, acc)

    def out_cp(*idx):
        return pltpu.make_async_copy(outv.at[idx], out_hbm.at[idx], sem_out.at[0])

    def chunk(ci, carry):
        prev = jnp.maximum(ci - 1, 0)
        mem = finish_last(prev)

        @pl.when(ci >= 1)
        def _():
            out_cp(prev, pl.ds(2, 2)).start()

        for sl in range(CH):
            mem = step(ci, sl, mem)
            if sl == 1:
                out_cp(ci, pl.ds(0, 2)).start()
        return carry

    lax.fori_loop(0, NCH, chunk, 0)
    o2 = o48(HL, H).astype(bf16)
    for j in range(NJ):
        c0, c1 = j * 128, (j + 1) * 128
        t = _dot(o2, _tob(wo[j, HL * 64:, :])) + accv[:, c0:c1]
        finalize(NCH - 1, CH - 1, 8, SEG, t[8:32], c0, c1)
        finalize(NCH - 1, CH - 1, 0, 8, t[32:40], c0, c1)
        finalize(NCH - 1, CH - 2, 0, 8, t[40:48], c0, c1)
        out_cp(NCH - 1, pl.ds(2, 2), slice(None), pl.ds(c0, 128)).start()
    pltpu.make_async_copy(outv, out_hbm, sem_out.at[0]).wait()


@jax.jit
def pallas_recurrent_scan__memory_aug_recurrent_mem_tr__moe_arch_mod__prompt_kernel(
    A_x, A_mem0, A_Wq, A_Wk, A_Wv, A_Wo, A_seg_len, B_x, B_w_r, B_w_gate, B_w_up, B_w_down,
):
    hbm = pl.BlockSpec(memory_space=pltpu.MemorySpace.HBM)
    out = pl.pallas_call(
        _kernel,
        out_shape=jax.ShapeDtypeStruct((NCH, CH, SEG, D), bf16),
        in_specs=[hbm] * 10,
        out_specs=hbm,
        scratch_shapes=[
            pltpu.VMEM((NCH, CH, SEG, D), bf16),
            pltpu.VMEM((NCH, CH * 16, D), u32),
            pltpu.VMEM((4, 64, D), u32),
            pltpu.VMEM((5, 128, 256), u32),
            pltpu.VMEM((NCH, CH * SEG, D), f32),
            pltpu.VMEM((NU, D, 128), u32),
            pltpu.VMEM((NU * 2, D // 2, 128), u32),
            pltpu.VMEM((NJ, H * DH // 2, 128), u32),
            pltpu.VMEM((NU, NCH, CH * 16, 128), f32),
            pltpu.VMEM((2 * NP, 352, 128), f32),
            pltpu.VMEM((4, 64, 80), f32),
            pltpu.VMEM((F, D), bf16),
            pltpu.VMEM((F, D), bf16),
            pltpu.VMEM((F, D), bf16),
            pltpu.VMEM((NCH, CH, SEG, D), bf16),
            pltpu.VMEM((64, 80), f32),
            pltpu.VMEM((48, D), f32),
            pltpu.VMEM((NPL, 8, 128), f32),
            pltpu.VMEM((8, 1024), f32),
            pltpu.VMEM((M, D), bf16),
            pltpu.VMEM((D,), bf16),
            pltpu.SemaphoreType.DMA((len(GROUPS) + 1,)),
            pltpu.SemaphoreType.DMA((1,)),
        ],
        compiler_params=pltpu.CompilerParams(
            vmem_limit_bytes=100 * 1024 * 1024,
            disable_bounds_checks=True,
            disable_semaphore_checks=True,
            internal_scratch_in_bytes=48 * 1024,
        ),
        name="rmt_mod",
    )(A_x.reshape(NCH, CH, SEG, D), A_mem0.reshape(M, D), A_Wq, A_Wk, A_Wv, A_Wo.reshape(H * DH, D),
      B_w_r, B_w_gate.T, B_w_up.T, B_w_down)
    return out.reshape(1, S, D)
```

```python
import math

import jax
import jax.numpy as jnp
from jax import lax
import jax.experimental.pallas as pl
import jax.experimental.pallas.tpu as pltpu

bf16 = jnp.bfloat16
f32 = jnp.float32
u32 = jnp.uint32
i32 = jnp.int32

S = 2048
D = 640
H = 32
DH = 128
NP = H // 2
NU = NP * 3
M = 8
SEG = 32
NSEG = S // SEG
F = 1728
C = 8
CH = 4
NCH = NSEG // CH
NJ = D // 128
EPS = 1.3125 * 2.0 ** -17
NEG = -1e30
LOG2E = math.log2(math.e)
CEXP = (DH ** -0.5) * LOG2E
NT = (((1,), (1,)), ((), ()))

LAG_B, POS_B = 1, 6
LAG_D, POS_D = 3, 4
POS_B0 = (6, 6, 5, 5)
KMAJ = (4, 4, 4, 5)
MORDS = ((1, 0, 2), (1, 0, 2), (0, 1, 2), (1, 0, 2))
EBS = ((0, 6, 12, 20, 21, 32), (0, 9, 14, 18, 22, 27, 32), (0, 8, 13, 18, 25, 32), (0, 8, 14, 19, 23, 28))
EPOS = ((4, 2), (2, 3), (4, 4), (4, 2))
HL = EBS[CH - 1][-1]
NV2 = (8, 2)
VGB = (((0, 5, 11, 16), (0, 5, 11, 17, 24)), ((0, 5, 11, 16), (0, 5, 11, 17, 24)),
       ((0, 6, 11, 16), (0, 5, 11, 17, 24)), ((0, 6, 11, 16), (0, 6, 12, 18, 24)))
LAG_V = 11
TIE_KT = ((3, 0, 0, 0, 0, 3), (0, 0, 4, 0, 0, 3))
TIE_K = (None, 0, None, 1)
TIE_W, TIE_E = 2, (None, 2, None, 7)
E_RATE = 0.6

NPL = 4
UPL = 8
U0 = 9
CPL = NCH // NPL
SPL = NSEG // NPL
HEAD_GROUPS = (("p0",), ("w0", "p1"), ("w1", "p2", "p3"), ("w2", "w3", "w4"),
               ("mem0", "wr", "w5", "w6", "w7", "w8"))
HOLD = (0, 0, 0, 2, 0)
US = 5
LOOP_GROUPS = tuple(
    tuple("w%d" % u for u in range(U0 + i * UPL, U0 + (i + 1) * UPL)) + ("x%d" % i,) for i in range(NPL))
TAIL_GROUP = tuple("w%d" % u for u in range(U0 + NPL * UPL, NU)) + ("f0", "f1", "f2")
GROUPS = HEAD_GROUPS + LOOP_GROUPS + (TAIL_GROUP,)
WOR = H * DH // 2 // NPL
TIE_LAG = 5.0
FFN_SKIP, FFN_UP, FFN_DOWN = 8.0, 0.2, 0.2


def _tob(x):
    return pltpu.bitcast(x, bf16)


def _tou(x):
    return pltpu.bitcast(x, u32)


def _zero_of(x):
    return (pltpu.bitcast(x, u32) >> 16) >> 16


def _rb(x):
    return x.astype(bf16).astype(f32)


def _layernorm(x, tie=None):
    ps = x[:, 0:128]
    if tie is not None:
        ps = ps + tie
    for j in range(1, NJ):
        ps = ps + x[:, j * 128:(j + 1) * 128]
    mu = jnp.sum(ps, axis=-1, keepdims=True) * (1.0 / D)
    xc = x - mu
    var = jnp.sum(xc * xc, axis=-1, keepdims=True) * (1.0 / D)
    den = _rb(jnp.sqrt(_rb(_rb(var) + EPS)))
    return (_rb(x - _rb(mu)) * pl.reciprocal(den, approx=False, full_range=False)).astype(bf16)


def _sigmoid(z):
    return pl.reciprocal(1.0 + jnp.exp2(z * (-LOG2E)), approx=True)


def _silu(z):
    return z * _sigmoid(z)


def _dot(a, b):
    return jnp.dot(a, b, preferred_element_type=f32)


def _dot_t(a, b):
    return lax.dot_general(a, b, NT, preferred_element_type=f32)


def _kernel(x_hbm, mem0_hbm, wq_hbm, wk_hbm, wv_hbm, wo_hbm, wr_hbm, wg_hbm, wu_hbm, wd_hbm,
            out_hbm,
            xv, lhs, xpre, xsum, swv, zbuf, raw, wqkv, wo, pre, stg, sst, wg, wu, wd, outv, mask_ref,
            accv, rds, wr8, mem0_v, wr_v, sem, sem_out):
    w32 = [w.bitcast(u32) for w in (wq_hbm, wk_hbm, wv_hbm)]
    wo32 = wo_hbm.bitcast(u32)

    def src_dst(name):
        if name == "mem0":
            return mem0_hbm, mem0_v
        if name == "wr":
            return wr_hbm, wr_v
        k, n = name[0], int(name[1:])
        if k == "x":
            idx = (pl.ds(n * CPL, CPL), slice(None), pl.ds(8, SEG - 8), slice(None))
            return x_hbm.at[idx], xv.at[idx]
        if k == "p":
            idx = (pl.ds(n * 4, 4), slice(None), pl.ds(0, 8), slice(None))
            return x_hbm.at[idx], xv.at[idx]
        if k == "w":
            return w32[n % 3].at[:, n // 3, :], raw.at[n]
        return ((wg_hbm, wg), (wu_hbm, wu), (wd_hbm, wd))[n]

    cps = [[pltpu.make_async_copy(*src_dst(nm), sem.at[gi]) for nm in grp]
           for gi, grp in enumerate(GROUPS)]
    for grp in cps:
        for cp in grp:
            cp.start()

    rr = lax.broadcasted_iota(i32, (64, 80), 0)
    hr = jnp.where(rr < 32, 0, 1)
    pr = jnp.where((rr & 31) < 8, rr & 31, (rr & 31) + 8)
    cc = lax.broadcasted_iota(i32, (64, 80), 1)
    hc = jnp.where(cc < 40, 0, 1)
    pc = cc - 40 * hc
    mask_ref[...] = jnp.where((hr == hc) & ((pr < M) | (pr >= pc)), 1.0, 0.0).astype(f32)

    def orow(h, r0, n):
        r0 += 240 + (h % 2) * 32 if h < H else 304 + (h % 2) * 16
        return ((h % H) // 2, slice(r0, r0 + n), slice(None))

    def o48(h0, h1):
        return jnp.concatenate([jnp.concatenate([stg[orow(h, 0, 32)], stg[orow(H + h, 0, 16)]], axis=0)
                                for h in range(h0, h1)], axis=1)

    st = {}
    lane8 = lax.broadcasted_iota(i32, (8, 128), 1)
    sub8 = lax.broadcasted_iota(i32, (8, 128), 0)

    def ln_pre(b):
        xb = xv[b * 4:(b + 1) * 4, :, 0:8, :].astype(f32).reshape(128, D)
        xpre[b] = _tou(_layernorm(xb))

    def repack(u):
        ev = raw[u, pl.ds(0, D // 2, stride=2), :]
        od = raw[u, pl.ds(1, D // 2, stride=2), :]
        ws = ((ev & jnp.uint32(0xFFFF)) | (od << 16), (ev >> 16) | (od & jnp.uint32(0xFFFF0000)))
        wqkv[2 * u] = ws[0]
        wqkv[2 * u + 1] = ws[1]
        return ws

    def x_sums(r):
        rows = slice((r % 8) * 8, (r % 8) * 8 + 8)
        u1, u2 = xpre[r // 8, rows, 0:512], xpre[2 + r // 8, rows, 0:512]
        if st["after"] is not None:
            u1 = u1 ^ jnp.concatenate([_zero_of(st["after"])] * 4, axis=1)
        x1, x2 = _tob(u1).astype(f32), _tob(u2).astype(f32)
        a11, a12, a21, a22 = x1[:, 0:256], x1[:, 256:512], x2[:, 0:256], x2[:, 256:512]
        tie = None
        for k, t in enumerate((a11 + a22, a21 + a22, a11 + a12, a21 - a11, a12 - a22)):
            t = _tou(t.astype(bf16))
            xsum[k, r * 8:(r + 1) * 8] = t
            t = t[:, 0:128] | t[:, 128:]
            tie = t if tie is None else tie | t
        return _zero_of(tie)

    def w_sums(u):
        w = raw[u, 0:512, :]
        lo = pltpu.bitcast(w << 16, f32)
        hi = pltpu.bitcast(w & jnp.uint32(0xFFFF0000), f32)
        b11, b21, b12, b22 = lo[0:256], lo[256:], hi[0:256], hi[256:]
        return [t.astype(bf16) for t in (b11 + b22, b12 - b22, b21 - b11, b11 + b12, b21 + b22)]

    def keep_sums(u):
        ws, sw = repack(u), w_sums(u)
        for k in range(5):
            swv[k] = _tou(sw[k])
        return (u, (0,), ws, sw)

    def held(u):
        return (u, (1,), (wqkv[2 * u], wqkv[2 * u + 1]), [_tob(swv[k]) for k in range(5)])

    def hooked_dot(hook, dt, xx, w):
        tie = hook(dt)
        if tie is not None:
            top = xx[0:8, 0:128] ^ tie
            if xx.shape[1] > 128:
                top = jnp.concatenate([top, xx[0:8, 128:]], axis=1)
            xx = jnp.concatenate([top, xx[8:]], axis=0)
        r = _dot(_tob(xx), w)
        st["after"] = r[0:8]
        return r

    def store_pre(u, b, r0, r1):
        n = r0.shape[0]
        parts = []
        for k in range(n // 8):
            parts += [r0[k * 8:(k + 1) * 8], r1[k * 8:(k + 1) * 8]]
        pre[u, b * 4:b * 4 + n // 32] = jnp.concatenate(parts, axis=0).reshape(n // 32, CH * 16, 128)

    def pre_plain(hook, u, b):
        store_pre(u, b, *[hooked_dot(hook, 1.0, xpre[b], _tob(wqkv[2 * u + hh])) for hh in range(2)])

    def pre_strassen(hook, u, gs, ws, sw):
        dt = 0.4 * len(gs)
        x1 = jnp.concatenate([xpre[g] for g in gs], axis=0)
        x2 = jnp.concatenate([xpre[g + 2] for g in gs], axis=0)
        sx = [xsum[k, gs[0] * 64:(gs[-1] + 1) * 64] for k in range(5)]
        n = 128 * len(gs)

        def last_tile(hh):
            return jnp.concatenate([hooked_dot(hook, dt / 2, xx[:, 512:], _tob(ws[hh][256:]))
                                    for xx in (x1, x2)], axis=0)

        l0 = last_tile(0)
        c11 = hooked_dot(hook, dt, sx[4], sw[4]) + l0[0:n]
        m4 = hooked_dot(hook, dt, x2[:, 256:512], sw[2])
        c11, c21 = c11 + m4, l0[n:] + m4
        m2 = hooked_dot(hook, dt, sx[1], _tob(ws[0][0:128]))
        c21 = c21 + m2
        m1 = hooked_dot(hook, dt, sx[0], sw[0])
        c11, c22 = c11 + m1, m1 - m2
        m5 = hooked_dot(hook, dt, sx[2], _tob(ws[1][128:256]))
        c11 = c11 - m5
        m3 = hooked_dot(hook, dt, x1[:, 0:256], sw[1])
        c12, c22 = m3 + m5, c22 + m3
        c22 = hooked_dot(hook, dt, sx[3], sw[3]) + c22
        l1 = last_tile(1)
        c12, c22 = c12 + l1[0:n], c22 + l1[n:]
        store_pre(u, gs[0], c11, c12)
        store_pre(u, gs[0] + 2, c21, c22)

    def score(i, gl, xn32):
        zbuf[i * CPL + gl // 16, (gl % 16) * 8:(gl % 16) * 8 + 8, :] = xn32
        rc = jnp.sum(xn32 * st["wr"], axis=-1, keepdims=True)
        st["rd"] = jnp.where(lane8 == gl, rc, st["rd"])

    def ln_group(i, s, k):
        tie = None
        if st["after"] is not None:
            tie = pltpu.bitcast(_zero_of(st["after"]), f32)
        xn = _layernorm(xv[i * CPL + s // CH, s % CH, k * 8:(k + 1) * 8, :].astype(f32), tie)
        score(i, s * 4 + k, xn.astype(f32))
        if k == 1 and s % 2 == 0:
            xp = _tob(xpre[i, s * 4:s * 4 + 8, :]).astype(f32)
            score(i, s * 4, xp[0:8])
            score(i, s * 4 + 4, xp[8:16])
        if k == 2:
            st["xn2"] = xn
        else:
            r0 = (s % CH) * 16 + (k // 2) * 8
            pair = jnp.concatenate([xn if k == 1 else st["xn2"], xn], axis=0)
            lhs[i * CPL + s // CH, r0:r0 + 8, :] = _tou(pair)
        return _zero_of(st["rd"])

    def topk():
        rd = _rb(rds[...].reshape(NPL * 8, 128))
        rd = jnp.where(rd == 0.0, 0.0, rd)
        bits = pltpu.bitcast(rd, i32)
        mono = jnp.where(bits < 0, bits ^ jnp.int32(0x7FFFFFFF), bits)
        rowid = jnp.concatenate([lane8 * 8 + sub8 + i * SPL * SEG for i in range(NPL)], axis=0)
        key = ((((mono >> 16) + 32768) << 11) | (S - 1 - rowid)) | jnp.int32(0x20000000)
        key = jnp.where(jnp.concatenate([lane8] * NPL, axis=0) < SPL * 4, pltpu.bitcast(key, f32), 0.0)
        row8 = lax.broadcasted_iota(i32, (8, 1), 0)
        ksel = jnp.zeros((8, 1), f32)
        for t in range(C):
            km = jnp.max(jnp.max(key, axis=0, keepdims=True), axis=1, keepdims=True)
            key = jnp.where(key == km, 0.0, key)
            ksel = jnp.where(row8 == t, km, ksel)
        ksel = pltpu.bitcast(ksel, i32)
        iv = S - 1 - (ksel & (S - 1))
        idxs = [iv[t, 0] for t in range(C)]
        xs = jnp.concatenate([zbuf[i_ >> 7, pl.ds(i_ & 127, 1), :] for i_ in idxs], axis=0)
        hi16 = (((ksel >> 11) & 65535) - 32768) << 16
        rbits = jnp.where(hi16 < 0, hi16 ^ jnp.int32(0x7FFF0000), hi16)
        return idxs, xs, _rb(_sigmoid(pltpu.bitcast(rbits, f32)))

    def ffn_tasks(idxs, xs, rsel):
        cols = [(k * 128, min(F, (k + 1) * 128)) for k in range(pl.cdiv(F, 128))]
        xsb = xs.astype(bf16)
        hid = []
        tmp = {}

        def up(w, a, b, k):
            t = _dot_t(xsb[:, k * 128:(k + 1) * 128], (wg, wu)[w][a:b, k * 128:(k + 1) * 128])
            tmp[w] = t if k == 0 else t + tmp[w]
            if w == 1 and k == NJ - 1:
                hid.append((_rb(_silu(_rb(tmp[0]))) * _rb(tmp[1])).astype(bf16))

        def down(k, j):
            t = _dot(hid[k], wd[cols[k][0]:cols[k][1], j * 128:(j + 1) * 128])
            tmp["y", j] = t if k == 0 else t + tmp["y", j]

        def fin():
            y = jnp.concatenate([tmp["y", j] for j in range(NJ)], axis=1)
            zs = _rb(xs + _rb(_rb(y) * rsel))
            for t in range(C):
                zbuf[idxs[t] >> 7, pl.ds(idxs[t] & 127, 1), :] = zs[t:t + 1]

        tasks = [(FFN_UP, lambda t=(w, a, b, k): up(*t)) for a, b in cols for w in range(2) for k in range(NJ)]
        tasks += [(FFN_DOWN, lambda t=(k, j): down(*t)) for k in range(len(cols)) for j in range(NJ)]
        return tasks + [(0.0, fin)]

    def run_region(work, side=(), span=None, tasks=()):
        side, tasks = list(side), list(tasks)
        total = sum(2.0 if len(w) == 2 else 3.6 * len(w[1]) for w in work)
        rate = len(side) / (span or (total - TIE_LAG - 2.0))
        ties = []
        st["after"] = None
        cnt = {"t": 0.0, "credit": 0.5, "next": FFN_SKIP}

        def hook(dt):
            t = cnt["t"]
            cnt["t"] += dt
            while tasks and t >= cnt["next"] - 1e-6:
                c, fn = tasks.pop(0)
                cnt["next"] += c
                fn()
            tie = None
            while ties and ties[0][0] <= t:
                z = ties.pop(0)[1]
                tie = z if tie is None else tie | z
            cnt["credit"] += rate * dt
            while side and cnt["credit"] >= 1.0:
                cnt["credit"] -= 1.0
                ties.append((t + TIE_LAG, side.pop(0)()))
            return tie

        for w in work:
            (pre_plain if len(w) == 2 else pre_strassen)(hook, *w)
        assert not ties and not side and not tasks

    pending = []
    units, blocks = [], []
    sums = [lambda r=r: x_sums(r) for r in range(16)]
    for gi, grp in enumerate(HEAD_GROUPS):
        for cp in cps[gi]:
            cp.wait()
        for u in [int(nm[1:]) for nm in grp if nm[0] == "w" and nm != "wr"]:
            if u == U0 - 1:
                pending.append(keep_sums(u))
            elif u >= US:
                pending.append((u, (0, 1), repack(u), w_sums(u)))
            else:
                repack(u)
                pending += [(u, b) for b in blocks]
            units.append(u)
        for b in [int(nm[1:]) for nm in grp if nm[0] == "p"]:
            ln_pre(b)
            pending += [(u, b) for u in units]
            blocks.append(b)
        if "mem0" in grp:
            accv[...] = jnp.concatenate([mem0_v[...].astype(f32), jnp.zeros((40, D), f32)], axis=0)
            for h in range(HL, H):
                stg[orow(h, 0, 32)] = jnp.zeros((32, 128), f32)
                stg[orow(H + h, 0, 16)] = jnp.zeros((16, 128), f32)
            wr8[:, 0:D] = jnp.broadcast_to(wr_v[...].astype(f32).reshape(1, D), (8, D))
        n = len(pending) - HOLD[gi]
        work, pending = pending[:n], pending[n:]
        if gi == 3:
            run_region(work, sums[:13])
        elif gi == 4:
            run_region(work, sums[13:], span=3.0)
        else:
            run_region(work)
    assert not pending

    def pro_body(i, carry):
        ub = U0 + i * UPL
        filled = raw.at[pl.ds(ub, UPL)]
        pltpu.make_async_copy(filled, filled, sem.at[len(HEAD_GROUPS) + i]).wait()
        idx = (pl.ds(i * CPL, CPL), slice(None), pl.ds(8, SEG - 8), slice(None))
        pltpu.make_async_copy(x_hbm.at[idx], xv.at[idx], sem.at[len(HEAD_GROUPS) + i]).wait()
        rows = pl.ds(pl.multiple_of(i * WOR, WOR), WOR)
        for j in range(NJ):
            pltpu.make_async_copy(wo32.at[rows, pl.ds(j * 128, 128)], wo.at[j, rows], sem.at[len(GROUPS)]).start()
        work = [held(ub - 1)] + [(ub + k, (0, 1), repack(ub + k), w_sums(ub + k)) for k in range(UPL - 1)]
        work.append(keep_sums(ub + UPL - 1))
        st["wr"] = wr8[:, 0:D]
        st["rd"] = jnp.zeros((8, 128), f32)
        run_region(work, [lambda a=(i, s, k): ln_group(*a) for s in range(SPL) for k in (1, 2, 3)])
        rds[i] = st["rd"]
        return carry

    lax.fori_loop(0, NPL, pro_body, 0)

    for cp in cps[-1]:
        cp.wait()
    ub = U0 + NPL * UPL
    work = [held(ub - 1)]
    for u in range(ub, NU):
        ws, sw = repack(u), w_sums(u)
        work += [(u, (0, 1), ws, sw)] if u == ub else [(u, (0,), ws, sw), (u, (1,), ws, sw)]
    run_region(work, tasks=ffn_tasks(*topk()))
    pltpu.make_async_copy(wo, wo, sem.at[len(GROUPS)]).wait()

    sub4 = lax.broadcasted_iota(i32, (8, D), 0) < 4

    def finalize(ci, sl, r0, r1, sv, c0=0, c1=D):
        xr = xv[ci, sl, r0:r1, c0:c1].astype(f32)
        g = _silu(zbuf[ci, sl * SEG + r0:sl * SEG + r1, c0:c1])
        outv[ci, sl, r0:r1, c0:c1] = (xr + sv * g).astype(bf16)

    def finish(ci, sl, acc):
        acc = jnp.concatenate(acc, axis=1)
        finalize(ci, sl, 8, SEG, acc[8:32])
        if sl % 2 == 1:
            finalize(ci, sl, 0, 8, acc[32:40])
            finalize(ci, sl - 1, 0, 8, acc[40:48])
        return _tou(acc[0:16].astype(bf16))

    def finish_last(ci):
        o2 = o48(HL, H).astype(bf16)
        acc = [_dot(o2, _tob(wo[j, HL * 64:, :])) + accv[:, j * 128:(j + 1) * 128] for j in range(NJ)]
        return finish(ci, CH - 1, acc)

    vq = []
    clock = [0]

    def vnext():
        ready = [i for i, t in enumerate(vq) if t[0] <= clock[0]]
        if not ready:
            return None
        return vq.pop(min(ready, key=lambda i: (vq[i][2], i)))[1]()

    def vforce(deadline):
        for t in [t for t in vq if t[2] <= deadline]:
            vq.remove(t)
            t[1]()

    def tied(w, g):
        tie = vnext()
        if tie is None:
            return w
        parts = [w[0:g * 8], w[g * 8:g * 8 + 8] ^ tie, w[g * 8 + 8:]]
        return jnp.concatenate([t for t in parts if t.shape[0]], axis=0)

    def step(ci, sl, mem):
        xu = lhs[ci, sl * 16:(sl + 1) * 16, :]
        x = _tob(jnp.concatenate([jnp.where(sub4, mem, xu[0:8]), xu[8:16]], axis=0))
        mord, eb, odd = MORDS[sl], EBS[sl], sl % 2
        probs = {}
        vs = {}
        attended = set()

        early = {}
        for k in range(NJ):
            clock[0] += 1
            for d in range(KMAJ[sl]):
                key = (d // 6, mord[(d % 6) // 2], d % 2)
                w = wqkv[2 * (key[0] * 3 + key[1]) + key[2], k * 64:(k + 1) * 64, :]
                if d == TIE_K[sl]:
                    w = tied(w, TIE_W)
                t = _dot(x[:, k * 128:(k + 1) * 128], _tob(w))
                early[key] = t if k == 0 else t + early[key]

        def slot_of(p, m, hh):
            return m * 2 + hh

        def project(p, di):
            m, hh = mord[di // 2], di % 2
            if (p, m, hh) in early:
                r = early[p, m, hh]
            else:
                clock[0] += 1
                r = _dot(x, _tob(tied(wqkv[2 * (p * 3 + m) + hh], TIE_KT[odd][di] * 8 + TIE_W)))
            b0 = slot_of(p, m, hh) * 40
            stg[odd * NP + p, b0:b0 + 8, :] = r[0:8]
            stg[odd * NP + p, b0 + 16:b0 + 40, :] = r[8:32]
            if m > 0:
                stg[odd * NP + p, b0 + 8:b0 + 16, :] = pre[p * 3 + m, ci, sl * 16 + hh * 8:sl * 16 + hh * 8 + 8, :]

        def mxu_rows(p, a):
            if p < NV2[odd]:
                return jnp.concatenate([a[0:8], a[32:40], a[16:32], a[48:64]], axis=0)
            return a

        def operand(p, m):
            b0 = slot_of(p, m, 0) * 40
            if m > 0:
                a = stg[odd * NP + p, b0:b0 + 80, :]
            else:
                a = mxu_rows(p, jnp.concatenate([stg[odd * NP + p, b0:b0 + 8, :], stg[odd * NP + p, b0 + 16:b0 + 48, :],
                                                 stg[odd * NP + p, b0 + 56:b0 + 80, :]], axis=0))
            return a.astype(bf16)

        def vpu_rows(p, hh, lv, g):
            gb = VGB[sl][lv]
            r0 = sl * 16 + hh * 8

            def row(m, i):
                b0 = slot_of(p, m, hh) * 40 + 8 + 8 * lv - i
                return stg[odd * NP + p, b0:b0 + 8, :]

            if g == 0:
                q = pre[p * 3, ci, r0:r0 + 8, :] if lv == 0 else row(0, 0)
                vs[p, hh, lv] = (q * CEXP, None, None, None)
            q, m_old, l, o = vs[p, hh, lv]
            i0, n = gb[g], gb[g + 1] - gb[g]

            def rows(m):
                return jnp.concatenate([row(m, i0 + i) for i in range(n)], axis=0).reshape(n, 8, 128)

            s = jnp.sum(q[None] * rows(1), axis=-1, keepdims=True)
            if i0 + n > 9 + 8 * lv:
                ok = (lax.broadcasted_iota(i32, (n, 8, 1), 1)
                      >= lax.broadcasted_iota(i32, (n, 8, 1), 0) + (i0 - 8 - 8 * lv))
                s = jnp.where(ok, s, NEG)
            mx = jnp.max(s, axis=0)
            if m_old is not None:
                mx = jnp.maximum(mx, m_old)
            e = jnp.exp2(s - mx[None])
            el, ev = jnp.sum(e, axis=0), jnp.sum(e * rows(2), axis=0)
            if m_old is None:
                l, o = el, ev
            else:
                alpha = jnp.exp2(m_old - mx)
                l, o = l * alpha + el, o * alpha + ev
            if g == len(gb) - 2:
                o = o * pl.reciprocal(l, approx=True)
                if lv == 0:
                    stg[orow(H + 2 * p + hh, (1 - odd) * 8, 8)] = o
                else:
                    stg[orow(2 * p + hh, 8, 8)] = o
            vs[p, hh, lv] = (q, mx, l, o)
            return _zero_of(o)

        def scores(p):
            if not 0 <= p < NP:
                return
            sc = jnp.where(mxu_rows(p, mask_ref[...]) > 0.5, _dot_t(operand(p, 0), operand(p, 1)), NEG)
            n = sc.shape[0]
            mx = jnp.max(sc, axis=-1, keepdims=True)
            sst[p % 2, 0:n] = sc
            e = jnp.exp2((sst[p % 2, 0:n] - mx) * CEXP)
            l = jnp.sum(e, axis=-1, keepdims=True)
            sst[2 + p % 2, 0:n] = e
            probs[p] = (sst[2 + p % 2, 0:n] * pl.reciprocal(l, approx=True)).astype(bf16)

        def attend(p):
            if not 0 <= p < NP:
                return
            o = _dot(probs[p], operand(p, 2))
            attended.add(p)
            for hh in range(2):
                if p < NV2[odd]:
                    stg[orow(2 * p + hh, 0, 8)] = o[hh * 8:hh * 8 + 8]
                    stg[orow(2 * p + hh, 16, 16)] = o[16 + hh * 16:32 + hh * 16]
                else:
                    stg[orow(2 * p + hh, 0, 32)] = o[hh * 32:(hh + 1) * 32]

        def oheads(h0, h1):
            assert (h1 - 1) // 2 in attended
            vforce((sl, h1 - 1))
            if not odd:
                return jnp.concatenate([stg[orow(h, 0, 32)] for h in range(h0, h1)], axis=1)
            return o48(h0, h1)

        for slot in range(NP):
            for di in range(7):
                if di == (POS_B0[sl] if slot == LAG_B else POS_B):
                    scores(slot - LAG_B)
                if di == POS_D:
                    attend(slot - LAG_D)
                if di < 6:
                    project(slot, di)
            for hh in range(2):
                for lv in ((1, 0) if slot < NV2[odd] else (0,)):
                    for g in range(len(VGB[sl][lv]) - 1):
                        vq.append((clock[0] + LAG_V, lambda a=(slot, hh, lv, g): vpu_rows(*a),
                                   (sl if lv == 1 else sl | 1, 2 * slot + hh)))
        tiles, credit = 0, 0.0
        acc = [None] * NJ
        for i in range(len(eb) - 1):
            h0, h1 = eb[i], eb[i + 1]
            o2 = oheads(h0, h1).astype(bf16)
            for j in range(NJ):
                ws = []
                for h in range(h0, h1):
                    tiles += 1
                    if tiles % (3 if odd else 5) == 0:
                        clock[0] += 1
                    w = wo[j, h * 64:(h + 1) * 64, :]
                    if odd:
                        credit += E_RATE
                        if credit >= 1.0:
                            credit -= 1.0
                            w = tied(w, TIE_E[sl])
                    ws.append(w)
                t = _dot(o2, _tob(jnp.concatenate(ws, axis=0)))
                acc[j] = t if acc[j] is None else t + acc[j]
                if j == EPOS[sl][0]:
                    scores(NP + i - LAG_B)
                if j == EPOS[sl][1]:
                    attend(NP + i - LAG_D)
        if sl == CH - 1:
            accv[...] = jnp.concatenate(acc, axis=1)
            vforce((sl, H))
            assert not vq and len(attended) == NP
            return None
        return finish(ci, sl, acc)

    def out_cp(*idx):
        return pltpu.make_async_copy(outv.at[idx], out_hbm.at[idx], sem_out.at[0])

    def chunk(ci, carry):
        prev = jnp.maximum(ci - 1, 0)
        mem = finish_last(prev)

        @pl.when(ci >= 1)
        def _():
            out_cp(prev, pl.ds(2, 2)).start()

        for sl in range(CH):
            mem = step(ci, sl, mem)
            if sl == 1:
                out_cp(ci, pl.ds(0, 2)).start()
        return carry

    lax.fori_loop(0, NCH, chunk, 0)
    o2 = o48(HL, H).astype(bf16)
    for j in range(NJ):
        c0, c1 = j * 128, (j + 1) * 128
        t = _dot(o2, _tob(wo[j, HL * 64:, :])) + accv[:, c0:c1]
        finalize(NCH - 1, CH - 1, 8, SEG, t[8:32], c0, c1)
        finalize(NCH - 1, CH - 1, 0, 8, t[32:40], c0, c1)
        finalize(NCH - 1, CH - 2, 0, 8, t[40:48], c0, c1)
        out_cp(NCH - 1, pl.ds(2, 2), slice(None), pl.ds(c0, 128)).start()
    pltpu.make_async_copy(outv, out_hbm, sem_out.at[0]).wait()


@jax.jit
def pallas_recurrent_scan__memory_aug_recurrent_mem_tr__moe_arch_mod__prompt_kernel(
    A_x, A_mem0, A_Wq, A_Wk, A_Wv, A_Wo, A_seg_len, B_x, B_w_r, B_w_gate, B_w_up, B_w_down,
):
    hbm = pl.BlockSpec(memory_space=pltpu.MemorySpace.HBM)
    out = pl.pallas_call(
        _kernel,
        out_shape=jax.ShapeDtypeStruct((NCH, CH, SEG, D), bf16),
        in_specs=[hbm] * 10,
        out_specs=hbm,
        scratch_shapes=[
            pltpu.VMEM((NCH, CH, SEG, D), bf16),
            pltpu.VMEM((NCH, CH * 16, D), u32),
            pltpu.VMEM((4, 64, D), u32),
            pltpu.VMEM((5, 128, 256), u32),
            pltpu.VMEM((5, 128, 128), u32),
            pltpu.VMEM((NCH, CH * SEG, D), f32),
            pltpu.VMEM((NU, D, 128), u32),
            pltpu.VMEM((NU * 2, D // 2, 128), u32),
            pltpu.VMEM((NJ, H * DH // 2, 128), u32),
            pltpu.VMEM((NU, NCH, CH * 16, 128), f32),
            pltpu.VMEM((2 * NP, 352, 128), f32),
            pltpu.VMEM((4, 64, 80), f32),
            pltpu.VMEM((F, D), bf16),
            pltpu.VMEM((F, D), bf16),
            pltpu.VMEM((F, D), bf16),
            pltpu.VMEM((NCH, CH, SEG, D), bf16),
            pltpu.VMEM((64, 80), f32),
            pltpu.VMEM((48, D), f32),
            pltpu.VMEM((NPL, 8, 128), f32),
            pltpu.VMEM((8, 1024), f32),
            pltpu.VMEM((M, D), bf16),
            pltpu.VMEM((D,), bf16),
            pltpu.SemaphoreType.DMA((len(GROUPS) + 1,)),
            pltpu.SemaphoreType.DMA((1,)),
        ],
        compiler_params=pltpu.CompilerParams(
            vmem_limit_bytes=100 * 1024 * 1024,
            disable_bounds_checks=True,
            disable_semaphore_checks=True,
            internal_scratch_in_bytes=48 * 1024,
        ),
        name="rmt_mod",
    )(A_x.reshape(NCH, CH, SEG, D), A_mem0.reshape(M, D), A_Wq, A_Wk, A_Wv, A_Wo.reshape(H * DH, D),
      B_w_r, B_w_gate.T, B_w_up.T, B_w_down)
    return out.reshape(1, S, D)
```
